```python
import jax
import jax.numpy as jnp

def _softmax(x, axis=-1):
    return jax.nn.softmax(x, axis=axis)
def _gelu(x):
    return jax.nn.gelu(x, approximate=True)
def _silu(x):
    return jax.nn.silu(x)
def _sigmoid(x):
    return jax.nn.sigmoid(x)
def _layernorm(x, axis=-1, eps=1e-5):
    m = jnp.mean(x, axis=axis, keepdims=True)
    v = jnp.var(x, axis=axis, keepdims=True)
    return (x - m) / jnp.sqrt(v + eps)
def _scatter_add(tgt, idx, src, axis=0):
    return tgt.at[idx].add(src)
def _segment_sum(src, seg, n):
    return jax.ops.segment_sum(src, seg, n)
class _Rng:
    def __init__(self, key):
        self._k = key
    def _next(self):
        self._k, sub = jax.random.split(self._k)
        return sub
    def normal(self, shape):
        return jax.random.normal(self._next(), shape, dtype=jnp.bfloat16)
    def randint(self, lo, hi, shape):
        return jax.random.randint(self._next(), shape, lo, hi, dtype=jnp.int32)
    def uniform(self, shape, lo=0.0, hi=1.0):
        return jax.random.uniform(self._next(), shape, jnp.bfloat16, lo, hi)
    def permutation(self, n):
        return jax.random.permutation(self._next(), n)


kernel_name = 'parallel_sum__sliding_local_dilated__mixer_token_mlp__prompt'

def setup_inputs():
    _rng = _Rng(jax.random.key(int.from_bytes(__import__("os").urandom(4), "little")))
    _w = (lambda a: (lambda t: t.astype(jnp.bfloat16) if jnp.issubdtype(t.dtype, jnp.floating) else t)(jnp.asarray(a)))
    def _A_setup():
        B, S, D = 1, 2048, 448
        return {
            "x": _w((lambda *s: _rng.normal(s) * 0.05)(B, S, D)),
            "wqkv": _w((lambda *s: _rng.normal(s) * 0.05)(D, 3 * D)),
            "wo": _w((lambda *s: _rng.normal(s) * 0.05)(D, D)),
        }
    _A_in = _A_setup()

    def _B_setup():
        B, S, D, F = 1, 2048, 448, 1792
        return {
            "x": _w((lambda *s: _rng.normal(s) * 0.05)(B, S, D)),
            "w1": _w((lambda *s: _rng.normal(s) * 0.05)(S, F) * (S ** -0.5)),
            "b1": _w((lambda *s: _rng.normal(s) * 0.05)(F) * 0.02),
            "w2": _w((lambda *s: _rng.normal(s) * 0.05)(F, S) * (F ** -0.5)),
            "b2": _w((lambda *s: _rng.normal(s) * 0.05)(S) * 0.02),
        }
    _B_in = _B_setup()

    return {
        "A_x": _A_in["x"],
        "A_wqkv": _A_in["wqkv"],
        "A_wo": _A_in["wo"],
        "B_x": _B_in["x"],
        "B_w1": _B_in["w1"],
        "B_b1": _B_in["b1"],
        "B_w2": _B_in["w2"],
        "B_b2": _B_in["b2"],
    }

def reference(A_x, A_wqkv, A_wo, B_x, B_w1, B_b1, B_w2, B_b2):
    def _A_ref(x, wqkv, wo):
        B, S, D = x.shape
        H = 16; Dh = D // H
        W, dil = 8, 2
        qkv = (lambda x, *d: x.transpose(*d))((x @ wqkv).reshape(B, S, 3, H, Dh), 2, 0, 3, 1, 4)
        q, k, v = qkv[0], qkv[1], qkv[2]
        scale = Dh ** -0.5
        pos = jnp.arange(S)
        off = jnp.arange(W) * dil
        idx = pos[:, None] - off[None, :]
        mask = idx >= 0
        idx_c = jnp.where(mask, idx, 0).reshape(-1)
        kg = k[:, :, idx_c, :].reshape(B, H, S, W, Dh)
        vg = v[:, :, idx_c, :].reshape(B, H, S, W, Dh)
        logits = jnp.einsum("bhsd,bhswd->bhsw", q, kg) * scale
        logits = jnp.where(mask[None, None, :, :], logits, -1e9)
        attn = _softmax(logits, axis=-1)
        o = jnp.einsum("bhsw,bhswd->bhsd", attn, vg)
        return (lambda x, *d: x.transpose(*d))(o, 0, 2, 1, 3).reshape(B, S, D) @ wo

    def _B_ref(x, w1, b1, w2, b2):
        B, S, D = x.shape
        h = _layernorm(x, axis=-1)
        u = jnp.einsum("bsd,sf->bdf", h, w1) + b1
        u = _gelu(u)
        y = jnp.einsum("bdf,fs->bds", u, w2) + b2
        return (lambda x, *d: x.transpose(*d))(y, 0, 2, 1)

    x = A_x
    xn = _layernorm(x, axis=-1)
    return x + _A_ref(xn, A_wqkv, A_wo) + _B_ref(xn, B_w1, B_b1, B_w2, B_b2)
```

```python
import jax
import jax.numpy as jnp
import jax.experimental.pallas as pl
import jax.experimental.pallas.tpu as pltpu

S = 2048
D = 448
F = 1792
H = 16
DH = D // H
WIN = 8
DIL = 2
EPS = 1e-5
LANES = 128
NT = S // LANES
F32 = jnp.float32
BF16 = jnp.bfloat16

P1_CHUNK = 256
P2_CHUNK = 512
P3_CHUNK = 512


def _dot(a, b):
    return jnp.dot(a, b, preferred_element_type=F32)


def _layernorm_t(x):
    m = jnp.mean(x, axis=0, keepdims=True)
    xc = x - m
    v = jnp.mean(xc * xc, axis=0, keepdims=True)
    return xc * jax.lax.rsqrt(v + EPS)


def _gelu(x):
    c = 0.7978845608028654
    inner = x * (c + (c * 0.044715) * (x * x))
    hx = 0.5 * x
    return hx + hx * jnp.tanh(inner)


def _kernel(x_hbm, wqkv_hbm, wo_hbm, w1_hbm, b1_hbm, w2_hbm, b2_hbm, out_hbm,
            x_v, w1_v, w2_v, wqkv_v, wo_v, b1_v, b2_v,
            xn_s, h_s, u_s, g_s, wt_s, wot_s, t32, o32, qkv_s, l_s, p_s, o8_s, o_s, out_v,
            sem_x, sem_w1, sem_misc, sem_out):
    n1 = S // P1_CHUNK

    def x_copy(i):
        return pltpu.make_async_copy(x_hbm.at[:, pl.ds(i * P1_CHUNK, P1_CHUNK)],
                                     x_v.at[:, pl.ds(i * P1_CHUNK, P1_CHUNK)], sem_x.at[i])

    def w1_copy(i):
        return pltpu.make_async_copy(w1_hbm.at[pl.ds(i * P1_CHUNK, P1_CHUNK), :],
                                     w1_v.at[pl.ds(i * P1_CHUNK, P1_CHUNK), :], sem_w1.at[i])

    c_b1 = pltpu.make_async_copy(b1_hbm, b1_v, sem_misc.at[0])
    c_b2 = pltpu.make_async_copy(b2_hbm, b2_v, sem_misc.at[1])
    c_wqkv = pltpu.make_async_copy(wqkv_hbm, wqkv_v, sem_misc.at[2])
    c_wo = pltpu.make_async_copy(wo_hbm, wo_v, sem_misc.at[3])
    c_w2 = pltpu.make_async_copy(w2_hbm, w2_v, sem_misc.at[4])

    x_copy(0).start()
    w1_copy(0).start()
    for i in range(1, n1):
        x_copy(i).start()
        w1_copy(i).start()
    c_b1.start()
    c_b2.start()
    c_wqkv.start()
    c_wo.start()
    c_w2.start()

    def ln_tile(col):
        x = x_v[:, pl.ds(col, LANES)].astype(F32)
        xn = _layernorm_t(x)
        xn_s[:, pl.ds(col, LANES)] = xn.astype(BF16)
        h_s[:, pl.ds(col, LANES)] = _layernorm_t(xn).astype(BF16)

    def ln_chunk(col0):
        for j in range(P1_CHUNK // LANES):
            c = col0 + j * LANES
            if not isinstance(c, int):
                c = pl.multiple_of(c, LANES)
            ln_tile(c)

    x_copy(0).wait()
    ln_chunk(0)

    def wprep():
        for c in range(4):
            r = min(LANES, D - c * LANES)
            blk = wqkv_v[pl.ds(c * LANES, r), :].astype(F32)
            t32[c, :, pl.ds(0, r)] = blk.T
        for p in range(3):
            for d in range(DH):
                for c in range(4):
                    r = min(LANES, D - c * LANES)
                    v = t32[c, pl.ds(p * D + d, H, stride=DH), :]
                    wt_s[pl.ds(p * D + d * H, H), pl.ds(c * LANES, r)] = v[:, :r].astype(BF16)
        for c in range(4):
            r = min(LANES, D - c * LANES)
            o32[c, :, pl.ds(0, r)] = wo_v[:, pl.ds(c * LANES, r)].astype(F32)
        for c in range(4):
            r = min(LANES, D - c * LANES)
            rows = jnp.concatenate(
                [o32[c, pl.ds(d, H, stride=DH), pl.ds(0, r)] for d in range(DH)], axis=0)
            wot_s[pl.ds(c * LANES, r), :] = rows.T.astype(BF16)

    for i in range(n1):
        w1_copy(i).wait()
        if i + 1 < n1:
            x_copy(i + 1).wait()
        if i == n1 - 1:
            c_wqkv.wait()
            c_wo.wait()
        off = i * P1_CHUNK
        part = _dot(h_s[:, pl.ds(off, P1_CHUNK)], w1_v[pl.ds(off, P1_CHUNK), :])
        if i == 0:
            u_s[...] = part
        else:
            u_s[...] += part
        if i + 1 < n1:
            ln_chunk(off + P1_CHUNK)
        else:
            wprep()

    c_b1.wait()
    c_b2.wait()
    lane = jax.lax.broadcasted_iota(jnp.int32, (H, LANES), 1)
    scale = DH ** -0.5

    def shift_back(prev, cur, a):
        return pltpu.roll(jnp.where(lane >= LANES - a, prev, cur), a, 1)

    def shift_fwd(cur, nxt, b):
        return pltpu.roll(jnp.where(lane < b, nxt, cur), LANES - b, 1)

    def s1_tile(t):
        tn = min(t + 1, NT - 1)
        tp = max(t - 1, 0)
        acc = [None] * WIN
        for d in range(DH):
            rq = pl.ds(d * H, H)
            rk = pl.ds(D + d * H, H)
            q0 = qkv_s[t, rq, :]
            q8 = shift_fwd(q0, qkv_s[tn, rq, :], 8)
            k0 = qkv_s[t, rk, :]
            kp = qkv_s[tp, rk, :]
            ks = [k0] + [shift_back(kp, k0, a) for a in (2, 4, 6)]
            for a in range(4):
                t0 = q0 * ks[a]
                t8 = q8 * ks[a]
                acc[a] = t0 if d == 0 else acc[a] + t0
                acc[4 + a] = t8 if d == 0 else acc[4 + a] + t8
        for a in range(4):
            l_s[t, pl.ds(a * H, H), :] = acc[4 + a]
        lg = [acc[a] for a in range(4)]
        for a in range(4):
            lg.append(shift_back(l_s[tp, pl.ds(a * H, H), :], acc[4 + a], 8))
        lg = [v * scale for v in lg]
        if t == 0:
            lg = [lg[0]] + [jnp.where(lane >= DIL * j, lg[j], -1e9) for j in range(1, WIN)]
        m = lg[0]
        for j in range(1, WIN):
            m = jnp.maximum(m, lg[j])
        e = [jnp.exp(v - m) for v in lg]
        ssum = e[0]
        for j in range(1, WIN):
            ssum = ssum + e[j]
        inv = 1.0 / ssum
        for j in range(WIN):
            p_s[t, pl.ds(j * H, H), :] = e[j] * inv

    def proj(rows0, nrows, blk):
        res = _dot(wt_s[pl.ds(rows0, nrows), :], xn_s[:, pl.ds(blk * P2_CHUNK, P2_CHUNK)])
        for j in range(P2_CHUNK // LANES):
            qkv_s[blk * (P2_CHUNK // LANES) + j, pl.ds(rows0, nrows), :] = res[:, j * LANES:(j + 1) * LANES]

    n2 = S // P2_CHUNK
    tpb = P2_CHUNK // LANES
    b1 = b1_v[...].astype(F32).reshape(1, F)
    grows = D // (2 * n2)
    grows = 64
    gchunks = list(range(D // grows))

    def gelu_chunk(c):
        r = pl.ds(c * grows, grows)
        g_s[r, :] = _gelu(u_s[r, :] + b1).astype(BF16)

    done_t = 0
    for blk in range(n2):
        proj(0, 2 * D, blk)
        gelu_chunk(gchunks.pop(0))
        lim = blk * tpb - 1
        while done_t < lim:
            s1_tile(done_t)
            done_t += 1
    for blk in range(n2):
        proj(2 * D, D, blk)
        if gchunks:
            gelu_chunk(gchunks.pop(0))
        for _ in range(2):
            if done_t < NT:
                s1_tile(done_t)
                done_t += 1
    assert done_t == NT and not gchunks

    c_w2.wait()
    o8_s[...] = jnp.zeros_like(o8_s)
    n3 = S // P3_CHUNK
    tp3 = P3_CHUNK // LANES

    def out_copy(i):
        col = pl.multiple_of(i * P3_CHUNK, P3_CHUNK)
        return pltpu.make_async_copy(out_v.at[:, pl.ds(col, P3_CHUNK)],
                                     out_hbm.at[:, pl.ds(col, P3_CHUNK)], sem_out.at[i])

    def s2_tile(t, j):
        tn = jnp.minimum(t + 1, NT - 1)
        tp = jnp.maximum(t - 1, 0)
        p0 = [p_s[t, pl.ds(a * H, H), :] for a in range(4)]
        p8 = [shift_fwd(p_s[t, pl.ds((4 + a) * H, H), :], p_s[tn, pl.ds((4 + a) * H, H), :], 8)
              for a in range(4)]
        for d in range(DH):
            rv = pl.ds(2 * D + d * H, H)
            r = pl.ds(d * H, H)
            v0 = qkv_s[t, rv, :]
            vp = qkv_s[tp, rv, :]
            vs = [v0] + [shift_back(vp, v0, a) for a in (2, 4, 6)]
            o0 = (p0[0] * vs[0] + p0[1] * vs[1]) + (p0[2] * vs[2] + p0[3] * vs[3])
            o8 = (p8[0] * vs[0] + p8[1] * vs[1]) + (p8[2] * vs[2] + p8[3] * vs[3])
            o = o0 + shift_back(o8_s[r, :], o8, 8)
            o8_s[r, :] = o8
            o_s[r, pl.ds(j * LANES, LANES)] = o.astype(BF16)

    def p3_body(i, carry):
        col = pl.multiple_of(i * P3_CHUNK, P3_CHUNK)
        for j in range(tp3):
            s2_tile(i * tp3 + j, j)
        y = _dot(g_s[...], w2_v[:, pl.ds(col, P3_CHUNK)])
        y = y + _dot(wot_s[...], o_s[...])
        b2 = b2_v[pl.ds(col, P3_CHUNK)].astype(F32).reshape(1, P3_CHUNK)
        res = x_v[:, pl.ds(col, P3_CHUNK)].astype(F32) + (y + b2)
        out_v[:, pl.ds(col, P3_CHUNK)] = res.astype(BF16)
        out_copy(i).start()
        return carry

    jax.lax.fori_loop(0, n3, p3_body, 0)
    for i in range(n3):
        out_copy(i).wait()


@jax.jit
def pallas_parallel_sum__sliding_local_dilated__mixer_token_mlp__prompt_kernel(
    A_x: jax.Array,
    A_wqkv: jax.Array,
    A_wo: jax.Array,
    B_x: jax.Array,
    B_w1: jax.Array,
    B_b1: jax.Array,
    B_w2: jax.Array,
    B_b2: jax.Array,
):
    del B_x
    xt = jnp.transpose(A_x[0], (1, 0))
    any_spec = pl.BlockSpec(memory_space=pl.ANY)
    out_t = pl.pallas_call(
        _kernel,
        out_shape=jax.ShapeDtypeStruct((D, S), BF16),
        in_specs=[any_spec] * 7,
        out_specs=any_spec,
        scratch_shapes=[
            pltpu.VMEM((D, S), BF16),
            pltpu.VMEM((S, F), BF16),
            pltpu.VMEM((F, S), BF16),
            pltpu.VMEM((D, 3 * D), BF16),
            pltpu.VMEM((D, D), BF16),
            pltpu.VMEM((F,), BF16),
            pltpu.VMEM((S,), BF16),
            pltpu.VMEM((D, S), BF16),
            pltpu.VMEM((D, S), BF16),
            pltpu.VMEM((D, F), F32),
            pltpu.VMEM((D, F), BF16),
            pltpu.VMEM((3 * D, D), BF16),
            pltpu.VMEM((D, D), BF16),
            pltpu.VMEM((4, 3 * D, LANES), F32),
            pltpu.VMEM((4, D, LANES), F32),
            pltpu.VMEM((NT, 3 * D, LANES), F32),
            pltpu.VMEM((NT, 4 * H, LANES), F32),
            pltpu.VMEM((NT, WIN * H, LANES), F32),
            pltpu.VMEM((D, LANES), F32),
            pltpu.VMEM((D, P3_CHUNK), BF16),
            pltpu.VMEM((D, S), BF16),
            pltpu.SemaphoreType.DMA((S // P1_CHUNK,)),
            pltpu.SemaphoreType.DMA((S // P1_CHUNK,)),
            pltpu.SemaphoreType.DMA((5,)),
            pltpu.SemaphoreType.DMA((S // P3_CHUNK,)),
        ],
        compiler_params=pltpu.CompilerParams(vmem_limit_bytes=100 * 1024 * 1024),
    )(xt, A_wqkv, A_wo, B_w1, B_b1, B_w2, B_b2)
    return jnp.transpose(out_t, (1, 0))[None]
```

```python
import jax
import jax.numpy as jnp
import jax.experimental.pallas as pl
import jax.experimental.pallas.tpu as pltpu

S = 2048
D = 448
F = 1792
H = 16
DH = D // H
WIN = 8
DIL = 2
EPS = 1e-5
LANES = 128
NT = S // LANES
NF = F // LANES
F32 = jnp.float32
BF16 = jnp.bfloat16

P1_T = 2
P2_T = 4
P3_T = 2
S2_EARLY = 4
N1 = NT // P1_T


def _dot(a, b):
    return jnp.dot(a, b, preferred_element_type=F32)


def _gelu(x):
    c = 0.7978845608028654
    inner = x * (c + (c * 0.044715) * (x * x))
    hx = 0.5 * x
    return hx + hx * jnp.tanh(inner)


def _u_at(j):
    return (NT + j // 3, (j % 3) * D)


def _kernel(x_hbm, wqkv_hbm, wo_hbm, w1_hbm, b1_hbm, w2_hbm, b2_hbm, out_hbm,
            x_v, w1_v, w2_v, wqkv_v, wo_v, b1_v, b2_v,
            xn_s, h_s, g_s, wt_s, wot_s, t32, o32, qkv_s, l_s, p_s, o8_s, o_s, out_v, z_s,
            sem_x, sem_w1, sem_misc, sem_out):
    c1 = P1_T * LANES

    def x_copy(t):
        col = t * LANES if isinstance(t, int) else pl.multiple_of(t * LANES, LANES)
        return pltpu.make_async_copy(x_hbm.at[:, pl.ds(col, LANES)], x_v.at[t], sem_x.at[t])

    def w1_copy(i):
        row = i * c1 if isinstance(i, int) else pl.multiple_of(i * c1, c1)
        return pltpu.make_async_copy(w1_hbm.at[pl.ds(row, c1), :], w1_v.at[pl.ds(row, c1), :],
                                     sem_w1.at[i])

    c_b1 = pltpu.make_async_copy(b1_hbm, b1_v, sem_misc.at[0])
    c_b2 = pltpu.make_async_copy(b2_hbm, b2_v, sem_misc.at[1])
    c_wqkv = pltpu.make_async_copy(wqkv_hbm, wqkv_v, sem_misc.at[2])
    c_wo = pltpu.make_async_copy(wo_hbm, wo_v, sem_misc.at[3])
    c_w2 = pltpu.make_async_copy(w2_hbm, w2_v, sem_misc.at[4])

    for i in range(N1):
        for j in range(P1_T):
            x_copy(i * P1_T + j).start()
        w1_copy(i).start()
    c_b1.start()
    c_b2.start()
    c_wqkv.start()
    c_wo.start()
    c_w2.start()

    for j in range(NF):
        ti, r0 = _u_at(j)
        qkv_s[ti, pl.ds(r0, D), :] = jnp.zeros((D, LANES), F32)
    z_s[...] = jnp.zeros_like(z_s)
    o8_s[...] = jnp.zeros_like(o8_s)

    def make_tie(zi):
        never = z_s[zi] != 0.0

        def tie(val, src):
            return jnp.where(never, src, val)
        return tie

    def colsum(slabs, init):
        a = [init, None]
        for d, v in enumerate(slabs):
            k = d % 2
            a[k] = v if a[k] is None else a[k] + v
        return jnp.sum(a[0] + a[1], axis=0, keepdims=True) * (1.0 / D)

    def ln_pass(src, t, dst, init):
        def ld(d):
            return src[t, pl.ds(d * H, H), :].astype(F32)
        m = colsum((ld(d) for d in range(DH)), init)
        m = jnp.broadcast_to(m, (H, LANES))

        def sq(d):
            c = ld(d) - m
            return c * c
        v = colsum((sq(d) for d in range(DH)), None)
        r = jnp.broadcast_to(jax.lax.rsqrt(v + EPS), (H, LANES))
        for d in range(DH):
            dst[t, pl.ds(d * H, H), :] = ((ld(d) - m) * r).astype(BF16)

    def ln_tile(t, init):
        ln_pass(x_v, t, xn_s, init)
        ln_pass(xn_s, t, h_s, None)

    def mixer1(i):
        row = i * c1 if isinstance(i, int) else pl.multiple_of(i * c1, c1)
        h = jnp.concatenate([h_s[i * P1_T + j] for j in range(P1_T)], axis=1)
        part = _dot(h, w1_v[pl.ds(row, c1), :])
        for j in range(NF):
            ti, r0 = _u_at(j)
            qkv_s[ti, pl.ds(r0, D), :] += part[:, j * LANES:(j + 1) * LANES]
        return part

    zeros16 = jnp.zeros((H, LANES), F32)

    for j in range(P1_T):
        x_copy(j).wait()
    for j in range(P1_T):
        ln_tile(j, None)

    def p1_body(i, carry):
        w1_copy(i).wait()
        for j in range(P1_T):
            x_copy((i + 1) * P1_T + j).wait()
        tie = make_tie(jnp.minimum(i, 1))
        part = mixer1(i)
        for j in range(P1_T):
            cj = (1 + 5 * j) * LANES
            ln_tile((i + 1) * P1_T + j, tie(zeros16, part[0:H, cj:cj + LANES]))
        return carry

    jax.lax.fori_loop(0, N1 - 1, p1_body, 0)

    w1_copy(N1 - 1).wait()
    c_wqkv.wait()
    c_wo.wait()
    c_b1.wait()
    c_b2.wait()
    tie = make_tie(0)
    part = mixer1(N1 - 1)

    k = 0
    for c in range(4):
        r = min(LANES, D - c * LANES)
        for j in range(11):
            n = min(LANES, 3 * D - j * LANES)
            blk = wqkv_v[pl.ds(c * LANES, r), pl.ds(j * LANES, n)].astype(F32)
            col = (k // 8) * LANES
            row = (k % 8) * 3 * H
            blk = jnp.concatenate([tie(blk[0:H], part[row:row + H, col:col + LANES][:, :n])
                                   if n == LANES else blk[0:H], blk[H:]], axis=0)
            t32[c, pl.ds(j * LANES, n), pl.ds(0, r)] = blk.T
            k += 1
    for p in range(3):
        for d in range(DH):
            for c in range(4):
                r = min(LANES, D - c * LANES)
                v = t32[c, pl.ds(p * D + d, H, stride=DH), :]
                wt_s[pl.ds(p * D + d * H, H), pl.ds(c * LANES, r)] = v[:, :r].astype(BF16)

    lane = jax.lax.broadcasted_iota(jnp.int32, (H, LANES), 1)
    scale = DH ** -0.5

    def shift_back(prev, cur, a):
        return pltpu.roll(jnp.where(lane >= LANES - a, prev, cur), a, 1)

    def shift_fwd(cur, nxt, b):
        return pltpu.roll(jnp.where(lane < b, nxt, cur), LANES - b, 1)

    def s1_tile(t):
        tn = min(t + 1, NT - 1)
        tp = max(t - 1, 0)
        acc = [None] * WIN
        for d in range(DH):
            rq = pl.ds(d * H, H)
            rk = pl.ds(D + d * H, H)
            q0 = qkv_s[t, rq, :]
            q8 = shift_fwd(q0, qkv_s[tn, rq, :], 8)
            k0 = qkv_s[t, rk, :]
            kp = qkv_s[tp, rk, :]
            ks = [k0] + [shift_back(kp, k0, a) for a in (2, 4, 6)]
            for a in range(4):
                t0 = q0 * ks[a]
                t8 = q8 * ks[a]
                acc[a] = t0 if d == 0 else acc[a] + t0
                acc[4 + a] = t8 if d == 0 else acc[4 + a] + t8
        for a in range(4):
            l_s[t, pl.ds(a * H, H), :] = acc[4 + a]
        lg = [acc[a] for a in range(4)]
        for a in range(4):
            lg.append(shift_back(l_s[tp, pl.ds(a * H, H), :], acc[4 + a], 8))
        lg = [v * scale for v in lg]
        if t == 0:
            lg = [lg[0]] + [jnp.where(lane >= DIL * j, lg[j], -1e9) for j in range(1, WIN)]
        m = lg[0]
        for j in range(1, WIN):
            m = jnp.maximum(m, lg[j])
        e = [jnp.exp(v - m) for v in lg]
        ssum = e[0]
        for j in range(1, WIN):
            ssum = ssum + e[j]
        inv = 1.0 / ssum
        for j in range(WIN):
            p_s[t, pl.ds(j * H, H), :] = e[j] * inv

    def s2_tile(t, src):
        tn = min(t + 1, NT - 1)
        tp = max(t - 1, 0)
        p0 = [p_s[t, pl.ds(a * H, H), :] for a in range(4)]
        p8 = [p_s[t, pl.ds((4 + a) * H, H), :] for a in range(4)]
        if src is not None:
            p0 = [tie(v, src) for v in p0]
            p8 = [tie(v, src) for v in p8]
        p8 = [shift_fwd(p8[a], p_s[tn, pl.ds((4 + a) * H, H), :], 8) for a in range(4)]
        for d in range(DH):
            rv = pl.ds(2 * D + d * H, H)
            r = pl.ds(d * H, H)
            v0 = qkv_s[t, rv, :]
            vp = qkv_s[tp, rv, :]
            vs = [v0] + [shift_back(vp, v0, a) for a in (2, 4, 6)]
            o0 = (p0[0] * vs[0] + p0[1] * vs[1]) + (p0[2] * vs[2] + p0[3] * vs[3])
            o8 = (p8[0] * vs[0] + p8[1] * vs[1]) + (p8[2] * vs[2] + p8[3] * vs[3])
            o = o0 + shift_back(o8_s[r, :], o8, 8)
            o8_s[r, :] = o8
            o_s[t, r, :] = o.astype(BF16)

    def proj(rows0, nrows, blk):
        xn = jnp.concatenate([xn_s[blk * P2_T + j] for j in range(P2_T)], axis=1)
        res = _dot(wt_s[pl.ds(rows0, nrows), :], xn)
        for j in range(P2_T):
            qkv_s[blk * P2_T + j, pl.ds(rows0, nrows), :] = res[:, j * LANES:(j + 1) * LANES]
        return res

    b1 = b1_v[...].astype(F32).reshape(1, F)
    GR = 64
    gelu_jobs = [(j, rr) for j in range(NF) for rr in range(D // GR)]

    def gelu_job(j, rr, src):
        ti, r0 = _u_at(j)
        bias = tie(jnp.broadcast_to(b1[:, j * LANES:(j + 1) * LANES], (H, LANES)), src)
        for q in range(GR // H):
            row = rr * GR + q * H
            g_s[j, pl.ds(row, H), :] = _gelu(qkv_s[ti, pl.ds(r0 + row, H), :] + bias).astype(BF16)

    def spread_gelu(res, njobs):
        nrows, ncols = res.shape
        nslab = (nrows // H) * (ncols // LANES)
        for k in range(njobs):
            if not gelu_jobs:
                return
            pos = (k * nslab) // njobs
            col, row = (pos // (nrows // H)) * LANES, (pos % (nrows // H)) * H
            gelu_job(*gelu_jobs.pop(0), res[row:row + H, col:col + LANES])

    def wo_prep(res):
        for c in range(4):
            r = min(LANES, D - c * LANES)
            blk = wo_v[:, pl.ds(c * LANES, r)].astype(F32)
            o32[c, :, pl.ds(0, r)] = blk
        for c in range(4):
            r = min(LANES, D - c * LANES)
            rows = jnp.concatenate(
                [o32[c, pl.ds(d, H, stride=DH), pl.ds(0, r)] for d in range(DH)], axis=0)
            wot_s[pl.ds(c * LANES, r), :] = rows.T.astype(BF16)

    n2 = NT // P2_T
    done_t = 0
    for blk in range(n2):
        res = proj(0, 2 * D, blk)
        spread_gelu(res, 14 if blk == 0 else 8)
        lim = (blk + 1) * P2_T - 1 if blk + 1 < n2 else NT
        while done_t < lim:
            s1_tile(done_t)
            done_t += 1
    done2 = 0
    for blk in range(n2):
        res = proj(2 * D, D, blk)
        spread_gelu(res, 15)
        if blk == 1:
            wo_prep(res)
        while done2 < min(S2_EARLY, (blk + 1) * P2_T):
            s2_tile(done2, None)
            done2 += 1
    assert done_t == NT and not gelu_jobs

    c_w2.wait()
    n3 = NT // P3_T
    c3 = P3_T * LANES

    def out_copy(t):
        return pltpu.make_async_copy(out_v.at[t], out_hbm.at[:, pl.ds(t * LANES, LANES)],
                                     sem_out.at[t])

    b2 = b2_v[...].astype(F32).reshape(1, S)
    for i in range(n3):
        g = jnp.concatenate([g_s[j] for j in range(NF)], axis=1)
        y = _dot(g, w2_v[:, pl.ds(i * c3, c3)])
        for j in range(P3_T):
            if done2 < NT:
                s2_tile(done2, y[0:H, j * LANES:(j + 1) * LANES])
                done2 += 1
        o = jnp.concatenate([o_s[i * P3_T + j] for j in range(P3_T)], axis=1)
        y = _dot(wot_s[...], o) + y
        for j in range(P3_T):
            t = i * P3_T + j
            bias = jnp.broadcast_to(b2[:, t * LANES:(t + 1) * LANES], (H, LANES))
            for d in range(DH):
                r = pl.ds(d * H, H)
                val = x_v[t, r, :].astype(F32) + (y[d * H:(d + 1) * H, j * LANES:(j + 1) * LANES] + bias)
                out_v[t, r, :] = val.astype(BF16)
            out_copy(t).start()

    for t in range(NT):
        out_copy(t).wait()


@jax.jit
def pallas_parallel_sum__sliding_local_dilated__mixer_token_mlp__prompt_kernel(
    A_x: jax.Array,
    A_wqkv: jax.Array,
    A_wo: jax.Array,
    B_x: jax.Array,
    B_w1: jax.Array,
    B_b1: jax.Array,
    B_w2: jax.Array,
    B_b2: jax.Array,
):
    del B_x
    xt = jnp.transpose(A_x[0], (1, 0))
    any_spec = pl.BlockSpec(memory_space=pl.ANY)
    out_t = pl.pallas_call(
        _kernel,
        out_shape=jax.ShapeDtypeStruct((D, S), BF16),
        in_specs=[any_spec] * 7,
        out_specs=any_spec,
        scratch_shapes=[
            pltpu.VMEM((NT, D, LANES), BF16),
            pltpu.VMEM((S, F), BF16),
            pltpu.VMEM((F, S), BF16),
            pltpu.VMEM((D, 3 * D), BF16),
            pltpu.VMEM((D, D), BF16),
            pltpu.VMEM((F,), BF16),
            pltpu.VMEM((S,), BF16),
            pltpu.VMEM((NT, D, LANES), BF16),
            pltpu.VMEM((NT, D, LANES), BF16),
            pltpu.VMEM((NF, D, LANES), BF16),
            pltpu.VMEM((3 * D, D), BF16),
            pltpu.VMEM((D, D), BF16),
            pltpu.VMEM((4, 3 * D, LANES), F32),
            pltpu.VMEM((4, D, LANES), F32),
            pltpu.VMEM((NT + 5, 3 * D, LANES), F32),
            pltpu.VMEM((NT, 4 * H, LANES), F32),
            pltpu.VMEM((NT, WIN * H, LANES), F32),
            pltpu.VMEM((D, LANES), F32),
            pltpu.VMEM((NT, D, LANES), BF16),
            pltpu.VMEM((NT, D, LANES), BF16),
            pltpu.VMEM((2, H, LANES), F32),
            pltpu.SemaphoreType.DMA((NT,)),
            pltpu.SemaphoreType.DMA((N1,)),
            pltpu.SemaphoreType.DMA((5,)),
            pltpu.SemaphoreType.DMA((NT,)),
        ],
        compiler_params=pltpu.CompilerParams(vmem_limit_bytes=100 * 1024 * 1024),
    )(xt, A_wqkv, A_wo, B_w1, B_b1, B_w2, B_b2)
    return jnp.transpose(out_t, (1, 0))[None]
```

```python
import jax
import jax.numpy as jnp
import jax.experimental.pallas as pl
import jax.experimental.pallas.tpu as pltpu

S = 2048
D = 448
F = 1792
H = 16
DH = D // H
WIN = 8
DIL = 2
EPS = 1e-5
LANES = 128
NT = S // LANES
NF = F // LANES
F32 = jnp.float32
BF16 = jnp.bfloat16

P1_T = 2
P2_T = 4
P3_T = 2
S2_EARLY = 4
N1 = NT // P1_T


def _dot(a, b):
    return jnp.dot(a, b, preferred_element_type=F32)


def _gelu(x):
    c = 0.7978845608028654
    inner = x * (c + (c * 0.044715) * (x * x))
    hx = 0.5 * x
    return hx + hx * jnp.tanh(inner)


def _u_at(j):
    return (NT + j // 3, (j % 3) * D)


def _kernel(x_hbm, wqkv_hbm, wo_hbm, w1_hbm, b1_hbm, w2_hbm, b2_hbm, out_hbm,
            x_v, w1_v, w2_v, wqkv_v, wo_v, b1_v, b2_v,
            xn_s, h_s, g_s, wt_s, wot_s, t32, o32, qkv_s, l_s, p_s, o8_s, o_s, out_v, z_s,
            sem_x, sem_w1, sem_misc, sem_out):
    c1 = P1_T * LANES

    def x_copy(t):
        col = t * LANES if isinstance(t, int) else pl.multiple_of(t * LANES, LANES)
        return pltpu.make_async_copy(x_hbm.at[:, pl.ds(col, LANES)], x_v.at[t], sem_x.at[t])

    def w1_copy(i):
        row = i * c1 if isinstance(i, int) else pl.multiple_of(i * c1, c1)
        return pltpu.make_async_copy(w1_hbm.at[pl.ds(row, c1), :], w1_v.at[pl.ds(row, c1), :],
                                     sem_w1.at[i])

    c_b1 = pltpu.make_async_copy(b1_hbm, b1_v, sem_misc.at[0])
    c_b2 = pltpu.make_async_copy(b2_hbm, b2_v, sem_misc.at[1])
    c_wqkv = pltpu.make_async_copy(wqkv_hbm, wqkv_v, sem_misc.at[2])
    c_wo = pltpu.make_async_copy(wo_hbm, wo_v, sem_misc.at[3])
    c_w2 = pltpu.make_async_copy(w2_hbm, w2_v, sem_misc.at[4])

    def start_x(i):
        for j in range(P1_T):
            x_copy(i * P1_T + j).start()

    start_x(0)
    w1_copy(0).start()

    for j in range(NF):
        ti, r0 = _u_at(j)
        qkv_s[ti, pl.ds(r0, D), :] = jnp.zeros((D, LANES), F32)
    z_s[...] = jnp.zeros_like(z_s)
    o8_s[...] = jnp.zeros_like(o8_s)

    def make_tie(zi):
        never8 = z_s[zi] != 0.0
        never16 = jnp.concatenate([z_s[zi], z_s[zi]], axis=0) != 0.0

        def tie(val, src):
            return jnp.where(never8 if val.shape[0] == 8 else never16, src, val)
        return tie

    def make_hold(tie, res, ntile_par, n, lo=0.0, hi=1.0):
        nrows = res.shape[0] // 8
        total = nrows * (res.shape[1] // (LANES * ntile_par))
        state = [0]

        def hold(v):
            k = state[0]
            state[0] += 1
            assert k < n
            pos = min(int((lo + (hi - lo) * k / n) * total), total - 1)
            col, row = (pos // nrows) * ntile_par * LANES, (pos % nrows) * 8
            return tie(v, res[row:row + 8, col:col + LANES])
        return hold

    LG = 7

    def ln_pass(src, t, dst, hold):
        def ld(d):
            return src[t, pl.ds(d * H, H), :].astype(F32)

        def colmean(f, c):
            acc = None
            for g in range(DH // LG):
                cg = hold(c)
                cg = jnp.concatenate([cg, cg], axis=0)
                part = None
                for d in range(g * LG, (g + 1) * LG):
                    v = f(ld(d), cg, d == g * LG)
                    part = v if part is None else part + v
                acc = part if acc is None else acc + part
            m = jnp.sum(acc, axis=0, keepdims=True) * (1.0 / D)
            return jnp.broadcast_to(m, (8, LANES))

        def sq(v, m, first):
            c = v - m
            return c * c
        m = colmean(lambda v, c, first: v + c if first else v, jnp.zeros((8, LANES), F32))
        r = jax.lax.rsqrt(colmean(sq, m) + EPS)
        r = jnp.concatenate([r, r], axis=0)
        for g in range(DH // LG):
            mg = hold(m)
            mg = jnp.concatenate([mg, mg], axis=0)
            for d in range(g * LG, (g + 1) * LG):
                dst[t, pl.ds(d * H, H), :] = ((ld(d) - mg) * r).astype(BF16)

    def ln_tile(t, hold):
        ln_pass(x_v, t, xn_s, hold)
        ln_pass(xn_s, t, h_s, hold)

    def mixer1(i):
        row = i * c1 if isinstance(i, int) else pl.multiple_of(i * c1, c1)
        h = jnp.concatenate([h_s[i * P1_T + j] for j in range(P1_T)], axis=1)
        part = _dot(h, w1_v[pl.ds(row, c1), :])
        for j in range(NF):
            ti, r0 = _u_at(j)
            qkv_s[ti, pl.ds(r0, D), :] += part[:, j * LANES:(j + 1) * LANES]
        return part

    zeros16 = jnp.zeros((H, LANES), F32)

    with jax.named_scope("wait_x0"):
        for j in range(P1_T):
            x_copy(j).wait()
    start_x(1)
    w1_copy(1).start()
    start_x(2)
    with jax.named_scope("ln0"):
        for j in range(P1_T):
            ln_tile(j, lambda v: v)

    def p1_body(i, carry):
        with jax.named_scope("p1_wait"):
            w1_copy(i).wait()
            for j in range(P1_T):
                x_copy((i + 1) * P1_T + j).wait()

        @pl.when(i + 2 < N1)
        def _():
            w1_copy(i + 2).start()

        @pl.when(i + 3 < N1)
        def _():
            start_x(i + 3)

        @pl.when(i == 1)
        def _():
            c_wqkv.start(priority=1)
            c_wo.start(priority=1)
            c_b1.start(priority=1)
            c_b2.start(priority=1)

        tie = make_tie(jnp.minimum(i, 1))
        part = mixer1(i)
        hold = make_hold(tie, part, 2, P1_T * 6 * (DH // LG), 0.0, 0.9)
        for j in range(P1_T):
            ln_tile((i + 1) * P1_T + j, hold)
        return carry

    jax.lax.fori_loop(0, N1 - 1, p1_body, 0)

    with jax.named_scope("big_wait"):
        w1_copy(N1 - 1).wait()
        c_wqkv.wait()
        c_wo.wait()
        c_b1.wait()
        c_b2.wait()
    c_w2.start()
    tie = make_tie(0)
    part = mixer1(N1 - 1)

    k = 0
    for c in range(4):
        r = min(LANES, D - c * LANES)
        for j in range(11):
            n = min(LANES, 3 * D - j * LANES)
            blk = wqkv_v[pl.ds(c * LANES, r), pl.ds(j * LANES, n)].astype(F32)
            col = (k // 8) * LANES
            row = (k % 8) * 3 * H
            blk = jnp.concatenate([tie(blk[0:H], part[row:row + H, col:col + LANES][:, :n])
                                   if n == LANES else blk[0:H], blk[H:]], axis=0)
            t32[c, pl.ds(j * LANES, n), pl.ds(0, r)] = blk.T
            k += 1
    for p in range(3):
        for d in range(DH):
            for c in range(4):
                r = min(LANES, D - c * LANES)
                v = t32[c, pl.ds(p * D + d, H, stride=DH), :]
                wt_s[pl.ds(p * D + d * H, H), pl.ds(c * LANES, r)] = v[:, :r].astype(BF16)

    lane = jax.lax.broadcasted_iota(jnp.int32, (H, LANES), 1)
    scale = DH ** -0.5

    def shift_back(prev, cur, a):
        return pltpu.roll(jnp.where(lane >= LANES - a, prev, cur), a, 1)

    def shift_fwd(cur, nxt, b):
        return pltpu.roll(jnp.where(lane < b, nxt, cur), LANES - b, 1)

    def s1_tile(t):
        tn = min(t + 1, NT - 1)
        tp = max(t - 1, 0)
        acc = [None] * WIN
        for d in range(DH):
            rq = pl.ds(d * H, H)
            rk = pl.ds(D + d * H, H)
            q0 = qkv_s[t, rq, :]
            q8 = shift_fwd(q0, qkv_s[tn, rq, :], 8)
            k0 = qkv_s[t, rk, :]
            kp = qkv_s[tp, rk, :]
            ks = [k0] + [shift_back(kp, k0, a) for a in (2, 4, 6)]
            for a in range(4):
                t0 = q0 * ks[a]
                t8 = q8 * ks[a]
                acc[a] = t0 if d == 0 else acc[a] + t0
                acc[4 + a] = t8 if d == 0 else acc[4 + a] + t8
        for a in range(4):
            l_s[t, pl.ds(a * H, H), :] = acc[4 + a]
        lg = [acc[a] for a in range(4)]
        for a in range(4):
            lg.append(shift_back(l_s[tp, pl.ds(a * H, H), :], acc[4 + a], 8))
        lg = [v * scale for v in lg]
        if t == 0:
            lg = [lg[0]] + [jnp.where(lane >= DIL * j, lg[j], -1e9) for j in range(1, WIN)]
        m = lg[0]
        for j in range(1, WIN):
            m = jnp.maximum(m, lg[j])
        e = [jnp.exp(v - m) for v in lg]
        ssum = e[0]
        for j in range(1, WIN):
            ssum = ssum + e[j]
        inv = 1.0 / ssum
        for j in range(WIN):
            p_s[t, pl.ds(j * H, H), :] = e[j] * inv

    def s2_tile(t, src):
        tn = min(t + 1, NT - 1)
        tp = max(t - 1, 0)
        p0 = [p_s[t, pl.ds(a * H, H), :] for a in range(4)]
        p8 = [p_s[t, pl.ds((4 + a) * H, H), :] for a in range(4)]
        if src is not None:
            p0 = [tie(v, src) for v in p0]
            p8 = [tie(v, src) for v in p8]
        p8 = [shift_fwd(p8[a], p_s[tn, pl.ds((4 + a) * H, H), :], 8) for a in range(4)]
        for d in range(DH):
            rv = pl.ds(2 * D + d * H, H)
            r = pl.ds(d * H, H)
            v0 = qkv_s[t, rv, :]
            vp = qkv_s[tp, rv, :]
            vs = [v0] + [shift_back(vp, v0, a) for a in (2, 4, 6)]
            o0 = (p0[0] * vs[0] + p0[1] * vs[1]) + (p0[2] * vs[2] + p0[3] * vs[3])
            o8 = (p8[0] * vs[0] + p8[1] * vs[1]) + (p8[2] * vs[2] + p8[3] * vs[3])
            o = o0 + shift_back(o8_s[r, :], o8, 8)
            o8_s[r, :] = o8
            o_s[t, r, :] = o.astype(BF16)

    def proj(rows0, nrows, blk):
        xn = jnp.concatenate([xn_s[blk * P2_T + j] for j in range(P2_T)], axis=1)
        res = _dot(wt_s[pl.ds(rows0, nrows), :], xn)
        for j in range(P2_T):
            qkv_s[blk * P2_T + j, pl.ds(rows0, nrows), :] = res[:, j * LANES:(j + 1) * LANES]
        return res

    b1 = b1_v[...].astype(F32).reshape(1, F)
    GR = 64
    gelu_jobs = [(j, rr) for j in range(NF) for rr in range(D // GR)]

    def gelu_job(j, rr, src):
        ti, r0 = _u_at(j)
        bias = tie(jnp.broadcast_to(b1[:, j * LANES:(j + 1) * LANES], (H, LANES)), src)
        for q in range(GR // H):
            row = rr * GR + q * H
            g_s[j, pl.ds(row, H), :] = _gelu(qkv_s[ti, pl.ds(r0 + row, H), :] + bias).astype(BF16)

    def spread_gelu(res, njobs):
        nrows, ncols = res.shape
        nslab = (nrows // H) * (ncols // LANES)
        for k in range(njobs):
            if not gelu_jobs:
                return
            pos = (k * nslab) // njobs
            col, row = (pos // (nrows // H)) * LANES, (pos % (nrows // H)) * H
            gelu_job(*gelu_jobs.pop(0), res[row:row + H, col:col + LANES])

    def wo_prep(res):
        for c in range(4):
            r = min(LANES, D - c * LANES)
            blk = wo_v[:, pl.ds(c * LANES, r)].astype(F32)
            o32[c, :, pl.ds(0, r)] = blk
        for c in range(4):
            r = min(LANES, D - c * LANES)
            rows = jnp.concatenate(
                [o32[c, pl.ds(d, H, stride=DH), pl.ds(0, r)] for d in range(DH)], axis=0)
            wot_s[pl.ds(c * LANES, r), :] = rows.T.astype(BF16)

    n2 = NT // P2_T
    done_t = 0
    for blk in range(n2):
        res = proj(0, 2 * D, blk)
        spread_gelu(res, 14 if blk == 0 else 8)
        lim = (blk + 1) * P2_T - 1 if blk + 1 < n2 else NT
        while done_t < lim:
            s1_tile(done_t)
            done_t += 1
    done2 = 0
    for blk in range(n2):
        res = proj(2 * D, D, blk)
        spread_gelu(res, 15)
        if blk == 1:
            wo_prep(res)
        while done2 < min(S2_EARLY, (blk + 1) * P2_T):
            s2_tile(done2, None)
            done2 += 1
    assert done_t == NT and not gelu_jobs

    with jax.named_scope("w2_wait"):
        c_w2.wait()
    n3 = NT // P3_T
    c3 = P3_T * LANES

    def out_copy(t):
        return pltpu.make_async_copy(out_v.at[t], out_hbm.at[:, pl.ds(t * LANES, LANES)],
                                     sem_out.at[t])

    b2 = b2_v[...].astype(F32).reshape(1, S)
    for i in range(n3):
        g = jnp.concatenate([g_s[j] for j in range(NF)], axis=1)
        y = _dot(g, w2_v[:, pl.ds(i * c3, c3)])
        for j in range(P3_T):
            if done2 < NT:
                s2_tile(done2, y[0:H, j * LANES:(j + 1) * LANES])
                done2 += 1
        o = jnp.concatenate([o_s[i * P3_T + j] for j in range(P3_T)], axis=1)
        y = _dot(wot_s[...], o) + y
        for j in range(P3_T):
            t = i * P3_T + j
            bias = jnp.broadcast_to(b2[:, t * LANES:(t + 1) * LANES], (H, LANES))
            for d in range(DH):
                r = pl.ds(d * H, H)
                val = x_v[t, r, :].astype(F32) + (y[d * H:(d + 1) * H, j * LANES:(j + 1) * LANES] + bias)
                out_v[t, r, :] = val.astype(BF16)
            out_copy(t).start()

    with jax.named_scope("out_wait"):
        for t in range(NT):
            out_copy(t).wait()


@jax.jit
def pallas_parallel_sum__sliding_local_dilated__mixer_token_mlp__prompt_kernel(
    A_x: jax.Array,
    A_wqkv: jax.Array,
    A_wo: jax.Array,
    B_x: jax.Array,
    B_w1: jax.Array,
    B_b1: jax.Array,
    B_w2: jax.Array,
    B_b2: jax.Array,
):
    del B_x
    xt = jnp.transpose(A_x[0], (1, 0))
    any_spec = pl.BlockSpec(memory_space=pl.ANY)
    out_t = pl.pallas_call(
        _kernel,
        out_shape=jax.ShapeDtypeStruct((D, S), BF16),
        in_specs=[any_spec] * 7,
        out_specs=any_spec,
        scratch_shapes=[
            pltpu.VMEM((NT, D, LANES), BF16),
            pltpu.VMEM((S, F), BF16),
            pltpu.VMEM((F, S), BF16),
            pltpu.VMEM((D, 3 * D), BF16),
            pltpu.VMEM((D, D), BF16),
            pltpu.VMEM((F,), BF16),
            pltpu.VMEM((S,), BF16),
            pltpu.VMEM((NT, D, LANES), BF16),
            pltpu.VMEM((NT, D, LANES), BF16),
            pltpu.VMEM((NF, D, LANES), BF16),
            pltpu.VMEM((3 * D, D), BF16),
            pltpu.VMEM((D, D), BF16),
            pltpu.VMEM((4, 3 * D, LANES), F32),
            pltpu.VMEM((4, D, LANES), F32),
            pltpu.VMEM((NT + 5, 3 * D, LANES), F32),
            pltpu.VMEM((NT, 4 * H, LANES), F32),
            pltpu.VMEM((NT, WIN * H, LANES), F32),
            pltpu.VMEM((D, LANES), F32),
            pltpu.VMEM((NT, D, LANES), BF16),
            pltpu.VMEM((NT, D, LANES), BF16),
            pltpu.VMEM((2, 8, LANES), F32),
            pltpu.SemaphoreType.DMA((NT,)),
            pltpu.SemaphoreType.DMA((N1,)),
            pltpu.SemaphoreType.DMA((5,)),
            pltpu.SemaphoreType.DMA((NT,)),
        ],
        compiler_params=pltpu.CompilerParams(vmem_limit_bytes=100 * 1024 * 1024),
    )(xt, A_wqkv, A_wo, B_w1, B_b1, B_w2, B_b2)
    return jnp.transpose(out_t, (1, 0))[None]
```

```python
import jax
import jax.numpy as jnp
import jax.experimental.pallas as pl
import jax.experimental.pallas.tpu as pltpu

S = 2048
D = 448
F = 1792
H = 16
DH = D // H
WIN = 8
DIL = 2
EPS = 1e-5
LANES = 128
NT = S // LANES
NF = F // LANES
F32 = jnp.float32
BF16 = jnp.bfloat16

P1_T = 2
P2_T = 4
P3_T = 2
S2_EARLY = 4
N1 = NT // P1_T


def _dot(a, b):
    return jnp.dot(a, b, preferred_element_type=F32)


def _gelu(x):
    c = 0.7978845608028654
    inner = x * (c + (c * 0.044715) * (x * x))
    hx = 0.5 * x
    return hx + hx * jnp.tanh(inner)


def _u_at(j):
    return (NT + j // 3, (j % 3) * D)


def _kernel(x_hbm, wqkv_hbm, wo_hbm, w1_hbm, b1_hbm, w2_hbm, b2_hbm, out_hbm,
            x_v, w1_v, w2_v, wqkv_v, wo_v, b1_v, b2_v,
            xn_s, h_s, g_s, wt_s, wot_s, t32, o32, qkv_s, l_s, p_s, o8_s, o_s, out_v, z_s,
            sems):
    c1 = P1_T * LANES
    SEM_LAST, SEM_W2, SEM_OUT = N1 + 1, N1 + 2, N1 + 3

    def x_copy(t, sem):
        col = t * LANES if isinstance(t, int) else pl.multiple_of(t * LANES, LANES)
        return pltpu.make_async_copy(x_hbm.at[:, pl.ds(col, LANES)], x_v.at[t], sems.at[sem])

    def w1_copy(row, nrows, sem):
        return pltpu.make_async_copy(w1_hbm.at[pl.ds(row, nrows), :], w1_v.at[pl.ds(row, nrows), :],
                                     sems.at[sem])

    def step_copies(i):
        row = i * c1 if isinstance(i, int) else pl.multiple_of(i * c1, c1)
        return [w1_copy(row, c1, 2 + i)] + [x_copy((i + 1) * P1_T + j, 2 + i) for j in range(P1_T)]

    copies_0 = [x_copy(0, 0)]
    copies_a = [w1_copy(0, LANES, 1), x_copy(1, 1)]
    copies_b = [w1_copy(LANES, LANES, 2), x_copy(2, 2), x_copy(3, 2)]
    c_w1_last = w1_copy((N1 - 1) * c1, c1, SEM_LAST)
    small = [pltpu.make_async_copy(src, dst, sems.at[SEM_LAST])
             for src, dst in ((wqkv_hbm, wqkv_v), (wo_hbm, wo_v), (b1_hbm, b1_v), (b2_hbm, b2_v))]
    c_w2 = pltpu.make_async_copy(w2_hbm, w2_v, sems.at[SEM_W2])

    for c in copies_0 + copies_a:
        c.start()

    z_s[...] = jnp.zeros_like(z_s)
    o8_s[...] = jnp.zeros_like(o8_s)

    def make_tie(zi):
        never8 = z_s[zi] != 0.0
        never16 = jnp.concatenate([z_s[zi], z_s[zi]], axis=0) != 0.0

        def tie(val, src):
            return jnp.where(never8 if val.shape[0] == 8 else never16, src, val)
        return tie

    def make_hold(tie, res, ntile_par, n, lo=0.0, hi=1.0):
        nrows = res.shape[0] // 8
        total = nrows * (-(-res.shape[1] // (LANES * ntile_par)))
        state = [0]

        def hold(v):
            k = state[0]
            state[0] += 1
            assert k < n
            pos = min(int((lo + (hi - lo) * k / n) * total), total - 1)
            col, row = (pos // nrows) * ntile_par * LANES, (pos % nrows) * 8
            return tie(v, res[row:row + 8, col:col + LANES])
        return hold

    LG = 7

    def ln_pass(src, t, dst, hold):
        def ld(d):
            return src[t, pl.ds(d * H, H), :].astype(F32)

        def colmean(f, c):
            acc = None
            for g in range(DH // LG):
                cg = hold(c)
                cg = jnp.concatenate([cg, cg], axis=0)
                part = None
                for d in range(g * LG, (g + 1) * LG):
                    v = f(ld(d), cg, d == g * LG)
                    part = v if part is None else part + v
                acc = part if acc is None else acc + part
            m = jnp.sum(acc, axis=0, keepdims=True) * (1.0 / D)
            return jnp.broadcast_to(m, (8, LANES))

        def sq(v, m, first):
            c = v - m
            return c * c
        m = colmean(lambda v, c, first: v + c if first else v, jnp.zeros((8, LANES), F32))
        r = jax.lax.rsqrt(colmean(sq, m) + EPS)
        r = jnp.concatenate([r, r], axis=0)
        for g in range(DH // LG):
            mg = hold(m)
            mg = jnp.concatenate([mg, mg], axis=0)
            for d in range(g * LG, (g + 1) * LG):
                dst[t, pl.ds(d * H, H), :] = ((ld(d) - mg) * r).astype(BF16)

    def ln_tile(t, hold):
        ln_pass(x_v, t, xn_s, hold)
        ln_pass(xn_s, t, h_s, hold)

    def mixer1(t0, nt, first=False):
        row = t0 * LANES if isinstance(t0, int) else pl.multiple_of(t0 * LANES, LANES)
        h = jnp.concatenate([h_s[t0 + j] for j in range(nt)], axis=1)
        part = _dot(h, w1_v[pl.ds(row, nt * LANES), :])
        for j in range(NF):
            ti, r0 = _u_at(j)
            if first:
                qkv_s[ti, pl.ds(r0, D), :] = part[:, j * LANES:(j + 1) * LANES]
            else:
                qkv_s[ti, pl.ds(r0, D), :] += part[:, j * LANES:(j + 1) * LANES]
        return part

    NH = 6 * (DH // LG)

    with jax.named_scope("wait_x0"):
        for c in copies_0:
            c.wait()
    for c in copies_b + step_copies(1):
        c.start()
    with jax.named_scope("ln0"):
        ln_tile(0, lambda v: v)

    with jax.named_scope("wait_a"):
        for c in copies_a:
            c.wait()
    for i in range(2, N1 - 1):
        for c in step_copies(i):
            c.start()
    c_w1_last.start()
    for c in small + [c_w2]:
        c.start(priority=1)
    tie = make_tie(0)
    part = mixer1(0, 1, first=True)
    ln_tile(1, make_hold(tie, part, 4, NH, 0.0, 0.8))

    with jax.named_scope("wait_b"):
        for c in copies_b:
            c.wait()
    tie = make_tie(0)
    part = mixer1(1, 1)
    hold = make_hold(tie, part, 4, 2 * NH, 0.0, 0.85)
    ln_tile(2, hold)
    ln_tile(3, hold)

    def p1_body(i, carry):
        with jax.named_scope("p1_wait"):
            for c in step_copies(i):
                c.wait()
        tie = make_tie(jnp.minimum(i, 1))
        part = mixer1(i * P1_T, P1_T)
        hold = make_hold(tie, part, 2, P1_T * NH, 0.0, 0.9)
        for j in range(P1_T):
            ln_tile((i + 1) * P1_T + j, hold)
        return carry

    jax.lax.fori_loop(1, N1 - 1, p1_body, 0)

    with jax.named_scope("big_wait"):
        for c in [c_w1_last] + small:
            c.wait()
    tie = make_tie(0)
    part = mixer1((N1 - 1) * P1_T, P1_T)

    k = 0
    for c in range(4):
        r = min(LANES, D - c * LANES)
        for j in range(11):
            n = min(LANES, 3 * D - j * LANES)
            blk = wqkv_v[pl.ds(c * LANES, r), pl.ds(j * LANES, n)].astype(F32)
            col = (k // 8) * LANES
            row = (k % 8) * 3 * H
            blk = jnp.concatenate([tie(blk[0:H], part[row:row + H, col:col + LANES][:, :n])
                                   if n == LANES else blk[0:H], blk[H:]], axis=0)
            t32[c, pl.ds(j * LANES, n), pl.ds(0, r)] = blk.T
            k += 1
    for p in range(3):
        for d in range(DH):
            for c in range(4):
                r = min(LANES, D - c * LANES)
                v = t32[c, pl.ds(p * D + d, H, stride=DH), :]
                wt_s[pl.ds(p * D + d * H, H), pl.ds(c * LANES, r)] = v[:, :r].astype(BF16)

    lane = jax.lax.broadcasted_iota(jnp.int32, (H, LANES), 1)
    scale = DH ** -0.5

    def shift_back(prev, cur, a):
        return pltpu.roll(jnp.where(lane >= LANES - a, prev, cur), a, 1)

    def shift_fwd(cur, nxt, b):
        return pltpu.roll(jnp.where(lane < b, nxt, cur), LANES - b, 1)

    def s1_tile(t):
        tn = min(t + 1, NT - 1)
        tp = max(t - 1, 0)
        acc = [None] * WIN
        for d in range(DH):
            rq = pl.ds(d * H, H)
            rk = pl.ds(D + d * H, H)
            q0 = qkv_s[t, rq, :]
            q8 = shift_fwd(q0, qkv_s[tn, rq, :], 8)
            k0 = qkv_s[t, rk, :]
            kp = qkv_s[tp, rk, :]
            ks = [k0] + [shift_back(kp, k0, a) for a in (2, 4, 6)]
            for a in range(4):
                t0 = q0 * ks[a]
                t8 = q8 * ks[a]
                acc[a] = t0 if d == 0 else acc[a] + t0
                acc[4 + a] = t8 if d == 0 else acc[4 + a] + t8
        for a in range(4):
            l_s[t, pl.ds(a * H, H), :] = acc[4 + a]
        lg = [acc[a] for a in range(4)]
        for a in range(4):
            lg.append(shift_back(l_s[tp, pl.ds(a * H, H), :], acc[4 + a], 8))
        lg = [v * scale for v in lg]
        if t == 0:
            lg = [lg[0]] + [jnp.where(lane >= DIL * j, lg[j], -1e9) for j in range(1, WIN)]
        m = lg[0]
        for j in range(1, WIN):
            m = jnp.maximum(m, lg[j])
        e = [jnp.exp(v - m) for v in lg]
        ssum = e[0]
        for j in range(1, WIN):
            ssum = ssum + e[j]
        inv = 1.0 / ssum
        for j in range(WIN):
            p_s[t, pl.ds(j * H, H), :] = e[j] * inv

    def s2_tile(t, src):
        tn = min(t + 1, NT - 1)
        tp = max(t - 1, 0)
        p0 = [p_s[t, pl.ds(a * H, H), :] for a in range(4)]
        p8 = [p_s[t, pl.ds((4 + a) * H, H), :] for a in range(4)]
        if src is not None:
            p0 = [tie(v, src) for v in p0]
            p8 = [tie(v, src) for v in p8]
        p8 = [shift_fwd(p8[a], p_s[tn, pl.ds((4 + a) * H, H), :], 8) for a in range(4)]
        for d in range(DH):
            rv = pl.ds(2 * D + d * H, H)
            r = pl.ds(d * H, H)
            v0 = qkv_s[t, rv, :]
            vp = qkv_s[tp, rv, :]
            vs = [v0] + [shift_back(vp, v0, a) for a in (2, 4, 6)]
            o0 = (p0[0] * vs[0] + p0[1] * vs[1]) + (p0[2] * vs[2] + p0[3] * vs[3])
            o8 = (p8[0] * vs[0] + p8[1] * vs[1]) + (p8[2] * vs[2] + p8[3] * vs[3])
            o = o0 + shift_back(o8_s[r, :], o8, 8)
            o8_s[r, :] = o8
            o_s[t, r, :] = o.astype(BF16)

    def proj(rows0, nrows, blk):
        xn = jnp.concatenate([xn_s[blk * P2_T + j] for j in range(P2_T)], axis=1)
        res = _dot(wt_s[pl.ds(rows0, nrows), :], xn)
        for j in range(P2_T):
            qkv_s[blk * P2_T + j, pl.ds(rows0, nrows), :] = res[:, j * LANES:(j + 1) * LANES]
        return res

    b1 = b1_v[...].astype(F32).reshape(1, F)
    GR = 64
    gelu_jobs = [(j, rr) for j in range(NF) for rr in range(D // GR)]

    def gelu_job(j, rr, src):
        ti, r0 = _u_at(j)
        bias = tie(jnp.broadcast_to(b1[:, j * LANES:(j + 1) * LANES], (H, LANES)), src)
        for q in range(GR // H):
            row = rr * GR + q * H
            g_s[j, pl.ds(row, H), :] = _gelu(qkv_s[ti, pl.ds(r0 + row, H), :] + bias).astype(BF16)

    def spread_gelu(res, njobs):
        nrows, ncols = res.shape
        nslab = (nrows // H) * (ncols // LANES)
        for k in range(njobs):
            if not gelu_jobs:
                return
            pos = (k * nslab) // njobs
            col, row = (pos // (nrows // H)) * LANES, (pos % (nrows // H)) * H
            gelu_job(*gelu_jobs.pop(0), res[row:row + H, col:col + LANES])

    def wo_prep(res):
        for c in range(4):
            r = min(LANES, D - c * LANES)
            blk = wo_v[:, pl.ds(c * LANES, r)].astype(F32)
            o32[c, :, pl.ds(0, r)] = blk
        for c in range(4):
            r = min(LANES, D - c * LANES)
            rows = jnp.concatenate(
                [o32[c, pl.ds(d, H, stride=DH), pl.ds(0, r)] for d in range(DH)], axis=0)
            wot_s[pl.ds(c * LANES, r), :] = rows.T.astype(BF16)

    n2 = NT // P2_T
    done_t = 0
    for blk in range(n2):
        res = proj(0, 2 * D, blk)
        spread_gelu(res, 14 if blk == 0 else 8)
        lim = (blk + 1) * P2_T - 1 if blk + 1 < n2 else NT
        while done_t < lim:
            s1_tile(done_t)
            done_t += 1
    done2 = 0
    for blk in range(n2):
        res = proj(2 * D, D, blk)
        spread_gelu(res, 15)
        if blk == 1:
            wo_prep(res)
        while done2 < min(S2_EARLY, (blk + 1) * P2_T):
            s2_tile(done2, None)
            done2 += 1
    assert done_t == NT and not gelu_jobs

    with jax.named_scope("w2_wait"):
        c_w2.wait()
    n3 = NT // P3_T
    c3 = P3_T * LANES

    def out_copy(t):
        return pltpu.make_async_copy(out_v.at[t], out_hbm.at[:, pl.ds(t * LANES, LANES)],
                                     sems.at[SEM_OUT])

    b2 = b2_v[...].astype(F32).reshape(1, S)
    for i in range(n3):
        g = jnp.concatenate([g_s[j] for j in range(NF)], axis=1)
        y = _dot(g, w2_v[:, pl.ds(i * c3, c3)])
        for j in range(P3_T):
            if done2 < NT:
                s2_tile(done2, y[0:H, j * LANES:(j + 1) * LANES])
                done2 += 1
        o = jnp.concatenate([o_s[i * P3_T + j] for j in range(P3_T)], axis=1)
        y = _dot(wot_s[...], o) + y
        for j in range(P3_T):
            t = i * P3_T + j
            bias = jnp.broadcast_to(b2[:, t * LANES:(t + 1) * LANES], (H, LANES))
            for d in range(DH):
                r = pl.ds(d * H, H)
                val = x_v[t, r, :].astype(F32) + (y[d * H:(d + 1) * H, j * LANES:(j + 1) * LANES] + bias)
                out_v[t, r, :] = val.astype(BF16)
            out_copy(t).start()

    with jax.named_scope("out_wait"):
        for t in range(NT):
            out_copy(t).wait()


@jax.jit
def pallas_parallel_sum__sliding_local_dilated__mixer_token_mlp__prompt_kernel(
    A_x: jax.Array,
    A_wqkv: jax.Array,
    A_wo: jax.Array,
    B_x: jax.Array,
    B_w1: jax.Array,
    B_b1: jax.Array,
    B_w2: jax.Array,
    B_b2: jax.Array,
):
    del B_x
    xt = jnp.transpose(A_x[0], (1, 0))
    any_spec = pl.BlockSpec(memory_space=pl.ANY)
    out_t = pl.pallas_call(
        _kernel,
        out_shape=jax.ShapeDtypeStruct((D, S), BF16),
        in_specs=[any_spec] * 7,
        out_specs=any_spec,
        scratch_shapes=[
            pltpu.VMEM((NT, D, LANES), BF16),
            pltpu.VMEM((S, F), BF16),
            pltpu.VMEM((F, S), BF16),
            pltpu.VMEM((D, 3 * D), BF16),
            pltpu.VMEM((D, D), BF16),
            pltpu.VMEM((F,), BF16),
            pltpu.VMEM((S,), BF16),
            pltpu.VMEM((NT, D, LANES), BF16),
            pltpu.VMEM((NT, D, LANES), BF16),
            pltpu.VMEM((NF, D, LANES), BF16),
            pltpu.VMEM((3 * D, D), BF16),
            pltpu.VMEM((D, D), BF16),
            pltpu.VMEM((4, 3 * D, LANES), F32),
            pltpu.VMEM((4, D, LANES), F32),
            pltpu.VMEM((NT + 5, 3 * D, LANES), F32),
            pltpu.VMEM((NT, 4 * H, LANES), F32),
            pltpu.VMEM((NT, WIN * H, LANES), F32),
            pltpu.VMEM((D, LANES), F32),
            pltpu.VMEM((NT, D, LANES), BF16),
            pltpu.VMEM((NT, D, LANES), BF16),
            pltpu.VMEM((2, 8, LANES), F32),
            pltpu.SemaphoreType.DMA((N1 + 4,)),
        ],
        compiler_params=pltpu.CompilerParams(vmem_limit_bytes=100 * 1024 * 1024,
                                             disable_bounds_checks=True,
                                             disable_semaphore_checks=True),
    )(xt, A_wqkv, A_wo, B_w1, B_b1, B_w2, B_b2)
    return jnp.transpose(out_t, (1, 0))[None]
```

```python
import jax
import jax.numpy as jnp
import jax.experimental.pallas as pl
import jax.experimental.pallas.tpu as pltpu

S = 2048
D = 448
F = 1792
H = 16
DH = D // H
WIN = 8
DIL = 2
EPS = 1e-5
LANES = 128
NT = S // LANES
NF = F // LANES
F32 = jnp.float32
BF16 = jnp.bfloat16
U32 = jnp.uint32

P1_T = 2
P2_T = 4
P3_T = 2
N1 = NT // P1_T
NA = 6


def _dot(a, b):
    return jnp.dot(a, b, preferred_element_type=F32)


def _gelu(x):
    c = 0.7978845608028654
    inner = x * (c + (c * 0.044715) * (x * x))
    hx = 0.5 * x
    return hx + hx * jnp.tanh(inner)


def _pack(v):
    return pltpu.bitcast(v.astype(BF16), U32)


def _unpack(v):
    return pltpu.bitcast(v, BF16)


def _kernel(x_hbm, wqkv_hbm, wo_hbm, w1_hbm, b1_hbm, w2_hbm, b2_hbm, out_hbm,
            x_v, w1_v, w2_v, wqkv_v, wo_v, b1_v, b2_v,
            xn_s, h_s, u_s, g_s, wt_s, wot_s, t32, o32, qk_s, v_s, l_s, p_s, o8_s, o_s, out_v, z_s,
            sems):
    c1 = P1_T * LANES
    SEM_LAST, SEM_W2, SEM_OUT = N1 + 1, N1 + 2, N1 + 3

    def x_copy(t, sem):
        col = t * LANES if isinstance(t, int) else pl.multiple_of(t * LANES, LANES)
        return pltpu.make_async_copy(x_hbm.at[:, pl.ds(col, LANES)], x_v.at[t], sems.at[sem])

    def w1_copy(row, sem, col=0, ncol=F):
        return pltpu.make_async_copy(w1_hbm.at[pl.ds(row, c1), pl.ds(col, ncol)],
                                     w1_v.at[pl.ds(row, c1), pl.ds(col, ncol)], sems.at[sem])

    def step_copies(i):
        row = i * c1 if isinstance(i, int) else pl.multiple_of(i * c1, c1)
        return [w1_copy(row, 2 + i)] + [x_copy((i + 1) * P1_T + j, 2 + i) for j in range(P1_T)]

    copies_0 = [x_copy(0, 0), x_copy(1, 0)]
    copies_a = [w1_copy(0, 1, 0, NA * LANES)]
    copies_b = [w1_copy(0, 2, NA * LANES, F - NA * LANES), x_copy(2, 2), x_copy(3, 2)]
    c_w1_last = w1_copy((N1 - 1) * c1, SEM_LAST)
    small = [pltpu.make_async_copy(src, dst, sems.at[SEM_LAST])
             for src, dst in ((wqkv_hbm, wqkv_v), (wo_hbm, wo_v), (b1_hbm, b1_v), (b2_hbm, b2_v))]
    c_w2 = pltpu.make_async_copy(w2_hbm, w2_v, sems.at[SEM_W2])

    for c in copies_0 + copies_a + copies_b:
        c.start()
    for i in range(1, N1 - 1):
        for c in step_copies(i):
            c.start()
    c_w1_last.start()
    for c in small + [c_w2]:
        c.start(priority=1)

    z_s[...] = jnp.zeros_like(z_s)
    o8_s[...] = jnp.zeros_like(o8_s)

    def make_tie(zi):
        never8 = z_s[zi] != 0.0
        never16 = jnp.concatenate([z_s[zi], z_s[zi]], axis=0) != 0.0

        def tie(val, src):
            if val.dtype != src.dtype:
                src = pltpu.bitcast(src, val.dtype)
            if val.shape[0] == 16 and src.shape[0] == 8:
                src = jnp.concatenate([src, src], axis=0)
            return jnp.where(never8 if val.shape[0] == 8 else never16, src, val)
        return tie

    def make_hold(tie, results, ntile_par, n, lo=0.0, hi=1.0):
        pts = []
        for res in results:
            for c in range(0, res.shape[1] // LANES, ntile_par):
                pts += [(res, r, c * LANES) for r in range(0, res.shape[0], 8)]
        state = [0]

        def hold(v):
            k = state[0]
            state[0] += 1
            assert k < n
            res, row, col = pts[min(int((lo + (hi - lo) * k / n) * len(pts)), len(pts) - 1)]
            return tie(v, res[row:row + 8, col:col + LANES])
        return hold

    LG = 7
    NH = 6 * (DH // LG)

    def ln_pass(ld, dst, t, hold):
        def colmean(f, c):
            acc = None
            for g in range(DH // LG):
                cg = hold(c)
                cg = jnp.concatenate([cg, cg], axis=0)
                part = None
                for d in range(g * LG, (g + 1) * LG):
                    v = f(ld(d), cg, d == g * LG)
                    part = v if part is None else part + v
                acc = part if acc is None else acc + part
            m = jnp.sum(acc, axis=0, keepdims=True) * (1.0 / D)
            return jnp.broadcast_to(m, (8, LANES))

        def sq(v, m, first):
            c = v - m
            return c * c
        m = colmean(lambda v, c, first: v + c if first else v, jnp.zeros((8, LANES), F32))
        r = jax.lax.rsqrt(colmean(sq, m) + EPS)
        r = jnp.concatenate([r, r], axis=0)
        for g in range(DH // LG):
            mg = hold(m)
            mg = jnp.concatenate([mg, mg], axis=0)
            for d in range(g * LG, (g + 1) * LG):
                dst[t, pl.ds(d * 8, 8), :] = _pack((ld(d) - mg) * r)

    def ln_tile(t, hold):
        ln_pass(lambda d: x_v[t, pl.ds(d * H, H), :].astype(F32), xn_s, t, hold)
        ln_pass(lambda d: _unpack(xn_s[t, pl.ds(d * 8, 8), :]).astype(F32), h_s, t, hold)

    def tiles(ref, t0, nt):
        return _unpack(jnp.concatenate([ref[t0 + j] for j in range(nt)], axis=1))

    def mixer1(i, j0=0, j1=NF, first=False):
        row = i * c1 if isinstance(i, int) else pl.multiple_of(i * c1, c1)
        part = _dot(tiles(h_s, i * P1_T, P1_T), w1_v[pl.ds(row, c1), pl.ds(j0 * LANES, (j1 - j0) * LANES)])
        for j in range(j0, j1):
            pj = part[:, (j - j0) * LANES:(j - j0 + 1) * LANES]
            if first:
                u_s[j] = pj
            else:
                u_s[j] += pj
        return part

    with jax.named_scope("wait_x0"):
        for c in copies_0:
            c.wait()
    with jax.named_scope("ln0"):
        ln_tile(0, lambda v: v)
        ln_tile(1, lambda v: v)

    with jax.named_scope("wait_a"):
        for c in copies_a:
            c.wait()
    mixer1(0, 0, NA, first=True)

    with jax.named_scope("wait_b"):
        for c in copies_b:
            c.wait()
    tie = make_tie(0)
    part = mixer1(0, NA, NF, first=True)
    hold = make_hold(tie, [part], 2, 2 * NH, 0.0, 0.85)
    ln_tile(2, hold)
    ln_tile(3, hold)

    def p1_body(i, carry):
        with jax.named_scope("p1_wait"):
            for c in step_copies(i):
                c.wait()
        tie = make_tie(jnp.minimum(i, 1))
        part = mixer1(i)
        hold = make_hold(tie, [part], 2, P1_T * NH, 0.0, 0.9)
        for j in range(P1_T):
            ln_tile((i + 1) * P1_T + j, hold)
        return carry

    jax.lax.fori_loop(1, N1 - 1, p1_body, 0)

    with jax.named_scope("big_wait"):
        for c in [c_w1_last] + small:
            c.wait()
    tie = make_tie(0)
    part = mixer1(N1 - 1)

    def wt_transpose(j, hold):
        n = min(LANES, 3 * D - j * LANES)
        for c in range(4):
            r = min(LANES, D - c * LANES)
            blk = wqkv_v[pl.ds(c * LANES, r), pl.ds(j * LANES, n)]
            if n == LANES:
                blk = jnp.concatenate([_unpack(hold(_pack(blk[0:H]))), blk[H:]], axis=0)
            t32[c, pl.ds(j * LANES, n), pl.ds(0, r)] = blk.astype(F32).T

    def wt_gather(p):
        for d in range(DH):
            dst = (2 * d + p) * 8 if p < 2 else (2 * DH + d) * 8
            for c in range(4):
                r = min(LANES, D - c * LANES)
                v = t32[c, pl.ds(p * D + d, H, stride=DH), pl.ds(0, r)]
                wt_s[pl.ds(dst, 8), pl.ds(c * LANES, r)] = _pack(v)

    hold = make_hold(tie, [part], 2, 28, 0.0, 0.6)
    for j in range(7):
        wt_transpose(j, hold)
    wt_gather(0)
    wt_gather(1)

    def wo_prep(hold):
        for c in range(4):
            r = min(LANES, D - c * LANES)
            for g in range(4):
                blk = wo_v[pl.ds(g * 112, 112), pl.ds(c * LANES, r)].astype(F32)
                if r == LANES:
                    blk = jnp.concatenate([hold(blk[q * 8:q * 8 + 8]) for q in range(14)], axis=0)
                o32[c, pl.ds(g * 112, 112), pl.ds(0, r)] = blk
        for c in range(4):
            r = min(LANES, D - c * LANES)
            rows = jnp.concatenate(
                [o32[c, pl.ds(d, H, stride=DH), pl.ds(0, r)] for d in range(DH)], axis=0)
            wot_s[pl.ds(c * 64, r // 2), :] = _pack(rows.T)

    lane = jax.lax.broadcasted_iota(jnp.int32, (H, LANES), 1)
    scale = DH ** -0.5

    def shift_back(prev, cur, a):
        return pltpu.roll(jnp.where(lane >= LANES - a, prev, cur), a, 1)

    def shift_fwd(cur, nxt, b):
        return pltpu.roll(jnp.where(lane < b, nxt, cur), LANES - b, 1)

    def s1_tile(t, hold=None):
        tn = min(t + 1, NT - 1)
        tp = max(t - 1, 0)
        acc = [None] * WIN
        for d in range(DH):
            rq = pl.ds(2 * d * H, H)
            rk = pl.ds((2 * d + 1) * H, H)
            q0 = qk_s[t, rq, :]
            qn = qk_s[tn, rq, :]
            k0 = qk_s[t, rk, :]
            if hold is None:
                k0 = tie(k0, qn)
            else:
                k0 = hold(k0)
                qn = tie(qn, k0)
            q8 = shift_fwd(q0, qn, 8)
            kp = qk_s[tp, rk, :]
            ks = [k0] + [shift_back(kp, k0, a) for a in (2, 4, 6)]
            for a in range(4):
                t0 = q0 * ks[a]
                t8 = q8 * ks[a]
                acc[a] = t0 if d == 0 else acc[a] + t0
                acc[4 + a] = t8 if d == 0 else acc[4 + a] + t8
        for a in range(4):
            l_s[t, pl.ds(a * H, H), :] = acc[4 + a]
        lg = [acc[a] for a in range(4)]
        for a in range(4):
            lg.append(shift_back(l_s[tp, pl.ds(a * H, H), :], acc[4 + a], 8))
        lg = [v * scale for v in lg]
        if t == 0:
            lg = [lg[0]] + [jnp.where(lane >= DIL * j, lg[j], -1e9) for j in range(1, WIN)]
        m = lg[0]
        for j in range(1, WIN):
            m = jnp.maximum(m, lg[j])
        e = [jnp.exp(v - m) for v in lg]
        ssum = e[0]
        for j in range(1, WIN):
            ssum = ssum + e[j]
        inv = 1.0 / ssum
        for j in range(WIN):
            p_s[t, pl.ds(j * H, H), :] = e[j] * inv

    def s2_tile(t, hold):
        tn = min(t + 1, NT - 1)
        tp = max(t - 1, 0)
        p0 = [p_s[t, pl.ds(a * H, H), :] for a in range(4)]
        p8 = [shift_fwd(p_s[t, pl.ds((4 + a) * H, H), :], p_s[tn, pl.ds((4 + a) * H, H), :], 8)
              for a in range(4)]
        for d in range(DH):
            r = pl.ds(d * H, H)
            v0 = hold(v_s[t, r, :])
            vp = v_s[tp, r, :]
            vs = [v0] + [shift_back(vp, v0, a) for a in (2, 4, 6)]
            o0 = (p0[0] * vs[0] + p0[1] * vs[1]) + (p0[2] * vs[2] + p0[3] * vs[3])
            o8 = (p8[0] * vs[0] + p8[1] * vs[1]) + (p8[2] * vs[2] + p8[3] * vs[3])
            o = o0 + shift_back(o8_s[r, :], o8, 8)
            o8_s[r, :] = o8
            o_s[t, pl.ds(d * 8, 8), :] = _pack(o)

    def proj(dst, rows0, nrows, blk):
        res = _dot(_unpack(wt_s[pl.ds(rows0 // 2, nrows // 2), :]), tiles(xn_s, blk * P2_T, P2_T))
        for j in range(P2_T):
            dst[blk * P2_T + j] = res[:, j * LANES:(j + 1) * LANES]
        return res

    b1 = b1_v[...].astype(F32).reshape(1, F)
    GR = 32
    gelu_jobs = [(j, rr) for j in range(NF) for rr in range(D // GR)]

    def gelu_job(j, rr, hold):
        bias = hold(jnp.broadcast_to(b1[:, j * LANES:(j + 1) * LANES], (8, LANES)))
        bias = jnp.concatenate([bias, bias], axis=0)
        for q in range(GR // H):
            row = rr * GR + q * H
            g_s[j, pl.ds(row // 2, 8), :] = _pack(_gelu(u_s[j, pl.ds(row, H), :] + bias))

    def spread_gelu(res, njobs, lo=0.0, hi=1.0):
        njobs = min(njobs, len(gelu_jobs))
        hold = make_hold(tie, [res], 1, njobs, lo, hi)
        for _ in range(njobs):
            gelu_job(*gelu_jobs.pop(0), hold)

    n2 = NT // P2_T
    done_t = 0
    for blk in range(n2):
        res = proj(qk_s, 0, 2 * D, blk)
        if blk == 0:
            spread_gelu(res, 20, 0.0, 0.25)
        if blk == 1:
            hold = make_hold(tie, [res], 1, 12, 0.0, 0.8)
            for j in range(7, 11):
                wt_transpose(j, hold)
            wt_gather(2)
        if blk == 2:
            wo_prep(make_hold(tie, [res], 1, 3 * 56, 0.0, 0.8))
        while done_t < (blk + 1) * P2_T - 1:
            s1_tile(done_t)
            done_t += 1
    for blk in range(n2):
        res = proj(v_s, 2 * D, D, blk)
        if blk == 0:
            s1_tile(NT - 1, make_hold(tie, [res], 1, DH, 0.0, 0.5))
            spread_gelu(res, 32)
        else:
            spread_gelu(res, 48, 0.0, 1.0 if blk + 1 < n2 else 0.9)
    assert not gelu_jobs

    with jax.named_scope("w2_wait"):
        c_w2.wait()
    tie = make_tie(0)
    n3 = NT // P3_T
    c3 = P3_T * LANES

    def out_copy(t):
        return pltpu.make_async_copy(out_v.at[t], out_hbm.at[:, pl.ds(t * LANES, LANES)],
                                     sems.at[SEM_OUT])

    b2 = b2_v[...].astype(F32).reshape(1, S)
    for i in range(n3):
        ys = []
        for k0, k1 in ((0, 4), (4, 8), (8, 12), (12, 14)):
            y = _dot(tiles(g_s, k0, k1 - k0),
                     w2_v[pl.ds(k0 * LANES, (k1 - k0) * LANES), pl.ds(i * c3, c3)])
            ys.append(y + ys[-1] if ys else y)
        hold = make_hold(tie, ys[:3], 1, P3_T * DH, 0.0, 0.9)
        for j in range(P3_T):
            s2_tile(i * P3_T + j, hold)
        y = _dot(_unpack(wot_s[...]), tiles(o_s, i * P3_T, P3_T)) + ys[-1]
        for j in range(P3_T):
            t = i * P3_T + j
            bias = jnp.broadcast_to(b2[:, t * LANES:(t + 1) * LANES], (H, LANES))
            for d in range(DH):
                r = pl.ds(d * H, H)
                val = x_v[t, r, :].astype(F32) + (y[d * H:(d + 1) * H, j * LANES:(j + 1) * LANES] + bias)
                out_v[t, r, :] = val.astype(BF16)
            out_copy(t).start()

    with jax.named_scope("out_wait"):
        for t in range(NT):
            out_copy(t).wait()


@jax.jit
def pallas_parallel_sum__sliding_local_dilated__mixer_token_mlp__prompt_kernel(
    A_x: jax.Array,
    A_wqkv: jax.Array,
    A_wo: jax.Array,
    B_x: jax.Array,
    B_w1: jax.Array,
    B_b1: jax.Array,
    B_w2: jax.Array,
    B_b2: jax.Array,
):
    del B_x
    xt = jnp.transpose(A_x[0], (1, 0))
    any_spec = pl.BlockSpec(memory_space=pl.ANY)
    out_t = pl.pallas_call(
        _kernel,
        out_shape=jax.ShapeDtypeStruct((D, S), BF16),
        in_specs=[any_spec] * 7,
        out_specs=any_spec,
        scratch_shapes=[
            pltpu.VMEM((NT, D, LANES), BF16),
            pltpu.VMEM((S, F), BF16),
            pltpu.VMEM((F, S), BF16),
            pltpu.VMEM((D, 3 * D), BF16),
            pltpu.VMEM((D, D), BF16),
            pltpu.VMEM((F,), BF16),
            pltpu.VMEM((S,), BF16),
            pltpu.VMEM((NT, D // 2, LANES), U32),
            pltpu.VMEM((NT, D // 2, LANES), U32),
            pltpu.VMEM((NF, D, LANES), F32),
            pltpu.VMEM((NF, D // 2, LANES), U32),
            pltpu.VMEM((3 * D // 2, D), U32),
            pltpu.VMEM((D // 2, D), U32),
            pltpu.VMEM((4, 3 * D, LANES), F32),
            pltpu.VMEM((4, D, LANES), F32),
            pltpu.VMEM((NT, 2 * D, LANES), F32),
            pltpu.VMEM((NT, D, LANES), F32),
            pltpu.VMEM((NT, 4 * H, LANES), F32),
            pltpu.VMEM((NT, WIN * H, LANES), F32),
            pltpu.VMEM((D, LANES), F32),
            pltpu.VMEM((NT, D // 2, LANES), U32),
            pltpu.VMEM((NT, D, LANES), BF16),
            pltpu.VMEM((2, 8, LANES), F32),
            pltpu.SemaphoreType.DMA((N1 + 4,)),
        ],
        compiler_params=pltpu.CompilerParams(vmem_limit_bytes=100 * 1024 * 1024,
                                             disable_bounds_checks=True,
                                             disable_semaphore_checks=True),
    )(xt, A_wqkv, A_wo, B_w1, B_b1, B_w2, B_b2)
    return jnp.transpose(out_t, (1, 0))[None]
```

```python
import jax
import jax.numpy as jnp
import jax.experimental.pallas as pl
import jax.experimental.pallas.tpu as pltpu

S = 2048
D = 448
F = 1792
H = 16
DH = D // H
WIN = 8
DIL = 2
EPS = 1e-5
LANES = 128
NT = S // LANES
NF = F // LANES
F32 = jnp.float32
BF16 = jnp.bfloat16
U32 = jnp.uint32

P1_T = 2
P2_T = 4
P3_T = 2
N1 = NT // P1_T
S1_LAG = 6
NA = 6


def _dot(a, b):
    return jnp.dot(a, b, preferred_element_type=F32)


def _gelu(x):
    c = 0.7978845608028654
    inner = x * (c + (c * 0.044715) * (x * x))
    hx = 0.5 * x
    return hx + hx * jnp.tanh(inner)


def _pack(v):
    return pltpu.bitcast(v.astype(BF16), U32)


def _unpack(v):
    return pltpu.bitcast(v, BF16)


def _kernel(x_hbm, wqkv_hbm, wo_hbm, w1_hbm, b1_hbm, w2_hbm, b2_hbm, out_hbm,
            x_v, w1_v, w2_v, wqkv_v, wo_v, b1_v, b2_v,
            xn_s, h_s, u_s, g_s, wt_s, wot_s, t32, o32, qk_s, v_s, l_s, p_s, o8_s, o_s, out_v, z_s,
            sems):
    c1 = P1_T * LANES
    SEM_LAST, SEM_W2, SEM_OUT = N1 + 1, N1 + 2, N1 + 3

    def x_copy(t, sem):
        col = t * LANES if isinstance(t, int) else pl.multiple_of(t * LANES, LANES)
        return pltpu.make_async_copy(x_hbm.at[:, pl.ds(col, LANES)], x_v.at[t], sems.at[sem])

    def w1_copy(row, sem, col=0, ncol=F):
        return pltpu.make_async_copy(w1_hbm.at[pl.ds(row, c1), pl.ds(col, ncol)],
                                     w1_v.at[pl.ds(row, c1), pl.ds(col, ncol)], sems.at[sem])

    def step_copies(i):
        row = i * c1 if isinstance(i, int) else pl.multiple_of(i * c1, c1)
        return [w1_copy(row, 2 + i)] + [x_copy((i + 1) * P1_T + j, 2 + i) for j in range(P1_T)]

    copies_0 = [x_copy(0, 0), x_copy(1, 0)]
    copies_a = [w1_copy(0, 1, 0, NA * LANES)]
    copies_b = [w1_copy(0, 2, NA * LANES, F - NA * LANES), x_copy(2, 2), x_copy(3, 2)]
    c_w1_last = w1_copy((N1 - 1) * c1, SEM_LAST)
    small = [pltpu.make_async_copy(src, dst, sems.at[SEM_LAST])
             for src, dst in ((wqkv_hbm, wqkv_v), (wo_hbm, wo_v), (b1_hbm, b1_v), (b2_hbm, b2_v))]
    c_w2 = pltpu.make_async_copy(w2_hbm, w2_v, sems.at[SEM_W2])

    for c in copies_0 + copies_a + copies_b:
        c.start()
    for i in range(1, N1 - 1):
        for c in step_copies(i):
            c.start()
    c_w1_last.start()
    for c in small + [c_w2]:
        c.start(priority=1)

    z_s[...] = jnp.zeros_like(z_s)
    o8_s[...] = jnp.zeros_like(o8_s)

    def make_tie(zi):
        never8 = z_s[zi] != 0.0
        never16 = jnp.concatenate([z_s[zi], z_s[zi]], axis=0) != 0.0

        def tie(val, src):
            if val.dtype != src.dtype:
                src = pltpu.bitcast(src, val.dtype)
            if val.shape[0] == 16 and src.shape[0] == 8:
                src = jnp.concatenate([src, src], axis=0)
            return jnp.where(never8 if val.shape[0] == 8 else never16, src, val)
        return tie

    def make_hold(tie, results, ntile_par, n, lo=0.0, hi=1.0):
        pts = []
        for res in results:
            for c in range(0, res.shape[1] // LANES, ntile_par):
                pts += [(res, r, c * LANES) for r in range(0, res.shape[0], 8)]
        state = [0]

        def hold(v):
            k = state[0]
            state[0] += 1
            assert k < n
            res, row, col = pts[min(int((lo + (hi - lo) * k / n) * len(pts)), len(pts) - 1)]
            return tie(v, res[row:row + 8, col:col + LANES])
        return hold

    LG = 7
    NH = 6 * (DH // LG)

    def ln_pass(ld, dst, t, hold):
        def colmean(f, c):
            acc = None
            for g in range(DH // LG):
                cg = hold(c)
                cg = jnp.concatenate([cg, cg], axis=0)
                part = None
                for d in range(g * LG, (g + 1) * LG):
                    v = f(ld(d), cg, d == g * LG)
                    part = v if part is None else part + v
                acc = part if acc is None else acc + part
            m = jnp.sum(acc, axis=0, keepdims=True) * (1.0 / D)
            return jnp.broadcast_to(m, (8, LANES))

        def sq(v, m, first):
            c = v - m
            return c * c
        m = colmean(lambda v, c, first: v + c if first else v, jnp.zeros((8, LANES), F32))
        r = jax.lax.rsqrt(colmean(sq, m) + EPS)
        r = jnp.concatenate([r, r], axis=0)
        for g in range(DH // LG):
            mg = hold(m)
            mg = jnp.concatenate([mg, mg], axis=0)
            for d in range(g * LG, (g + 1) * LG):
                dst[t, pl.ds(d * 8, 8), :] = _pack((ld(d) - mg) * r)

    def ln_tile(t, hold):
        ln_pass(lambda d: x_v[t, pl.ds(d * H, H), :].astype(F32), xn_s, t, hold)
        ln_pass(lambda d: _unpack(xn_s[t, pl.ds(d * 8, 8), :]).astype(F32), h_s, t, hold)

    def tiles(ref, t0, nt):
        return _unpack(jnp.concatenate([ref[t0 + j] for j in range(nt)], axis=1))

    def mixer1(i, j0=0, j1=NF, first=False):
        row = i * c1 if isinstance(i, int) else pl.multiple_of(i * c1, c1)
        part = _dot(tiles(h_s, i * P1_T, P1_T), w1_v[pl.ds(row, c1), pl.ds(j0 * LANES, (j1 - j0) * LANES)])
        for j in range(j0, j1):
            pj = part[:, (j - j0) * LANES:(j - j0 + 1) * LANES]
            if first:
                u_s[j] = pj
            else:
                u_s[j] += pj
        return part

    with jax.named_scope("wait_x0"):
        for c in copies_0:
            c.wait()
    with jax.named_scope("ln0"):
        ln_tile(0, lambda v: v)
        ln_tile(1, lambda v: v)

    with jax.named_scope("wait_a"):
        for c in copies_a:
            c.wait()
    mixer1(0, 0, NA, first=True)

    with jax.named_scope("wait_b"):
        for c in copies_b:
            c.wait()
    tie = make_tie(0)
    part = mixer1(0, NA, NF, first=True)
    hold = make_hold(tie, [part], 2, 2 * NH, 0.0, 0.85)
    ln_tile(2, hold)
    ln_tile(3, hold)

    def p1_body(i, carry):
        with jax.named_scope("p1_wait"):
            for c in step_copies(i):
                c.wait()
        tie = make_tie(jnp.minimum(i, 1))
        part = mixer1(i)
        hold = make_hold(tie, [part], 2, P1_T * NH, 0.0, 0.9)
        for j in range(P1_T):
            ln_tile((i + 1) * P1_T + j, hold)
        return carry

    jax.lax.fori_loop(1, N1 - 1, p1_body, 0)

    with jax.named_scope("big_wait"):
        for c in [c_w1_last] + small:
            c.wait()
    tie = make_tie(0)
    part = mixer1(N1 - 1)

    def wt_transpose(j, hold):
        n = min(LANES, 3 * D - j * LANES)
        for c in range(4):
            r = min(LANES, D - c * LANES)
            blk = wqkv_v[pl.ds(c * LANES, r), pl.ds(j * LANES, n)]
            if n == LANES:
                blk = jnp.concatenate([_unpack(hold(_pack(blk[0:H]))), blk[H:]], axis=0)
            t32[c, pl.ds(j * LANES, n), pl.ds(0, r)] = blk.astype(F32).T

    def wt_gather(p):
        for d in range(DH):
            dst = (2 * d + p) * 8 if p < 2 else (2 * DH + d) * 8
            for c in range(4):
                r = min(LANES, D - c * LANES)
                v = t32[c, pl.ds(p * D + d, H, stride=DH), pl.ds(0, r)]
                wt_s[pl.ds(dst, 8), pl.ds(c * LANES, r)] = _pack(v)

    hold = make_hold(tie, [part], 2, 40, 0.0, 0.75)
    for j in range(7):
        wt_transpose(j, hold)
    wt_gather(0)
    wt_gather(1)
    for j in range(7, 11):
        wt_transpose(j, hold)
    wt_gather(2)

    def wo_prep(hold):
        for c in range(4):
            r = min(LANES, D - c * LANES)
            for g in range(4):
                blk = wo_v[pl.ds(g * 112, 112), pl.ds(c * LANES, r)].astype(F32)
                if r == LANES:
                    blk = jnp.concatenate([hold(blk[q * 8:q * 8 + 8]) for q in range(14)], axis=0)
                o32[c, pl.ds(g * 112, 112), pl.ds(0, r)] = blk
        for c in range(4):
            r = min(LANES, D - c * LANES)
            rows = jnp.concatenate(
                [o32[c, pl.ds(d, H, stride=DH), pl.ds(0, r)] for d in range(DH)], axis=0)
            wot_s[pl.ds(c * 64, r // 2), :] = _pack(rows.T)

    wo_prep(make_hold(tie, [part], 2, 3 * 56, 0.7, 1.0))

    lane = jax.lax.broadcasted_iota(jnp.int32, (H, LANES), 1)
    scale = DH ** -0.5

    def shift_back(prev, cur, a):
        return pltpu.roll(jnp.where(lane >= LANES - a, prev, cur), a, 1)

    def shift_fwd(cur, nxt, b):
        return pltpu.roll(jnp.where(lane < b, nxt, cur), LANES - b, 1)

    def s1_tile(t, hold=None):
        tn = min(t + 1, NT - 1)
        tp = max(t - 1, 0)
        acc = [None] * WIN
        hist = []
        for d in range(DH):
            rq = pl.ds(2 * d * H, H)
            rk = pl.ds((2 * d + 1) * H, H)
            q0 = qk_s[t, rq, :]
            qn = qk_s[tn, rq, :]
            k0 = qk_s[t, rk, :]
            if hold is None:
                k0 = tie(k0, qn)
            else:
                k0 = hold(k0)
                qn = tie(qn, k0)
            kp = qk_s[tp, rk, :]
            pre = [jnp.where(lane < 8, qn, q0)] + [jnp.where(lane >= LANES - a, kp, k0) for a in (2, 4, 6)]
            if d >= S1_LAG:
                pre = [tie(pre[i], hist[d - S1_LAG][4 * (d % 2) + i]) for i in range(4)]
            q8 = pltpu.roll(pre[0], LANES - 8, 1)
            ks = [k0] + [pltpu.roll(pre[i], 2 * i, 1) for i in (1, 2, 3)]
            for a in range(4):
                t0 = q0 * ks[a]
                t8 = q8 * ks[a]
                acc[a] = t0 if d == 0 else acc[a] + t0
                acc[4 + a] = t8 if d == 0 else acc[4 + a] + t8
            hist.append(list(acc))
        for a in range(4):
            l_s[t, pl.ds(a * H, H), :] = acc[4 + a]
        lg = [acc[a] for a in range(4)]
        for a in range(4):
            lg.append(shift_back(l_s[tp, pl.ds(a * H, H), :], acc[4 + a], 8))
        lg = [v * scale for v in lg]
        if t == 0:
            lg = [lg[0]] + [jnp.where(lane >= DIL * j, lg[j], -1e9) for j in range(1, WIN)]
        m = lg[0]
        for j in range(1, WIN):
            m = jnp.maximum(m, lg[j])
        e = [jnp.exp(v - m) for v in lg]
        ssum = e[0]
        for j in range(1, WIN):
            ssum = ssum + e[j]
        inv = 1.0 / ssum
        for j in range(WIN):
            p_s[t, pl.ds(j * H, H), :] = e[j] * inv

    def s2_tile(t, hold):
        tn = min(t + 1, NT - 1)
        tp = max(t - 1, 0)
        p0 = [p_s[t, pl.ds(a * H, H), :] for a in range(4)]
        p8 = [shift_fwd(p_s[t, pl.ds((4 + a) * H, H), :], p_s[tn, pl.ds((4 + a) * H, H), :], 8)
              for a in range(4)]
        for d in range(DH):
            r = pl.ds(d * H, H)
            v0 = hold(v_s[t, r, :])
            vp = v_s[tp, r, :]
            vs = [v0] + [shift_back(vp, v0, a) for a in (2, 4, 6)]
            o0 = (p0[0] * vs[0] + p0[1] * vs[1]) + (p0[2] * vs[2] + p0[3] * vs[3])
            o8 = (p8[0] * vs[0] + p8[1] * vs[1]) + (p8[2] * vs[2] + p8[3] * vs[3])
            o = o0 + shift_back(o8_s[r, :], o8, 8)
            o8_s[r, :] = o8
            o_s[t, pl.ds(d * 8, 8), :] = _pack(o)

    def proj(dst, rows0, nrows, blk):
        res = _dot(_unpack(wt_s[pl.ds(rows0 // 2, nrows // 2), :]), tiles(xn_s, blk * P2_T, P2_T))
        for j in range(P2_T):
            dst[blk * P2_T + j] = res[:, j * LANES:(j + 1) * LANES]
        return res

    b1 = b1_v[...].astype(F32).reshape(1, F)
    GR = 32
    gelu_jobs = [(j, rr) for j in range(NF) for rr in range(D // GR)]

    def gelu_job(j, rr, hold):
        bias = hold(jnp.broadcast_to(b1[:, j * LANES:(j + 1) * LANES], (8, LANES)))
        bias = jnp.concatenate([bias, bias], axis=0)
        for q in range(GR // H):
            row = rr * GR + q * H
            g_s[j, pl.ds(row // 2, 8), :] = _pack(_gelu(u_s[j, pl.ds(row, H), :] + bias))

    def spread_gelu(res, njobs, lo=0.0, hi=1.0):
        njobs = min(njobs, len(gelu_jobs))
        hold = make_hold(tie, [res], 1, njobs, lo, hi)
        for _ in range(njobs):
            gelu_job(*gelu_jobs.pop(0), hold)

    n2 = NT // P2_T
    done_t = 0
    for blk in range(n2):
        res = proj(qk_s, 0, 2 * D, blk)
        if blk == 0:
            spread_gelu(res, 20, 0.0, 0.25)
        while done_t < (blk + 1) * P2_T - 1:
            s1_tile(done_t)
            done_t += 1
    for blk in range(n2):
        res = proj(v_s, 2 * D, D, blk)
        if blk == 0:
            s1_tile(NT - 1, make_hold(tie, [res], 1, DH, 0.0, 0.5))
            spread_gelu(res, 32)
        else:
            spread_gelu(res, 48, 0.0, 1.0 if blk + 1 < n2 else 0.9)
    assert not gelu_jobs

    with jax.named_scope("w2_wait"):
        c_w2.wait()
    tie = make_tie(0)
    n3 = NT // P3_T
    c3 = P3_T * LANES

    def out_copy(t):
        return pltpu.make_async_copy(out_v.at[t], out_hbm.at[:, pl.ds(t * LANES, LANES)],
                                     sems.at[SEM_OUT])

    b2 = b2_v[...].astype(F32).reshape(1, S)
    for i in range(n3):
        ys = []
        for k0, k1 in ((0, 4), (4, 8), (8, 12), (12, 14)):
            y = _dot(tiles(g_s, k0, k1 - k0),
                     w2_v[pl.ds(k0 * LANES, (k1 - k0) * LANES), pl.ds(i * c3, c3)])
            ys.append(y + ys[-1] if ys else y)
        hold = make_hold(tie, ys[:3], 1, P3_T * DH, 0.0, 0.9)
        for j in range(P3_T):
            s2_tile(i * P3_T + j, hold)
        y = _dot(_unpack(wot_s[...]), tiles(o_s, i * P3_T, P3_T)) + ys[-1]
        for j in range(P3_T):
            t = i * P3_T + j
            bias = jnp.broadcast_to(b2[:, t * LANES:(t + 1) * LANES], (H, LANES))
            for d in range(DH):
                r = pl.ds(d * H, H)
                val = x_v[t, r, :].astype(F32) + (y[d * H:(d + 1) * H, j * LANES:(j + 1) * LANES] + bias)
                out_v[t, r, :] = val.astype(BF16)
            out_copy(t).start()

    with jax.named_scope("out_wait"):
        for t in range(NT):
            out_copy(t).wait()


@jax.jit
def pallas_parallel_sum__sliding_local_dilated__mixer_token_mlp__prompt_kernel(
    A_x: jax.Array,
    A_wqkv: jax.Array,
    A_wo: jax.Array,
    B_x: jax.Array,
    B_w1: jax.Array,
    B_b1: jax.Array,
    B_w2: jax.Array,
    B_b2: jax.Array,
):
    del B_x
    xt = jnp.transpose(A_x[0], (1, 0))
    any_spec = pl.BlockSpec(memory_space=pl.ANY)
    out_t = pl.pallas_call(
        _kernel,
        out_shape=jax.ShapeDtypeStruct((D, S), BF16),
        in_specs=[any_spec] * 7,
        out_specs=any_spec,
        scratch_shapes=[
            pltpu.VMEM((NT, D, LANES), BF16),
            pltpu.VMEM((S, F), BF16),
            pltpu.VMEM((F, S), BF16),
            pltpu.VMEM((D, 3 * D), BF16),
            pltpu.VMEM((D, D), BF16),
            pltpu.VMEM((F,), BF16),
            pltpu.VMEM((S,), BF16),
            pltpu.VMEM((NT, D // 2, LANES), U32),
            pltpu.VMEM((NT, D // 2, LANES), U32),
            pltpu.VMEM((NF, D, LANES), F32),
            pltpu.VMEM((NF, D // 2, LANES), U32),
            pltpu.VMEM((3 * D // 2, D), U32),
            pltpu.VMEM((D // 2, D), U32),
            pltpu.VMEM((4, 3 * D, LANES), F32),
            pltpu.VMEM((4, D, LANES), F32),
            pltpu.VMEM((NT, 2 * D, LANES), F32),
            pltpu.VMEM((NT, D, LANES), F32),
            pltpu.VMEM((NT, 4 * H, LANES), F32),
            pltpu.VMEM((NT, WIN * H, LANES), F32),
            pltpu.VMEM((D, LANES), F32),
            pltpu.VMEM((NT, D // 2, LANES), U32),
            pltpu.VMEM((NT, D, LANES), BF16),
            pltpu.VMEM((2, 8, LANES), F32),
            pltpu.SemaphoreType.DMA((N1 + 4,)),
        ],
        compiler_params=pltpu.CompilerParams(vmem_limit_bytes=100 * 1024 * 1024,
                                             disable_bounds_checks=True,
                                             disable_semaphore_checks=True),
    )(xt, A_wqkv, A_wo, B_w1, B_b1, B_w2, B_b2)
    return jnp.transpose(out_t, (1, 0))[None]
```

```python
import jax
import jax.numpy as jnp
import jax.experimental.pallas as pl
import jax.experimental.pallas.tpu as pltpu

S = 2048
D = 448
F = 1792
H = 16
DH = D // H
WIN = 8
DIL = 2
EPS = 1e-5
LANES = 128
NT = S // LANES
NF = F // LANES
F32 = jnp.float32
BF16 = jnp.bfloat16
U32 = jnp.uint32

P1_T = 2
P2_T = 4
P3_T = 2
N1 = NT // P1_T
S1_LAG = 6
NA = 6


def _dot(a, b):
    return jnp.dot(a, b, preferred_element_type=F32)


def _gelu(x):
    c = 0.7978845608028654
    inner = x * (c + (c * 0.044715) * (x * x))
    hx = 0.5 * x
    return hx + hx * jnp.tanh(inner)


def _pack(v):
    return pltpu.bitcast(v.astype(BF16), U32)


def _unpack(v):
    return pltpu.bitcast(v, BF16)


def _kernel(x_hbm, wqkv_hbm, wo_hbm, w1_hbm, b1_hbm, w2_hbm, b2_hbm, out_hbm,
            x_v, w1_v, w2_v, wqkv_v, wo_v, b1_v, b2_v,
            xn_s, h_s, u_s, g_s, wt_s, wot_s, t32, o32, qk_s, v_s, l_s, p_s, o8_s, o_s, out_v, z_s,
            sems):
    c1 = P1_T * LANES
    SEM_LAST, SEM_W2, SEM_OUT = N1 + 1, N1 + 2, N1 + 3

    def x_copy(t, sem):
        col = t * LANES if isinstance(t, int) else pl.multiple_of(t * LANES, LANES)
        return pltpu.make_async_copy(x_hbm.at[:, pl.ds(col, LANES)], x_v.at[t], sems.at[sem])

    def w1_copy(row, sem, col=0, ncol=F):
        return pltpu.make_async_copy(w1_hbm.at[pl.ds(row, c1), pl.ds(col, ncol)],
                                     w1_v.at[pl.ds(row, c1), pl.ds(col, ncol)], sems.at[sem])

    def step_copies(i):
        row = i * c1 if isinstance(i, int) else pl.multiple_of(i * c1, c1)
        return [w1_copy(row, 2 + i)] + [x_copy((i + 1) * P1_T + j, 2 + i) for j in range(P1_T)]

    copies_0 = [x_copy(0, 0), x_copy(1, 0)]
    copies_a = [w1_copy(0, 1, 0, NA * LANES)]
    copies_b = [w1_copy(0, 2, NA * LANES, F - NA * LANES), x_copy(2, 2), x_copy(3, 2)]
    c_w1_last = w1_copy((N1 - 1) * c1, SEM_LAST)
    small = [pltpu.make_async_copy(src, dst, sems.at[SEM_LAST])
             for src, dst in ((wqkv_hbm, wqkv_v), (wo_hbm, wo_v), (b1_hbm, b1_v), (b2_hbm, b2_v))]
    c_w2 = pltpu.make_async_copy(w2_hbm, w2_v, sems.at[SEM_W2])

    for c in copies_0 + copies_a + copies_b:
        c.start()
    for i in range(1, N1 - 1):
        for c in step_copies(i):
            c.start()
    c_w1_last.start()
    for c in small + [c_w2]:
        c.start(priority=1)

    z_s[...] = jnp.zeros_like(z_s)
    o8_s[...] = jnp.zeros_like(o8_s)

    def make_tie(zi):
        never8 = z_s[zi] != 0.0
        never16 = jnp.concatenate([z_s[zi], z_s[zi]], axis=0) != 0.0

        def tie(val, src):
            if val.dtype != src.dtype:
                src = pltpu.bitcast(src, val.dtype)
            if val.shape[0] == 16 and src.shape[0] == 8:
                src = jnp.concatenate([src, src], axis=0)
            return jnp.where(never8 if val.shape[0] == 8 else never16, src, val)
        return tie

    def make_hold(tie, results, ntile_par, n, lo=0.0, hi=1.0):
        pts = []
        for res in results:
            for c in range(0, res.shape[1] // LANES, ntile_par):
                pts += [(res, r, c * LANES) for r in range(0, res.shape[0], 8)]
        state = [0]

        def hold(v):
            k = state[0]
            state[0] += 1
            assert k < n
            res, row, col = pts[min(int((lo + (hi - lo) * k / n) * len(pts)), len(pts) - 1)]
            return tie(v, res[row:row + 8, col:col + LANES])
        return hold

    LG = 7
    NH = 6 * (DH // LG)

    def ln_pass(ld, dst, t, hold):
        def colmean(f, c):
            acc = None
            for g in range(DH // LG):
                cg = hold(c)
                cg = jnp.concatenate([cg, cg], axis=0)
                part = None
                for d in range(g * LG, (g + 1) * LG):
                    v = f(ld(d), cg, d == g * LG)
                    part = v if part is None else part + v
                acc = part if acc is None else acc + part
            m = jnp.sum(acc, axis=0, keepdims=True) * (1.0 / D)
            return jnp.broadcast_to(m, (8, LANES))

        def sq(v, m, first):
            c = v - m
            return c * c
        m = colmean(lambda v, c, first: v + c if first else v, jnp.zeros((8, LANES), F32))
        r = jax.lax.rsqrt(colmean(sq, m) + EPS)
        r = jnp.concatenate([r, r], axis=0)
        for g in range(DH // LG):
            mg = hold(m)
            mg = jnp.concatenate([mg, mg], axis=0)
            for d in range(g * LG, (g + 1) * LG):
                dst[t, pl.ds(d * 8, 8), :] = _pack((ld(d) - mg) * r)

    def ln_tile(t, hold):
        ln_pass(lambda d: x_v[t, pl.ds(d * H, H), :].astype(F32), xn_s, t, hold)
        ln_pass(lambda d: _unpack(xn_s[t, pl.ds(d * 8, 8), :]).astype(F32), h_s, t, hold)

    def tiles(ref, t0, nt):
        return _unpack(jnp.concatenate([ref[t0 + j] for j in range(nt)], axis=1))

    def mixer1(i, j0=0, j1=NF, first=False, tie=None):
        row = i * c1 if isinstance(i, int) else pl.multiple_of(i * c1, c1)
        h = jnp.concatenate([h_s[i * P1_T + j] for j in range(P1_T)], axis=1)
        if tie is not None:
            zero = z_s[0]
            h = jnp.concatenate(
                [jnp.concatenate([tie(h[r:r + 8, j * LANES:(j + 1) * LANES], zero) for j in range(P1_T)], axis=1)
                 for r in range(0, D // 2, 8)], axis=0)
        part = _dot(_unpack(h), w1_v[pl.ds(row, c1), pl.ds(j0 * LANES, (j1 - j0) * LANES)])
        for j in range(j0, j1):
            pj = part[:, (j - j0) * LANES:(j - j0 + 1) * LANES]
            if first:
                u_s[j] = pj
            else:
                u_s[j] += pj
        return part

    with jax.named_scope("wait_x0"):
        for c in copies_0:
            c.wait()
    with jax.named_scope("ln0"):
        ln_tile(0, lambda v: v)
        ln_tile(1, lambda v: v)

    with jax.named_scope("wait_a"):
        for c in copies_a:
            c.wait()
    mixer1(0, 0, NA, first=True)

    with jax.named_scope("wait_b"):
        for c in copies_b:
            c.wait()
    tie = make_tie(0)
    part = mixer1(0, NA, NF, first=True)
    hold = make_hold(tie, [part], 2, 2 * NH, 0.0, 0.85)
    ln_tile(2, hold)
    ln_tile(3, hold)

    def p1_body(i, carry):
        with jax.named_scope("p1_wait"):
            for c in step_copies(i):
                c.wait()
        tie = make_tie(jnp.minimum(i, 1))
        part = mixer1(i, tie=tie)
        hold = make_hold(tie, [part], 2, P1_T * NH, 0.0, 0.9)
        for j in range(P1_T):
            ln_tile((i + 1) * P1_T + j, hold)
        return carry

    jax.lax.fori_loop(1, N1 - 1, p1_body, 0)

    with jax.named_scope("big_wait"):
        for c in [c_w1_last] + small:
            c.wait()
    tie = make_tie(0)
    part = mixer1(N1 - 1)

    def wt_transpose(j, hold):
        n = min(LANES, 3 * D - j * LANES)
        for c in range(4):
            r = min(LANES, D - c * LANES)
            blk = wqkv_v[pl.ds(c * LANES, r), pl.ds(j * LANES, n)]
            if n == LANES:
                blk = jnp.concatenate([_unpack(hold(_pack(blk[0:H]))), blk[H:]], axis=0)
            t32[c, pl.ds(j * LANES, n), pl.ds(0, r)] = blk.astype(F32).T

    def wt_gather(p):
        for d in range(DH):
            dst = (2 * d + p) * 8 if p < 2 else (2 * DH + d) * 8
            for c in range(4):
                r = min(LANES, D - c * LANES)
                v = t32[c, pl.ds(p * D + d, H, stride=DH), pl.ds(0, r)]
                wt_s[pl.ds(dst, 8), pl.ds(c * LANES, r)] = _pack(v)

    hold = make_hold(tie, [part], 2, 40, 0.0, 0.75)
    for j in range(7):
        wt_transpose(j, hold)
    wt_gather(0)
    wt_gather(1)
    for j in range(7, 11):
        wt_transpose(j, hold)
    wt_gather(2)

    def wo_prep(hold):
        for c in range(4):
            r = min(LANES, D - c * LANES)
            for g in range(4):
                blk = wo_v[pl.ds(g * 112, 112), pl.ds(c * LANES, r)].astype(F32)
                if r == LANES:
                    blk = jnp.concatenate([hold(blk[q * 8:q * 8 + 8]) for q in range(14)], axis=0)
                o32[c, pl.ds(g * 112, 112), pl.ds(0, r)] = blk
        for c in range(4):
            r = min(LANES, D - c * LANES)
            rows = jnp.concatenate(
                [o32[c, pl.ds(d, H, stride=DH), pl.ds(0, r)] for d in range(DH)], axis=0)
            wot_s[pl.ds(c * 64, r // 2), :] = _pack(rows.T)

    wo_prep(make_hold(tie, [part], 2, 3 * 56, 0.7, 1.0))

    lane = jax.lax.broadcasted_iota(jnp.int32, (H, LANES), 1)
    scale = DH ** -0.5

    def shift_back(prev, cur, a):
        return pltpu.roll(jnp.where(lane >= LANES - a, prev, cur), a, 1)

    def shift_fwd(cur, nxt, b):
        return pltpu.roll(jnp.where(lane < b, nxt, cur), LANES - b, 1)

    def s1_tile(t, hold=None):
        tn = min(t + 1, NT - 1)
        tp = max(t - 1, 0)
        acc = [None] * WIN
        hist = []
        for d in range(DH):
            rq = pl.ds(2 * d * H, H)
            rk = pl.ds((2 * d + 1) * H, H)
            q0 = qk_s[t, rq, :]
            qn = qk_s[tn, rq, :]
            k0 = qk_s[t, rk, :]
            if hold is None:
                k0 = tie(k0, qn)
            else:
                k0 = hold(k0)
                qn = tie(qn, k0)
            kp = qk_s[tp, rk, :]
            pre = [jnp.where(lane < 8, qn, q0)] + [jnp.where(lane >= LANES - a, kp, k0) for a in (2, 4, 6)]
            if d >= S1_LAG:
                pre = [tie(pre[i], hist[d - S1_LAG][4 * (d % 2) + i]) for i in range(4)]
            q8 = pltpu.roll(pre[0], LANES - 8, 1)
            ks = [k0] + [pltpu.roll(pre[i], 2 * i, 1) for i in (1, 2, 3)]
            for a in range(4):
                t0 = q0 * ks[a]
                t8 = q8 * ks[a]
                acc[a] = t0 if d == 0 else acc[a] + t0
                acc[4 + a] = t8 if d == 0 else acc[4 + a] + t8
            hist.append(list(acc))
        for a in range(4):
            l_s[t, pl.ds(a * H, H), :] = acc[4 + a]
        lg = [acc[a] for a in range(4)]
        for a in range(4):
            lg.append(shift_back(l_s[tp, pl.ds(a * H, H), :], acc[4 + a], 8))
        lg = [v * scale for v in lg]
        if t == 0:
            lg = [lg[0]] + [jnp.where(lane >= DIL * j, lg[j], -1e9) for j in range(1, WIN)]
        m = lg[0]
        for j in range(1, WIN):
            m = jnp.maximum(m, lg[j])
        e = [jnp.exp(v - m) for v in lg]
        ssum = e[0]
        for j in range(1, WIN):
            ssum = ssum + e[j]
        inv = 1.0 / ssum
        for j in range(WIN):
            p_s[t, pl.ds(j * H, H), :] = e[j] * inv

    def s2_tile(t, hold):
        tn = min(t + 1, NT - 1)
        tp = max(t - 1, 0)
        p0 = [p_s[t, pl.ds(a * H, H), :] for a in range(4)]
        p8 = [shift_fwd(p_s[t, pl.ds((4 + a) * H, H), :], p_s[tn, pl.ds((4 + a) * H, H), :], 8)
              for a in range(4)]
        for d in range(DH):
            r = pl.ds(d * H, H)
            v0 = hold(v_s[t, r, :])
            vp = v_s[tp, r, :]
            vs = [v0] + [shift_back(vp, v0, a) for a in (2, 4, 6)]
            o0 = (p0[0] * vs[0] + p0[1] * vs[1]) + (p0[2] * vs[2] + p0[3] * vs[3])
            o8 = (p8[0] * vs[0] + p8[1] * vs[1]) + (p8[2] * vs[2] + p8[3] * vs[3])
            o = o0 + shift_back(o8_s[r, :], o8, 8)
            o8_s[r, :] = o8
            o_s[t, pl.ds(d * 8, 8), :] = _pack(o)

    def proj(dst, rows0, nrows, blk):
        res = _dot(_unpack(wt_s[pl.ds(rows0 // 2, nrows // 2), :]), tiles(xn_s, blk * P2_T, P2_T))
        for j in range(P2_T):
            dst[blk * P2_T + j] = res[:, j * LANES:(j + 1) * LANES]
        return res

    b1 = b1_v[...].astype(F32).reshape(1, F)
    GR = 32
    gelu_jobs = [(j, rr) for j in range(NF) for rr in range(D // GR)]

    def gelu_job(j, rr, hold):
        bias = hold(jnp.broadcast_to(b1[:, j * LANES:(j + 1) * LANES], (8, LANES)))
        bias = jnp.concatenate([bias, bias], axis=0)
        for q in range(GR // H):
            row = rr * GR + q * H
            g_s[j, pl.ds(row // 2, 8), :] = _pack(_gelu(u_s[j, pl.ds(row, H), :] + bias))

    def spread_gelu(res, njobs, lo=0.0, hi=1.0):
        njobs = min(njobs, len(gelu_jobs))
        hold = make_hold(tie, [res], 1, njobs, lo, hi)
        for _ in range(njobs):
            gelu_job(*gelu_jobs.pop(0), hold)

    n2 = NT // P2_T
    done_t = 0
    for blk in range(n2):
        res = proj(qk_s, 0, 2 * D, blk)
        if blk == 0:
            spread_gelu(res, 20, 0.0, 0.25)
        while done_t < (blk + 1) * P2_T - 1:
            s1_tile(done_t)
            done_t += 1
    for blk in range(n2):
        res = proj(v_s, 2 * D, D, blk)
        if blk == 0:
            s1_tile(NT - 1, make_hold(tie, [res], 1, DH, 0.0, 0.5))
            spread_gelu(res, 32)
        else:
            spread_gelu(res, 48, 0.0, 1.0 if blk + 1 < n2 else 0.9)
    assert not gelu_jobs

    with jax.named_scope("w2_wait"):
        c_w2.wait()
    tie = make_tie(0)
    n3 = NT // P3_T
    c3 = P3_T * LANES

    def out_copy(t):
        return pltpu.make_async_copy(out_v.at[t], out_hbm.at[:, pl.ds(t * LANES, LANES)],
                                     sems.at[SEM_OUT])

    b2 = b2_v[...].astype(F32).reshape(1, S)
    for i in range(n3):
        ys = []
        for k0, k1 in ((0, 4), (4, 8), (8, 12), (12, 14)):
            y = _dot(tiles(g_s, k0, k1 - k0),
                     w2_v[pl.ds(k0 * LANES, (k1 - k0) * LANES), pl.ds(i * c3, c3)])
            ys.append(y + ys[-1] if ys else y)
        hold = make_hold(tie, ys[:3], 1, P3_T * DH, 0.0, 0.9)
        for j in range(P3_T):
            s2_tile(i * P3_T + j, hold)
        y = _dot(_unpack(wot_s[...]), tiles(o_s, i * P3_T, P3_T)) + ys[-1]
        for j in range(P3_T):
            t = i * P3_T + j
            bias = jnp.broadcast_to(b2[:, t * LANES:(t + 1) * LANES], (H, LANES))
            for d in range(DH):
                r = pl.ds(d * H, H)
                val = x_v[t, r, :].astype(F32) + (y[d * H:(d + 1) * H, j * LANES:(j + 1) * LANES] + bias)
                out_v[t, r, :] = val.astype(BF16)
            out_copy(t).start()

    with jax.named_scope("out_wait"):
        for t in range(NT):
            out_copy(t).wait()


@jax.jit
def pallas_parallel_sum__sliding_local_dilated__mixer_token_mlp__prompt_kernel(
    A_x: jax.Array,
    A_wqkv: jax.Array,
    A_wo: jax.Array,
    B_x: jax.Array,
    B_w1: jax.Array,
    B_b1: jax.Array,
    B_w2: jax.Array,
    B_b2: jax.Array,
):
    del B_x
    xt = jnp.transpose(A_x[0], (1, 0))
    any_spec = pl.BlockSpec(memory_space=pl.ANY)
    out_t = pl.pallas_call(
        _kernel,
        out_shape=jax.ShapeDtypeStruct((D, S), BF16),
        in_specs=[any_spec] * 7,
        out_specs=any_spec,
        scratch_shapes=[
            pltpu.VMEM((NT, D, LANES), BF16),
            pltpu.VMEM((S, F), BF16),
            pltpu.VMEM((F, S), BF16),
            pltpu.VMEM((D, 3 * D), BF16),
            pltpu.VMEM((D, D), BF16),
            pltpu.VMEM((F,), BF16),
            pltpu.VMEM((S,), BF16),
            pltpu.VMEM((NT, D // 2, LANES), U32),
            pltpu.VMEM((NT, D // 2, LANES), U32),
            pltpu.VMEM((NF, D, LANES), F32),
            pltpu.VMEM((NF, D // 2, LANES), U32),
            pltpu.VMEM((3 * D // 2, D), U32),
            pltpu.VMEM((D // 2, D), U32),
            pltpu.VMEM((4, 3 * D, LANES), F32),
            pltpu.VMEM((4, D, LANES), F32),
            pltpu.VMEM((NT, 2 * D, LANES), F32),
            pltpu.VMEM((NT, D, LANES), F32),
            pltpu.VMEM((NT, 4 * H, LANES), F32),
            pltpu.VMEM((NT, WIN * H, LANES), F32),
            pltpu.VMEM((D, LANES), F32),
            pltpu.VMEM((NT, D // 2, LANES), U32),
            pltpu.VMEM((NT, D, LANES), BF16),
            pltpu.VMEM((2, 8, LANES), F32),
            pltpu.SemaphoreType.DMA((N1 + 4,)),
        ],
        compiler_params=pltpu.CompilerParams(vmem_limit_bytes=100 * 1024 * 1024,
                                             disable_bounds_checks=True,
                                             disable_semaphore_checks=True),
    )(xt, A_wqkv, A_wo, B_w1, B_b1, B_w2, B_b2)
    return jnp.transpose(out_t, (1, 0))[None]
```

```python
import jax
import jax.numpy as jnp
import jax.experimental.pallas as pl
import jax.experimental.pallas.tpu as pltpu

S = 2048
D = 448
F = 1792
H = 16
DH = D // H
WIN = 8
DIL = 2
EPS = 1e-5
LANES = 128
NT = S // LANES
NF = F // LANES
F32 = jnp.float32
BF16 = jnp.bfloat16
U32 = jnp.uint32

P1_T = 2
P2_T = 4
P3_T = 2
N1 = NT // P1_T
S1_LAG = 6
NA = 6


def _dot(a, b):
    return jnp.dot(a, b, preferred_element_type=F32)


def _gelu(x):
    c = 0.7978845608028654
    inner = x * (c + (c * 0.044715) * (x * x))
    hx = 0.5 * x
    return hx + hx * jnp.tanh(inner)


def _pack(v):
    return pltpu.bitcast(v.astype(BF16), U32)


def _unpack(v):
    return pltpu.bitcast(v, BF16)


def _kernel(x_hbm, wqkv_hbm, wo_hbm, w1_hbm, b1_hbm, w2_hbm, b2_hbm, out_hbm,
            x_v, w1_v, w2_v, wqkv_v, wo_v, b1_v, b2_v,
            xn_s, h_s, u_s, g_s, wt_s, wot_s, t32, o32, qk_s, v_s, l_s, p_s, o8_s, o_s, out_v, z_s,
            sems):
    c1 = P1_T * LANES
    SEM_LAST, SEM_W2, SEM_OUT = N1 + 1, N1 + 2, N1 + 3

    def x_copy(t, sem):
        col = t * LANES if isinstance(t, int) else pl.multiple_of(t * LANES, LANES)
        return pltpu.make_async_copy(x_hbm.at[:, pl.ds(col, LANES)], x_v.at[t], sems.at[sem])

    def w1_copy(row, sem, col=0, ncol=F):
        return pltpu.make_async_copy(w1_hbm.at[pl.ds(row, c1), pl.ds(col, ncol)],
                                     w1_v.at[pl.ds(row, c1), pl.ds(col, ncol)], sems.at[sem])

    def step_copies(i):
        row = i * c1 if isinstance(i, int) else pl.multiple_of(i * c1, c1)
        return [w1_copy(row, 2 + i)] + [x_copy((i + 1) * P1_T + j, 2 + i) for j in range(P1_T)]

    copies_0 = [x_copy(0, 0), x_copy(1, 0)]
    copies_a = [w1_copy(0, 1, 0, NA * LANES)]
    copies_b = [w1_copy(0, 2, NA * LANES, F - NA * LANES), x_copy(2, 2), x_copy(3, 2)]
    c_w1_last = w1_copy((N1 - 1) * c1, SEM_LAST)
    small = [pltpu.make_async_copy(src, dst, sems.at[SEM_LAST])
             for src, dst in ((wqkv_hbm, wqkv_v), (wo_hbm, wo_v), (b1_hbm, b1_v), (b2_hbm, b2_v))]
    c_w2 = pltpu.make_async_copy(w2_hbm, w2_v.at[:, pl.ds(0, S)], sems.at[SEM_W2])

    for c in copies_0 + copies_a + copies_b:
        c.start()
    for i in range(1, N1 - 1):
        for c in step_copies(i):
            c.start()
    c_w1_last.start()
    for c in small + [c_w2]:
        c.start(priority=1)

    z_s[...] = jnp.zeros_like(z_s)
    o8_s[...] = jnp.zeros_like(o8_s)

    def make_tie(zi):
        never8 = z_s[zi] != 0.0
        never16 = jnp.concatenate([z_s[zi], z_s[zi]], axis=0) != 0.0

        def tie(val, src):
            if val.dtype != src.dtype:
                src = pltpu.bitcast(src, val.dtype)
            if val.shape[0] == 16 and src.shape[0] == 8:
                src = jnp.concatenate([src, src], axis=0)
            return jnp.where(never8 if val.shape[0] == 8 else never16, src, val)
        return tie

    def make_hold(tie, results, ntile_par, n, lo=0.0, hi=1.0):
        pts = []
        for res in results:
            for c in range(0, res.shape[1] // LANES, ntile_par):
                pts += [(res, r, c * LANES) for r in range(0, res.shape[0], 8)]
        state = [0]

        def hold(v):
            k = state[0]
            state[0] += 1
            assert k < n
            res, row, col = pts[min(int((lo + (hi - lo) * k / n) * len(pts)), len(pts) - 1)]
            return tie(v, res[row:row + 8, col:col + LANES])
        return hold

    LG = 7
    NH = 6 * (DH // LG)

    def ln_pass(ld, dst, t, hold):
        def colmean(f, c):
            acc = None
            for g in range(DH // LG):
                cg = hold(c)
                cg = jnp.concatenate([cg, cg], axis=0)
                part = None
                for d in range(g * LG, (g + 1) * LG):
                    v = f(ld(d), cg, d == g * LG)
                    part = v if part is None else part + v
                acc = part if acc is None else acc + part
            m = jnp.sum(acc, axis=0, keepdims=True) * (1.0 / D)
            return jnp.broadcast_to(m, (8, LANES))

        def sq(v, m, first):
            c = v - m
            return c * c
        m = colmean(lambda v, c, first: v + c if first else v, jnp.zeros((8, LANES), F32))
        r = jax.lax.rsqrt(colmean(sq, m) + EPS)
        r = jnp.concatenate([r, r], axis=0)
        for g in range(DH // LG):
            mg = hold(m)
            mg = jnp.concatenate([mg, mg], axis=0)
            for d in range(g * LG, (g + 1) * LG):
                dst[t, pl.ds(d * 8, 8), :] = _pack((ld(d) - mg) * r)

    def ln_tile(t, hold):
        ln_pass(lambda d: x_v[t, pl.ds(d * H, H), :].astype(F32), xn_s, t, hold)
        ln_pass(lambda d: _unpack(xn_s[t, pl.ds(d * 8, 8), :]).astype(F32), h_s, t, hold)

    def tiles(ref, t0, nt):
        return _unpack(jnp.concatenate([ref[t0 + j] for j in range(nt)], axis=1))

    def mixer1(i, j0=0, j1=NF, first=False, tie=None):
        row = i * c1 if isinstance(i, int) else pl.multiple_of(i * c1, c1)
        h = jnp.concatenate([h_s[i * P1_T + j] for j in range(P1_T)], axis=1)
        if tie is not None:
            zero = z_s[0]
            h = jnp.concatenate(
                [jnp.concatenate([tie(h[r:r + 8, j * LANES:(j + 1) * LANES], zero) for j in range(P1_T)], axis=1)
                 for r in range(0, D // 2, 8)], axis=0)
        part = _dot(_unpack(h), w1_v[pl.ds(row, c1), pl.ds(j0 * LANES, (j1 - j0) * LANES)])
        for j in range(j0, j1):
            pj = part[:, (j - j0) * LANES:(j - j0 + 1) * LANES]
            if first:
                u_s[j] = pj
            else:
                u_s[j] += pj
        return part

    with jax.named_scope("wait_x0"):
        for c in copies_0:
            c.wait()
    with jax.named_scope("ln0"):
        ln_tile(0, lambda v: v)
        ln_tile(1, lambda v: v)

    with jax.named_scope("wait_a"):
        for c in copies_a:
            c.wait()
    mixer1(0, 0, NA, first=True)

    with jax.named_scope("wait_b"):
        for c in copies_b:
            c.wait()
    tie = make_tie(0)
    part = mixer1(0, NA, NF, first=True)
    hold = make_hold(tie, [part], 2, 2 * NH, 0.0, 0.85)
    ln_tile(2, hold)
    ln_tile(3, hold)

    def p1_body(i, carry):
        with jax.named_scope("p1_wait"):
            for c in step_copies(i):
                c.wait()
        tie = make_tie(jnp.minimum(i, 1))
        part = mixer1(i, tie=tie)
        hold = make_hold(tie, [part], 2, P1_T * NH, 0.0, 0.9)
        for j in range(P1_T):
            ln_tile((i + 1) * P1_T + j, hold)
        return carry

    jax.lax.fori_loop(1, N1 - 1, p1_body, 0)

    with jax.named_scope("big_wait"):
        for c in [c_w1_last] + small:
            c.wait()
    tie = make_tie(0)
    part = mixer1(N1 - 1)

    def wt_transpose(j, hold):
        n = min(LANES, 3 * D - j * LANES)
        for c in range(4):
            r = min(LANES, D - c * LANES)
            blk = wqkv_v[pl.ds(c * LANES, r), pl.ds(j * LANES, n)]
            if n == LANES:
                blk = jnp.concatenate([_unpack(hold(_pack(blk[0:H]))), blk[H:]], axis=0)
            t32[c, pl.ds(j * LANES, n), pl.ds(0, r)] = blk.astype(F32).T

    def wt_gather(p):
        for d in range(DH):
            dst = (2 * d + p) * 8 if p < 2 else (2 * DH + d) * 8
            for c in range(4):
                r = min(LANES, D - c * LANES)
                v = t32[c, pl.ds(p * D + d, H, stride=DH), pl.ds(0, r)]
                wt_s[pl.ds(dst, 8), pl.ds(c * LANES, r)] = _pack(v)

    hold = make_hold(tie, [part], 2, 40, 0.0, 0.75)
    for j in range(7):
        wt_transpose(j, hold)
    wt_gather(0)
    wt_gather(1)
    for j in range(7, 11):
        wt_transpose(j, hold)
    wt_gather(2)

    def wo_prep(hold):
        for c in range(4):
            r = min(LANES, D - c * LANES)
            for g in range(4):
                blk = wo_v[pl.ds(g * 112, 112), pl.ds(c * LANES, r)].astype(F32)
                if r == LANES:
                    blk = jnp.concatenate([hold(blk[q * 8:q * 8 + 8]) for q in range(14)], axis=0)
                o32[c, pl.ds(g * 112, 112), pl.ds(0, r)] = blk
        for c in range(4):
            r = min(LANES, D - c * LANES)
            rows = jnp.concatenate(
                [o32[c, pl.ds(d, H, stride=DH), pl.ds(0, r)] for d in range(DH)], axis=0)
            wot_s[pl.ds(c * 64, r // 2), :] = _pack(rows.T)

    wo_prep(make_hold(tie, [part], 2, 3 * 56, 0.7, 1.0))

    lane = jax.lax.broadcasted_iota(jnp.int32, (H, LANES), 1)
    scale = DH ** -0.5

    def shift_back(prev, cur, a):
        return pltpu.roll(jnp.where(lane >= LANES - a, prev, cur), a, 1)

    def shift_fwd(cur, nxt, b):
        return pltpu.roll(jnp.where(lane < b, nxt, cur), LANES - b, 1)

    def s1_tile(t, res, hold=None):
        tn = min(t + 1, NT - 1)
        tp = max(t - 1, 0)
        acc = [None] * WIN
        hist = []
        for d in range(DH):
            rq = pl.ds(2 * d * H, H)
            rk = pl.ds((2 * d + 1) * H, H)
            q0 = qk_s[t, rq, :]
            k0 = qk_s[t, rk, :]
            if hold is None:
                cn = (tn % P2_T) * LANES
                qn = res[2 * d * H:(2 * d + 1) * H, cn:cn + LANES]
                k0 = tie(k0, qn)
            else:
                qn = q0
                k0 = hold(k0)
                qn = tie(qn, k0)
            kp = qk_s[tp, rk, :]
            pre = [jnp.where(lane < 8, qn, q0)] + [jnp.where(lane >= LANES - a, kp, k0) for a in (2, 4, 6)]
            if d >= S1_LAG:
                pre = [tie(pre[i], hist[d - S1_LAG][4 * (d % 2) + i]) for i in range(4)]
            q8 = pltpu.roll(pre[0], LANES - 8, 1)
            ks = [k0] + [pltpu.roll(pre[i], 2 * i, 1) for i in (1, 2, 3)]
            for a in range(4):
                t0 = q0 * ks[a]
                t8 = q8 * ks[a]
                acc[a] = t0 if d == 0 else acc[a] + t0
                acc[4 + a] = t8 if d == 0 else acc[4 + a] + t8
            hist.append(list(acc))
        for a in range(4):
            l_s[t, pl.ds(a * H, H), :] = acc[4 + a]
        lg = [acc[a] for a in range(4)]
        for a in range(4):
            lg.append(shift_back(l_s[tp, pl.ds(a * H, H), :], acc[4 + a], 8))
        lg = [v * scale for v in lg]
        if t == 0:
            lg = [lg[0]] + [jnp.where(lane >= DIL * j, lg[j], -1e9) for j in range(1, WIN)]
        m = lg[0]
        for j in range(1, WIN):
            m = jnp.maximum(m, lg[j])
        e = [jnp.exp(v - m) for v in lg]
        ssum = e[0]
        for j in range(1, WIN):
            ssum = ssum + e[j]
        inv = 1.0 / ssum
        for j in range(WIN):
            p_s[t, pl.ds(j * H, H), :] = e[j] * inv

    def s2_tile(t, hold):
        tn = min(t + 1, NT - 1)
        tp = max(t - 1, 0)
        p0 = [p_s[t, pl.ds(a * H, H), :] for a in range(4)]
        p8 = [shift_fwd(p_s[t, pl.ds((4 + a) * H, H), :], p_s[tn, pl.ds((4 + a) * H, H), :], 8)
              for a in range(4)]
        for d in range(DH):
            r = pl.ds(d * H, H)
            v0 = hold(v_s[t, r, :])
            vp = v_s[tp, r, :]
            vs = [v0] + [shift_back(vp, v0, a) for a in (2, 4, 6)]
            o0 = (p0[0] * vs[0] + p0[1] * vs[1]) + (p0[2] * vs[2] + p0[3] * vs[3])
            o8 = (p8[0] * vs[0] + p8[1] * vs[1]) + (p8[2] * vs[2] + p8[3] * vs[3])
            o = o0 + shift_back(o8_s[r, :], o8, 8)
            o8_s[r, :] = o8
            o_s[t, pl.ds(d * 8, 8), :] = _pack(o)

    def proj(dst, rows0, nrows, blk):
        res = _dot(_unpack(wt_s[pl.ds(rows0 // 2, nrows // 2), :]), tiles(xn_s, blk * P2_T, P2_T))
        for j in range(P2_T):
            dst[blk * P2_T + j] = res[:, j * LANES:(j + 1) * LANES]
        return res

    b1 = b1_v[...].astype(F32).reshape(1, F)
    GR = 32
    gelu_jobs = [(j, rr) for j in range(NF) for rr in range(D // GR)]

    def gelu_job(j, rr, hold):
        bias = hold(jnp.broadcast_to(b1[:, j * LANES:(j + 1) * LANES], (8, LANES)))
        bias = jnp.concatenate([bias, bias], axis=0)
        for q in range(GR // H):
            row = rr * GR + q * H
            g_s[j, pl.ds(row // 2, 8), :] = _pack(_gelu(u_s[j, pl.ds(row, H), :] + bias))

    def spread_gelu(res, njobs, lo=0.0, hi=1.0):
        njobs = min(njobs, len(gelu_jobs))
        hold = make_hold(tie, [res], 1, njobs, lo, hi)
        for _ in range(njobs):
            gelu_job(*gelu_jobs.pop(0), hold)

    n2 = NT // P2_T
    done_t = 0
    for half in range(2):
        blks = range(half * n2 // 2, (half + 1) * n2 // 2)
        for blk in blks:
            res = proj(qk_s, 0, 2 * D, blk)
            if blk == 0:
                spread_gelu(res, 20, 0.0, 0.25)
            while done_t < (blk + 1) * P2_T - 1:
                s1_tile(done_t, res)
                done_t += 1
        for blk in blks:
            res = proj(v_s, 2 * D, D, blk)
            if blk == n2 // 2:
                s1_tile(NT - 1, None, make_hold(tie, [res], 1, DH, 0.0, 0.5))
                spread_gelu(res, 32)
            else:
                spread_gelu(res, 48, 0.15 if blk == 0 else 0.0, 0.9 if blk == 1 else 1.0)
        if half == 0:
            with jax.named_scope("w2_wait"):
                c_w2.wait()

            @pl.when(z_s[0, 0, 0] != 0.0)
            def _():
                o8_s[...] = jnp.zeros_like(o8_s)

            tie = make_tie(0)
    assert not gelu_jobs

    n3 = NT // P3_T
    c3 = P3_T * LANES

    def out_copy(t):
        return pltpu.make_async_copy(out_v.at[t], out_hbm.at[:, pl.ds(t * LANES, LANES)],
                                     sems.at[SEM_OUT])

    b2 = b2_v[...].astype(F32).reshape(1, S)
    for i in range(n3):
        ys = []
        for k0, k1 in ((0, 4), (4, 8), (8, 12), (12, 14)):
            y = _dot(tiles(g_s, k0, k1 - k0),
                     w2_v[pl.ds(k0 * LANES, (k1 - k0) * LANES), pl.ds(i * c3, c3)])
            ys.append(y + ys[-1] if ys else y)
        hold = make_hold(tie, ys[:3], 1, P3_T * DH, 0.0, 0.9)
        for j in range(P3_T):
            s2_tile(i * P3_T + j, hold)
        y = _dot(_unpack(wot_s[...]), tiles(o_s, i * P3_T, P3_T)) + ys[-1]
        for j in range(P3_T):
            t = i * P3_T + j
            bias = jnp.broadcast_to(b2[:, t * LANES:(t + 1) * LANES], (H, LANES))
            for d in range(DH):
                r = pl.ds(d * H, H)
                val = x_v[t, r, :].astype(F32) + (y[d * H:(d + 1) * H, j * LANES:(j + 1) * LANES] + bias)
                out_v[t, r, :] = val.astype(BF16)
            out_copy(t).start()

    with jax.named_scope("out_wait"):
        for t in range(NT):
            out_copy(t).wait()


@jax.jit
def pallas_parallel_sum__sliding_local_dilated__mixer_token_mlp__prompt_kernel(
    A_x: jax.Array,
    A_wqkv: jax.Array,
    A_wo: jax.Array,
    B_x: jax.Array,
    B_w1: jax.Array,
    B_b1: jax.Array,
    B_w2: jax.Array,
    B_b2: jax.Array,
):
    del B_x
    xt = jnp.transpose(A_x[0], (1, 0))
    any_spec = pl.BlockSpec(memory_space=pl.ANY)
    out_t = pl.pallas_call(
        _kernel,
        out_shape=jax.ShapeDtypeStruct((D, S), BF16),
        in_specs=[any_spec] * 7,
        out_specs=any_spec,
        scratch_shapes=[
            pltpu.VMEM((NT, D, LANES), BF16),
            pltpu.VMEM((S, F), BF16),
            pltpu.VMEM((F, S + LANES), BF16),
            pltpu.VMEM((D, 3 * D), BF16),
            pltpu.VMEM((D, D), BF16),
            pltpu.VMEM((F,), BF16),
            pltpu.VMEM((S,), BF16),
            pltpu.VMEM((NT, D // 2, LANES), U32),
            pltpu.VMEM((NT, D // 2, LANES), U32),
            pltpu.VMEM((NF, D, LANES), F32),
            pltpu.VMEM((NF, D // 2, LANES), U32),
            pltpu.VMEM((3 * D // 2, D), U32),
            pltpu.VMEM((D // 2, D), U32),
            pltpu.VMEM((4, 3 * D, LANES), F32),
            pltpu.VMEM((4, D, LANES), F32),
            pltpu.VMEM((NT, 2 * D, LANES), F32),
            pltpu.VMEM((NT, D, LANES), F32),
            pltpu.VMEM((NT, 4 * H, LANES), F32),
            pltpu.VMEM((NT, WIN * H, LANES), F32),
            pltpu.VMEM((D, LANES), F32),
            pltpu.VMEM((NT, D // 2, LANES), U32),
            pltpu.VMEM((NT, D, LANES), BF16),
            pltpu.VMEM((2, 8, LANES), F32),
            pltpu.SemaphoreType.DMA((N1 + 4,)),
        ],
        compiler_params=pltpu.CompilerParams(vmem_limit_bytes=100 * 1024 * 1024,
                                             disable_bounds_checks=True,
                                             disable_semaphore_checks=True),
    )(xt, A_wqkv, A_wo, B_w1, B_b1, B_w2, B_b2)
    return jnp.transpose(out_t, (1, 0))[None]
```

```python
import jax
import jax.numpy as jnp
import jax.experimental.pallas as pl
import jax.experimental.pallas.tpu as pltpu

S = 2048
D = 448
F = 1792
H = 16
DH = D // H
WIN = 8
DIL = 2
EPS = 1e-5
LOG2E = 1.4426950408889634
LANES = 128
NT = S // LANES
NF = F // LANES
F32 = jnp.float32
BF16 = jnp.bfloat16
U32 = jnp.uint32

P1_T = 2
P3_T = 2
N1 = NT // P1_T
S1_LAG = 6
NA = 6


def _dot(a, b):
    return jnp.dot(a, b, preferred_element_type=F32)


def _gelu(x):
    c = 0.7978845608028654
    inner = x * (c + (c * 0.044715) * (x * x))
    hx = 0.5 * x
    return hx + hx * jnp.tanh(inner)


def _pack(v):
    return pltpu.bitcast(v.astype(BF16), U32)


def _unpack(v):
    return pltpu.bitcast(v, BF16)


def _kernel(x_hbm, wqkv_hbm, wo_hbm, w1_hbm, b1_hbm, w2_hbm, b2_hbm, out_hbm,
            x_v, w1_v, w2_v, wqkv_v, wo_v, b1_v, b2_v,
            xn_s, h_s, u_s, g_s, wt_s, wot_s, t32, o32, qk_s, v_s, l_s, p_s, o8_s, o_s, out_v, z_s,
            sems):
    c1 = P1_T * LANES
    SEM_LAST, SEM_W2, SEM_OUT = N1 + 1, N1 + 2, N1 + 3

    def x_copy(t, sem):
        col = t * LANES if isinstance(t, int) else pl.multiple_of(t * LANES, LANES)
        return pltpu.make_async_copy(x_hbm.at[:, pl.ds(col, LANES)], x_v.at[t], sems.at[sem])

    def w1_copy(row, sem, col=0, ncol=F):
        return pltpu.make_async_copy(w1_hbm.at[pl.ds(row, c1), pl.ds(col, ncol)],
                                     w1_v.at[pl.ds(row, c1), pl.ds(col, ncol)], sems.at[sem])

    def step_copies(i):
        row = i * c1 if isinstance(i, int) else pl.multiple_of(i * c1, c1)
        return [w1_copy(row, 2 + i)] + [x_copy((i + 1) * P1_T + j, 2 + i) for j in range(P1_T)]

    copies_0 = [x_copy(0, 0), x_copy(1, 0)]
    copies_a = [w1_copy(0, 1, 0, NA * LANES)]
    copies_b = [w1_copy(0, 2, NA * LANES, F - NA * LANES), x_copy(2, 2), x_copy(3, 2)]
    c_w1_last = w1_copy((N1 - 1) * c1, SEM_LAST)
    small = [pltpu.make_async_copy(src, dst, sems.at[SEM_LAST])
             for src, dst in ((wqkv_hbm, wqkv_v), (wo_hbm, wo_v), (b1_hbm, b1_v), (b2_hbm, b2_v))]
    c_w2 = pltpu.make_async_copy(w2_hbm, w2_v.at[:, pl.ds(0, S)], sems.at[SEM_W2])

    for c in copies_0 + copies_a + copies_b:
        c.start()
    for i in range(1, N1 - 1):
        for c in step_copies(i):
            c.start()
    c_w1_last.start()
    for c in small + [c_w2]:
        c.start(priority=1)

    z_s[...] = jnp.zeros_like(z_s)
    o8_s[...] = jnp.zeros_like(o8_s)

    def make_tie(zi):
        never8 = z_s[zi] != 0.0
        never16 = jnp.concatenate([z_s[zi], z_s[zi]], axis=0) != 0.0

        def tie(val, src):
            if val.dtype != src.dtype:
                src = pltpu.bitcast(src, val.dtype)
            if val.shape[0] == 16 and src.shape[0] == 8:
                src = jnp.concatenate([src, src], axis=0)
            return jnp.where(never8 if val.shape[0] == 8 else never16, src, val)
        return tie

    def make_hold(tie, results, ntile_par, n, lo=0.0, hi=1.0):
        pts = []
        for res in results:
            for c in range(0, res.shape[1] // LANES, ntile_par):
                pts += [(res, r, c * LANES) for r in range(0, res.shape[0], 8)]
        state = [0]

        def hold(v):
            k = state[0]
            state[0] += 1
            assert k < n
            res, row, col = pts[min(int((lo + (hi - lo) * k / n) * len(pts)), len(pts) - 1)]
            return tie(v, res[row:row + 8, col:col + LANES])
        return hold

    LG = 7
    NH = 6 * (DH // LG)

    def ln_pass(ld, dst, t, hold):
        def colmean(f, c):
            acc = None
            for g in range(DH // LG):
                cg = hold(c)
                cg = jnp.concatenate([cg, cg], axis=0)
                part = None
                for d in range(g * LG, (g + 1) * LG):
                    v = f(ld(d), cg, d == g * LG)
                    part = v if part is None else part + v
                acc = part if acc is None else acc + part
            m = jnp.sum(acc, axis=0, keepdims=True) * (1.0 / D)
            return jnp.broadcast_to(m, (8, LANES))

        def sq(v, m, first):
            c = v - m
            return c * c
        m = colmean(lambda v, c, first: v + c if first else v, jnp.zeros((8, LANES), F32))
        r = jax.lax.rsqrt(colmean(sq, m) + EPS)
        r = jnp.concatenate([r, r], axis=0)
        for g in range(DH // LG):
            mg = hold(m)
            mg = jnp.concatenate([mg, mg], axis=0)
            for d in range(g * LG, (g + 1) * LG):
                dst[t, pl.ds(d * H, H), :] = ((ld(d) - mg) * r).astype(BF16)

    def ln_tile(t, hold):
        ln_pass(lambda d: x_v[t, pl.ds(d * H, H), :].astype(F32), xn_s, t, hold)
        ln_pass(lambda d: xn_s[t, pl.ds(d * H, H), :].astype(F32), h_s, t, hold)

    def tiles(ref, t0, nt):
        return jnp.concatenate([ref[t0 + j] for j in range(nt)], axis=1)

    def mixer1(i, j0=0, j1=NF, first=False):
        row = i * c1 if isinstance(i, int) else pl.multiple_of(i * c1, c1)
        part = _dot(tiles(h_s, i * P1_T, P1_T), w1_v[pl.ds(row, c1), pl.ds(j0 * LANES, (j1 - j0) * LANES)])
        for j in range(j0, j1):
            pj = part[:, (j - j0) * LANES:(j - j0 + 1) * LANES]
            if first:
                u_s[j] = pj
            else:
                u_s[j] += pj
        return part

    with jax.named_scope("wait_x0"):
        for c in copies_0:
            c.wait()
    with jax.named_scope("ln0"):
        ln_tile(0, lambda v: v)
        ln_tile(1, lambda v: v)

    with jax.named_scope("wait_a"):
        for c in copies_a:
            c.wait()
    mixer1(0, 0, NA, first=True)

    with jax.named_scope("wait_b"):
        for c in copies_b:
            c.wait()
    tie = make_tie(0)
    part = mixer1(0, NA, NF, first=True)
    hold = make_hold(tie, [part], 2, 2 * NH, 0.0, 0.85)
    ln_tile(2, hold)
    ln_tile(3, hold)

    def p1_body(i, carry):
        with jax.named_scope("p1_wait"):
            for c in step_copies(i):
                c.wait()
        tie = make_tie(jnp.minimum(i, 1))
        part = mixer1(i)
        hold = make_hold(tie, [part], 2, P1_T * NH, 0.0, 0.9)
        for j in range(P1_T):
            ln_tile((i + 1) * P1_T + j, hold)
        return carry

    jax.lax.fori_loop(1, N1 - 1, p1_body, 0)

    with jax.named_scope("big_wait"):
        for c in [c_w1_last] + small:
            c.wait()
    tie = make_tie(0)
    part = mixer1(N1 - 1)

    def wt_transpose(j, hold):
        n = min(LANES, 3 * D - j * LANES)
        for c in range(4):
            r = min(LANES, D - c * LANES)
            blk = wqkv_v[pl.ds(c * LANES, r), pl.ds(j * LANES, n)]
            if n == LANES:
                blk = jnp.concatenate([_unpack(hold(_pack(blk[0:H]))), blk[H:]], axis=0)
            t32[c, pl.ds(j * LANES, n), pl.ds(0, r)] = blk.astype(F32).T

    def wt_gather(p):
        for d in range(DH):
            dst = (2 * d + p) * 8 if p < 2 else (2 * DH + d) * 8
            for c in range(4):
                r = min(LANES, D - c * LANES)
                v = t32[c, pl.ds(p * D + d, H, stride=DH), pl.ds(0, r)]
                wt_s[pl.ds(dst, 8), pl.ds(c * LANES, r)] = _pack(v)

    hold = make_hold(tie, [part], 2, 40, 0.0, 0.75)
    for j in range(7):
        wt_transpose(j, hold)
    wt_gather(0)
    wt_gather(1)
    for j in range(7, 11):
        wt_transpose(j, hold)
    wt_gather(2)

    def wo_prep(hold):
        for c in range(4):
            r = min(LANES, D - c * LANES)
            for g in range(4):
                blk = wo_v[pl.ds(g * 112, 112), pl.ds(c * LANES, r)].astype(F32)
                if r == LANES:
                    blk = jnp.concatenate([hold(blk[q * 8:q * 8 + 8]) for q in range(14)], axis=0)
                o32[c, pl.ds(g * 112, 112), pl.ds(0, r)] = blk
        for c in range(4):
            r = min(LANES, D - c * LANES)
            rows = jnp.concatenate(
                [o32[c, pl.ds(d, H, stride=DH), pl.ds(0, r)] for d in range(DH)], axis=0)
            wot_s[pl.ds(c * 64, r // 2), :] = _pack(rows.T)

    wo_prep(make_hold(tie, [part], 2, 3 * 56, 0.7, 1.0))

    lane = jax.lax.broadcasted_iota(jnp.int32, (H, LANES), 1)
    scale = DH ** -0.5

    def shift_back(prev, cur, a):
        return pltpu.roll(jnp.where(lane >= LANES - a, prev, cur), a, 1)

    def shift_fwd(cur, nxt, b):
        return pltpu.roll(jnp.where(lane < b, nxt, cur), LANES - b, 1)

    def tree(op, vs):
        while len(vs) > 1:
            vs = [op(vs[i], vs[i + 1]) for i in range(0, len(vs), 2)]
        return vs[0]

    hist = []

    def s1_tile(t, res, hold=None):
        tn = min(t + 1, NT - 1)
        tp = max(t - 1, 0)
        acc = [None] * WIN
        for d in range(DH):
            rq = pl.ds(2 * d * H, H)
            rk = pl.ds((2 * d + 1) * H, H)
            q0 = qk_s[t, rq, :]
            k0 = qk_s[t, rk, :]
            if hold is None:
                qn = res[2 * d * H:(2 * d + 1) * H, :]
                k0 = tie(k0, qn)
            else:
                qn = q0
                k0 = hold(k0)
                qn = tie(qn, k0)
            kp = qk_s[tp, rk, :]
            pre = [jnp.where(lane < 8, qn, q0)] + [jnp.where(lane >= LANES - a, kp, k0) for a in (2, 4, 6)]
            if len(hist) >= S1_LAG:
                pre = [tie(pre[i], hist[-S1_LAG][4 * (d % 2) + i]) for i in range(4)]
            q8 = pltpu.roll(pre[0], LANES - 8, 1)
            ks = [k0] + [pltpu.roll(pre[i], 2 * i, 1) for i in (1, 2, 3)]
            for a in range(4):
                t0 = q0 * ks[a]
                t8 = q8 * ks[a]
                acc[a] = t0 if d == 0 else acc[a] + t0
                acc[4 + a] = t8 if d == 0 else acc[4 + a] + t8
            hist.append(list(acc))
        for a in range(WIN):
            l_s[t, pl.ds(a * H, H), :] = acc[a]
        return tree(jnp.add, acc)

    def softmax_job(t, hh, hold):
        tp = max(t - 1, 0)
        lane8 = lane[0:8]

        def rows(j):
            return pl.ds(j * H + hh * 8, 8)
        lg = [l_s[t, rows(j), :] for j in range(WIN)]
        lg[4] = hold(lg[4])
        lg[5:] = [tie(v, lg[4]) for v in lg[5:]]
        for j in range(4, WIN):
            lg[j] = pltpu.roll(jnp.where(lane8 >= LANES - 8, l_s[tp, rows(j), :], lg[j]), 8, 1)
        if t == 0:
            lg = [lg[0]] + [jnp.where(lane8 >= DIL * j, lg[j], -1e9 / scale) for j in range(1, WIN)]
        m = tree(jnp.maximum, lg)
        e = [jnp.exp2((v - m) * (scale * LOG2E)) for v in lg]
        ssum = tree(jnp.add, e)
        inv = pl.reciprocal(ssum, approx=True)
        inv = inv * (2.0 - ssum * inv)
        for j in range(WIN):
            p_s[t, rows(j), :] = e[j] * inv

    def s2_tile(t, hold):
        tn = min(t + 1, NT - 1)
        tp = max(t - 1, 0)
        p0 = [p_s[t, pl.ds(a * H, H), :] for a in range(4)]
        p8 = [shift_fwd(p_s[t, pl.ds((4 + a) * H, H), :], p_s[tn, pl.ds((4 + a) * H, H), :], 8)
              for a in range(4)]
        for d in range(DH):
            r = pl.ds(d * H, H)
            v0 = hold(v_s[t, r, :])
            vp = v_s[tp, r, :]
            vs = [v0] + [shift_back(vp, v0, a) for a in (2, 4, 6)]
            o0 = (p0[0] * vs[0] + p0[1] * vs[1]) + (p0[2] * vs[2] + p0[3] * vs[3])
            o8 = (p8[0] * vs[0] + p8[1] * vs[1]) + (p8[2] * vs[2] + p8[3] * vs[3])
            o = o0 + shift_back(o8_s[r, :], o8, 8)
            o8_s[r, :] = o8
            o_s[t, r, :] = o.astype(BF16)

    def proj(dst, rows0, nrows, t, after=None):
        xn = xn_s[t]
        if after is not None:
            xn = jnp.concatenate([_unpack(tie(_pack(xn[0:2 * H]), after)), xn[2 * H:]], axis=0)
        res = _dot(_unpack(wt_s[pl.ds(rows0 // 2, nrows // 2), :]), xn)
        dst[t] = res
        return res

    b1 = b1_v[...].astype(F32).reshape(1, F)
    GR = 32
    gelu_jobs = [(j, rr) for j in range(NF) for rr in range(D // GR)]

    def gelu_job(j, rr, hold):
        bias = hold(jnp.broadcast_to(b1[:, j * LANES:(j + 1) * LANES], (8, LANES)))
        bias = jnp.concatenate([bias, bias], axis=0)
        for q in range(GR // H):
            row = rr * GR + q * H
            g_s[j, pl.ds(row, H), :] = _gelu(u_s[j, pl.ds(row, H), :] + bias).astype(BF16)

    def spread_gelu(res, njobs, lo=0.0, hi=1.0):
        njobs = min(njobs, len(gelu_jobs))
        hold = make_hold(tie, res, 1, njobs, lo, hi)
        for _ in range(njobs):
            gelu_job(*gelu_jobs.pop(0), hold)

    for half in range(2):
        ts = range(half * NT // 2, (half + 1) * NT // 2)
        fin = []
        for t in ts:
            res = proj(qk_s, 0, 2 * D, t, fin.pop(0) if len(fin) >= 2 else None)
            if t == 0:
                spread_gelu([res], 20)
            else:
                fin.append(s1_tile(t - 1, res))
                if half == 0:
                    fin.pop()
        vres = []
        for t in ts:
            k = t - ts[0]
            vres.append(proj(v_s, 2 * D, D, t, fin.pop(0) if fin and k in (0, 2, 5) else None))
            if half == 1 and k == 1:
                fin.append(s1_tile(NT - 1, None, make_hold(tie, vres, 1, DH)))
        sm = range(0, NT // 2 - 1) if half == 0 else range(NT // 2 - 1, NT)
        hold = make_hold(tie, vres, 1, 2 * len(sm), 0.1, 0.85)
        for t in sm:
            softmax_job(t, 0, hold)
            softmax_job(t, 1, hold)
        if half == 0:
            spread_gelu(vres, 96, 0.07, 0.95)
        else:
            spread_gelu(vres[:2], 8)
            spread_gelu(vres[2:], 72)
        if half == 0:
            with jax.named_scope("w2_wait"):
                c_w2.wait()

            @pl.when(z_s[0, 0, 0] != 0.0)
            def _():
                o8_s[...] = jnp.zeros_like(o8_s)

            tie = make_tie(0)
            hist.clear()
    assert not gelu_jobs

    n3 = NT // P3_T
    c3 = P3_T * LANES

    def out_copy(t):
        return pltpu.make_async_copy(out_v.at[t], out_hbm.at[:, pl.ds(t * LANES, LANES)],
                                     sems.at[SEM_OUT])

    b2 = b2_v[...].astype(F32).reshape(1, S)
    ksplit = ((0, 4), (4, 8), (8, 12), (12, 14))
    gs = [tiles(g_s, k0, k1 - k0) for k0, k1 in ksplit]
    for i in range(n3):
        ys = []
        for g, (k0, k1) in zip(gs, ksplit):
            y = _dot(g,
                     w2_v[pl.ds(k0 * LANES, (k1 - k0) * LANES), pl.ds(i * c3, c3)])
            ys.append(y + ys[-1] if ys else y)
        hold = make_hold(tie, ys[:3], 1, P3_T * DH, 0.0, 0.9)
        for j in range(P3_T):
            s2_tile(i * P3_T + j, hold)
        y = _dot(_unpack(wot_s[...]), tiles(o_s, i * P3_T, P3_T)) + ys[-1]
        for j in range(P3_T):
            t = i * P3_T + j
            bias = jnp.broadcast_to(b2[:, t * LANES:(t + 1) * LANES], (H, LANES))
            for d in range(DH):
                r = pl.ds(d * H, H)
                val = x_v[t, r, :].astype(F32) + (y[d * H:(d + 1) * H, j * LANES:(j + 1) * LANES] + bias)
                out_v[t, r, :] = val.astype(BF16)
            out_copy(t).start()

    with jax.named_scope("out_wait"):
        for t in range(NT):
            out_copy(t).wait()


@jax.jit
def pallas_parallel_sum__sliding_local_dilated__mixer_token_mlp__prompt_kernel(
    A_x: jax.Array,
    A_wqkv: jax.Array,
    A_wo: jax.Array,
    B_x: jax.Array,
    B_w1: jax.Array,
    B_b1: jax.Array,
    B_w2: jax.Array,
    B_b2: jax.Array,
):
    del B_x
    xt = jnp.transpose(A_x[0], (1, 0))
    any_spec = pl.BlockSpec(memory_space=pl.ANY)
    out_t = pl.pallas_call(
        _kernel,
        out_shape=jax.ShapeDtypeStruct((D, S), BF16),
        in_specs=[any_spec] * 7,
        out_specs=any_spec,
        scratch_shapes=[
            pltpu.VMEM((NT, D, LANES), BF16),
            pltpu.VMEM((S, F), BF16),
            pltpu.VMEM((F, S + LANES), BF16),
            pltpu.VMEM((D, 3 * D), BF16),
            pltpu.VMEM((D, D), BF16),
            pltpu.VMEM((F,), BF16),
            pltpu.VMEM((S,), BF16),
            pltpu.VMEM((NT, D, LANES), BF16),
            pltpu.VMEM((NT, D, LANES), BF16),
            pltpu.VMEM((NF, D, LANES), F32),
            pltpu.VMEM((NF, D, LANES), BF16),
            pltpu.VMEM((3 * D // 2, D), U32),
            pltpu.VMEM((D // 2, D), U32),
            pltpu.VMEM((4, 3 * D, LANES), F32),
            pltpu.VMEM((4, D, LANES), F32),
            pltpu.VMEM((NT, 2 * D, LANES), F32),
            pltpu.VMEM((NT, D, LANES), F32),
            pltpu.VMEM((NT, WIN * H, LANES), F32),
            pltpu.VMEM((NT, WIN * H, LANES), F32),
            pltpu.VMEM((D, LANES), F32),
            pltpu.VMEM((NT, D, LANES), BF16),
            pltpu.VMEM((NT, D, LANES), BF16),
            pltpu.VMEM((2, 8, LANES), F32),
            pltpu.SemaphoreType.DMA((N1 + 4,)),
        ],
        compiler_params=pltpu.CompilerParams(vmem_limit_bytes=100 * 1024 * 1024,
                                             disable_bounds_checks=True,
                                             disable_semaphore_checks=True),
    )(xt, A_wqkv, A_wo, B_w1, B_b1, B_w2, B_b2)
    return jnp.transpose(out_t, (1, 0))[None]
```

```python
import jax
import jax.numpy as jnp
import jax.experimental.pallas as pl
import jax.experimental.pallas.tpu as pltpu

S = 2048
D = 448
F = 1792
H = 16
DH = D // H
WIN = 8
DIL = 2
EPS = 1e-5
LOG2E = 1.4426950408889634
LANES = 128
NT = S // LANES
NF = F // LANES
F32 = jnp.float32
BF16 = jnp.bfloat16
U32 = jnp.uint32

P1_T = 2
P3_T = 2
N1 = NT // P1_T
S1_LAG = 6
NA = 6


def _dot(a, b):
    return jnp.dot(a, b, preferred_element_type=F32)


def _gelu(x):
    c = 0.7978845608028654
    inner = x * (c + (c * 0.044715) * (x * x))
    hx = 0.5 * x
    return hx + hx * jnp.tanh(inner)


def _pack(v):
    return pltpu.bitcast(v.astype(BF16), U32)


def _unpack(v):
    return pltpu.bitcast(v, BF16)


def _kernel(x_hbm, wqkv_hbm, wo_hbm, w1_hbm, b1_hbm, w2_hbm, b2_hbm, out_hbm,
            x_v, w1_v, w2_v, wqkv_v, wo_v, b1_v, b2_v,
            xn_s, h_s, u_s, g_s, wt_s, wot_s, t32, o32, qk_s, v_s, l_s, p_s, o8_s, o_s, out_v, z_s,
            sems):
    c1 = P1_T * LANES
    SEM_LAST, SEM_W2, SEM_OUT = N1 + 1, N1 + 2, N1 + 3

    def x_copy(t, sem):
        col = t * LANES if isinstance(t, int) else pl.multiple_of(t * LANES, LANES)
        return pltpu.make_async_copy(x_hbm.at[:, pl.ds(col, LANES)], x_v.at[t], sems.at[sem])

    def w1_copy(row, sem, col=0, ncol=F):
        return pltpu.make_async_copy(w1_hbm.at[pl.ds(row, c1), pl.ds(col, ncol)],
                                     w1_v.at[pl.ds(row, c1), pl.ds(col, ncol)], sems.at[sem])

    def step_copies(i):
        row = i * c1 if isinstance(i, int) else pl.multiple_of(i * c1, c1)
        return [w1_copy(row, 2 + i)] + [x_copy((i + 1) * P1_T + j, 2 + i) for j in range(P1_T)]

    copies_0 = [x_copy(0, 0), x_copy(1, 0)]
    copies_a = [w1_copy(0, 1, 0, NA * LANES)]
    copies_b = [w1_copy(0, 2, NA * LANES, F - NA * LANES), x_copy(2, 2), x_copy(3, 2)]
    c_w1_last = w1_copy((N1 - 1) * c1, SEM_LAST)
    small = [pltpu.make_async_copy(src, dst, sems.at[SEM_LAST])
             for src, dst in ((wqkv_hbm, wqkv_v), (wo_hbm, wo_v), (b1_hbm, b1_v), (b2_hbm, b2_v))]
    c_w2 = pltpu.make_async_copy(w2_hbm, w2_v.at[:, pl.ds(0, S)], sems.at[SEM_W2])

    for c in copies_0 + copies_a + copies_b:
        c.start()
    for i in range(1, N1 - 1):
        for c in step_copies(i):
            c.start()
    c_w1_last.start()
    for c in small + [c_w2]:
        c.start(priority=1)

    z_s[...] = jnp.zeros_like(z_s)
    o8_s[...] = jnp.zeros_like(o8_s)

    def make_tie(zi):
        never8 = z_s[zi] != 0.0
        never16 = jnp.concatenate([z_s[zi], z_s[zi]], axis=0) != 0.0

        def tie(val, src):
            if val.dtype != src.dtype:
                src = pltpu.bitcast(src, val.dtype)
            if val.shape[0] == 16 and src.shape[0] == 8:
                src = jnp.concatenate([src, src], axis=0)
            return jnp.where(never8 if val.shape[0] == 8 else never16, src, val)
        return tie

    def make_hold(tie, results, ntile_par, n, lo=0.0, hi=1.0):
        pts = []
        for res in results:
            for c in range(0, res.shape[1] // LANES, ntile_par):
                pts += [(res, r, c * LANES) for r in range(0, res.shape[0], 8)]
        state = [0]

        def hold(v):
            k = state[0]
            state[0] += 1
            assert k < n
            res, row, col = pts[min(int((lo + (hi - lo) * k / n) * len(pts)), len(pts) - 1)]
            return tie(v, res[row:row + 8, col:col + LANES])
        return hold

    LG = 7
    NH = 6 * (DH // LG)

    def ln_pass(ld, dst, t, hold):
        def colmean(f, c):
            acc = None
            for g in range(DH // LG):
                cg = hold(c)
                cg = jnp.concatenate([cg, cg], axis=0)
                part = None
                for d in range(g * LG, (g + 1) * LG):
                    v = f(ld(d), cg, d == g * LG)
                    part = v if part is None else part + v
                acc = part if acc is None else acc + part
            m = jnp.sum(acc, axis=0, keepdims=True) * (1.0 / D)
            return jnp.broadcast_to(m, (8, LANES))

        def sq(v, m, first):
            c = v - m
            return c * c
        m = colmean(lambda v, c, first: v + c if first else v, jnp.zeros((8, LANES), F32))
        r = jax.lax.rsqrt(colmean(sq, m) + EPS)
        r = jnp.concatenate([r, r], axis=0)
        for g in range(DH // LG):
            mg = hold(m)
            mg = jnp.concatenate([mg, mg], axis=0)
            for d in range(g * LG, (g + 1) * LG):
                dst[t, pl.ds(d * H, H), :] = ((ld(d) - mg) * r).astype(BF16)

    def ln_tile(t, hold):
        ln_pass(lambda d: x_v[t, pl.ds(d * H, H), :].astype(F32), xn_s, t, hold)
        ln_pass(lambda d: xn_s[t, pl.ds(d * H, H), :].astype(F32), h_s, t, hold)

    def tiles(ref, t0, nt):
        return jnp.concatenate([ref[t0 + j] for j in range(nt)], axis=1)

    def mixer1(i, j0=0, j1=NF, first=False):
        row = i * c1 if isinstance(i, int) else pl.multiple_of(i * c1, c1)
        part = _dot(tiles(h_s, i * P1_T, P1_T), w1_v[pl.ds(row, c1), pl.ds(j0 * LANES, (j1 - j0) * LANES)])
        for j in range(j0, j1):
            pj = part[:, (j - j0) * LANES:(j - j0 + 1) * LANES]
            if first:
                u_s[j] = pj
            else:
                u_s[j] += pj
        return part

    with jax.named_scope("wait_x0"):
        for c in copies_0:
            c.wait()
    with jax.named_scope("ln0"):
        ln_tile(0, lambda v: v)
        ln_tile(1, lambda v: v)

    with jax.named_scope("wait_a"):
        for c in copies_a:
            c.wait()
    mixer1(0, 0, NA, first=True)

    with jax.named_scope("wait_b"):
        for c in copies_b:
            c.wait()
    tie = make_tie(0)
    part = mixer1(0, NA, NF, first=True)
    hold = make_hold(tie, [part], 2, 2 * NH, 0.0, 0.85)
    ln_tile(2, hold)
    ln_tile(3, hold)

    def p1_body(i, carry):
        with jax.named_scope("p1_wait"):
            for c in step_copies(i):
                c.wait()
        tie = make_tie(jnp.minimum(i, 1))
        part = mixer1(i)
        hold = make_hold(tie, [part], 2, P1_T * NH, 0.0, 0.9)
        for j in range(P1_T):
            ln_tile((i + 1) * P1_T + j, hold)
        return carry

    jax.lax.fori_loop(1, N1 - 1, p1_body, 0)

    with jax.named_scope("big_wait"):
        for c in [c_w1_last] + small:
            c.wait()
    tie = make_tie(0)
    part = mixer1(N1 - 1)

    def wt_transpose(j, hold):
        n = min(LANES, 3 * D - j * LANES)
        for c in range(4):
            r = min(LANES, D - c * LANES)
            blk = wqkv_v[pl.ds(c * LANES, r), pl.ds(j * LANES, n)]
            if n == LANES:
                blk = jnp.concatenate([_unpack(hold(_pack(blk[0:H]))), blk[H:]], axis=0)
            t32[c, pl.ds(j * LANES, n), pl.ds(0, r)] = blk.astype(F32).T

    def wt_gather(p):
        for d in range(DH):
            dst = (2 * d + p) * 8 if p < 2 else (2 * DH + d) * 8
            for c in range(4):
                r = min(LANES, D - c * LANES)
                v = t32[c, pl.ds(p * D + d, H, stride=DH), pl.ds(0, r)]
                wt_s[pl.ds(dst, 8), pl.ds(c * LANES, r)] = _pack(v)

    hold = make_hold(tie, [part], 2, 40, 0.0, 0.75)
    for j in range(7):
        wt_transpose(j, hold)
    wt_gather(0)
    wt_gather(1)
    for j in range(7, 11):
        wt_transpose(j, hold)
    wt_gather(2)

    def wo_prep(hold):
        for c in range(4):
            r = min(LANES, D - c * LANES)
            for g in range(4):
                blk = wo_v[pl.ds(g * 112, 112), pl.ds(c * LANES, r)].astype(F32)
                if r == LANES:
                    blk = jnp.concatenate([hold(blk[q * 8:q * 8 + 8]) for q in range(14)], axis=0)
                o32[c, pl.ds(g * 112, 112), pl.ds(0, r)] = blk
        for c in range(4):
            r = min(LANES, D - c * LANES)
            rows = jnp.concatenate(
                [o32[c, pl.ds(d, H, stride=DH), pl.ds(0, r)] for d in range(DH)], axis=0)
            wot_s[pl.ds(c * 64, r // 2), :] = _pack(rows.T)

    wo_prep(make_hold(tie, [part], 2, 3 * 56, 0.7, 1.0))

    lane = jax.lax.broadcasted_iota(jnp.int32, (H, LANES), 1)
    scale = DH ** -0.5

    def shift_back(prev, cur, a):
        return pltpu.roll(jnp.where(lane >= LANES - a, prev, cur), a, 1)

    def shift_fwd(cur, nxt, b):
        return pltpu.roll(jnp.where(lane < b, nxt, cur), LANES - b, 1)

    def tree(op, vs):
        while len(vs) > 1:
            vs = [op(vs[i], vs[i + 1]) for i in range(0, len(vs), 2)]
        return vs[0]

    hist = []

    def s1_tile(t, res, hold=None):
        tn = min(t + 1, NT - 1)
        tp = max(t - 1, 0)
        acc = [None] * WIN
        for d in range(DH):
            rq = pl.ds(2 * d * H, H)
            rk = pl.ds((2 * d + 1) * H, H)
            q0 = qk_s[t, rq, :]
            k0 = qk_s[t, rk, :]
            if hold is None:
                qn = res[2 * d * H:(2 * d + 1) * H, :]
                k0 = tie(k0, qn)
            else:
                qn = q0
                k0 = hold(k0)
                qn = tie(qn, k0)
            kp = qk_s[tp, rk, :]
            pre = [jnp.where(lane < 8, qn, q0)] + [jnp.where(lane >= LANES - a, kp, k0) for a in (2, 4, 6)]
            if len(hist) >= S1_LAG:
                pre = [tie(pre[i], hist[-S1_LAG][4 * (d % 2) + i]) for i in range(4)]
            q8 = pltpu.roll(pre[0], LANES - 8, 1)
            ks = [k0] + [pltpu.roll(pre[i], 2 * i, 1) for i in (1, 2, 3)]
            for a in range(4):
                t0 = q0 * ks[a]
                t8 = q8 * ks[a]
                acc[a] = t0 if d == 0 else acc[a] + t0
                acc[4 + a] = t8 if d == 0 else acc[4 + a] + t8
            hist.append(list(acc))
        for a in range(WIN):
            l_s[t, pl.ds(a * H, H), :] = acc[a]
        return tree(jnp.add, acc)

    def softmax_job(t, hh):
        tp = max(t - 1, 0)
        lane8 = lane[0:8]

        def rows(j):
            return pl.ds(j * H + hh * 8, 8)
        lg = [l_s[t, rows(j), :] for j in range(WIN)]
        for j in range(4, WIN):
            lg[j] = pltpu.roll(jnp.where(lane8 >= LANES - 8, l_s[tp, rows(j), :], lg[j]), 8, 1)
        if t == 0:
            lg = [lg[0]] + [jnp.where(lane8 >= DIL * j, lg[j], -1e9 / scale) for j in range(1, WIN)]
        m = tree(jnp.maximum, lg)
        e = [jnp.exp2((v - m) * (scale * LOG2E)) for v in lg]
        ssum = tree(jnp.add, e)
        inv = pl.reciprocal(ssum, approx=True)
        inv = inv * (2.0 - ssum * inv)
        for j in range(WIN):
            p_s[t, rows(j), :] = e[j] * inv

    def s2_tile(t, hold):
        tn = min(t + 1, NT - 1)
        tp = max(t - 1, 0)
        p0 = [p_s[t, pl.ds(a * H, H), :] for a in range(4)]
        p8 = [shift_fwd(p_s[t, pl.ds((4 + a) * H, H), :], p_s[tn, pl.ds((4 + a) * H, H), :], 8)
              for a in range(4)]
        for d in range(DH):
            r = pl.ds(d * H, H)
            v0 = hold(v_s[t, r, :])
            vp = v_s[tp, r, :]
            vs = [v0] + [shift_back(vp, v0, a) for a in (2, 4, 6)]
            o0 = (p0[0] * vs[0] + p0[1] * vs[1]) + (p0[2] * vs[2] + p0[3] * vs[3])
            o8 = (p8[0] * vs[0] + p8[1] * vs[1]) + (p8[2] * vs[2] + p8[3] * vs[3])
            o = o0 + shift_back(o8_s[r, :], o8, 8)
            o8_s[r, :] = o8
            o_s[t, r, :] = o.astype(BF16)

    def proj(dst, rows0, nrows, t, after=None):
        xn = xn_s[t]
        if after is not None:
            xn = jnp.concatenate([_unpack(tie(_pack(xn[0:2 * H]), after)), xn[2 * H:]], axis=0)
        res = _dot(_unpack(wt_s[pl.ds(rows0 // 2, nrows // 2), :]), xn)
        dst[t] = res
        return res

    b1 = b1_v[...].astype(F32).reshape(1, F)
    GR = 32
    gelu_jobs = [(j, rr) for j in range(NF) for rr in range(D // GR)]

    def gelu_job(j, rr, hold):
        bias = hold(jnp.broadcast_to(b1[:, j * LANES:(j + 1) * LANES], (8, LANES)))
        bias = jnp.concatenate([bias, bias], axis=0)
        for q in range(GR // H):
            row = rr * GR + q * H
            g_s[j, pl.ds(row, H), :] = _gelu(u_s[j, pl.ds(row, H), :] + bias).astype(BF16)

    def spread_gelu(res, njobs, lo=0.0, hi=1.0):
        njobs = min(njobs, len(gelu_jobs))
        hold = make_hold(tie, res, 1, njobs, lo, hi)
        for _ in range(njobs):
            gelu_job(*gelu_jobs.pop(0), hold)

    for half in range(2):
        ts = range(half * NT // 2, (half + 1) * NT // 2)
        fin = []
        for t in ts:
            res = proj(qk_s, 0, 2 * D, t, fin.pop(0) if len(fin) >= 2 else None)
            if t == 0:
                spread_gelu([res], 20)
            else:
                fin.append(s1_tile(t - 1, res))
                if half == 0:
                    fin.pop()
        vres = []
        for t in ts:
            k = t - ts[0]
            vres.append(proj(v_s, 2 * D, D, t, fin.pop(0) if fin and k in (0, 2, 5) else None))
            if half == 1 and k == 1:
                fin.append(s1_tile(NT - 1, None, make_hold(tie, vres, 1, DH)))
        if half == 0:
            spread_gelu(vres, 96, 0.07, 0.95)
        else:
            spread_gelu(vres[:2], 8)
            spread_gelu(vres[2:], 72)
        if half == 0:
            with jax.named_scope("w2_wait"):
                c_w2.wait()

            @pl.when(z_s[0, 0, 0] != 0.0)
            def _():
                o8_s[...] = jnp.zeros_like(o8_s)

            tie = make_tie(0)
            hist.clear()
    assert not gelu_jobs
    for t in range(NT):
        softmax_job(t, 0)
        softmax_job(t, 1)

    n3 = NT // P3_T
    c3 = P3_T * LANES

    def out_copy(t):
        return pltpu.make_async_copy(out_v.at[t], out_hbm.at[:, pl.ds(t * LANES, LANES)],
                                     sems.at[SEM_OUT])

    b2 = b2_v[...].astype(F32).reshape(1, S)
    ksplit = ((0, 4), (4, 8), (8, 12), (12, 14))
    gs = [tiles(g_s, k0, k1 - k0) for k0, k1 in ksplit]
    for i in range(n3):
        ys = []
        for g, (k0, k1) in zip(gs, ksplit):
            y = _dot(g,
                     w2_v[pl.ds(k0 * LANES, (k1 - k0) * LANES), pl.ds(i * c3, c3)])
            ys.append(y + ys[-1] if ys else y)
        hold = make_hold(tie, ys[:3], 1, P3_T * DH, 0.0, 0.9)
        for j in range(P3_T):
            s2_tile(i * P3_T + j, hold)
        y = _dot(_unpack(wot_s[...]), tiles(o_s, i * P3_T, P3_T)) + ys[-1]
        for j in range(P3_T):
            t = i * P3_T + j
            bias = jnp.broadcast_to(b2[:, t * LANES:(t + 1) * LANES], (H, LANES))
            for d in range(DH):
                r = pl.ds(d * H, H)
                val = x_v[t, r, :].astype(F32) + (y[d * H:(d + 1) * H, j * LANES:(j + 1) * LANES] + bias)
                out_v[t, r, :] = val.astype(BF16)
            out_copy(t).start()

    with jax.named_scope("out_wait"):
        for t in range(NT):
            out_copy(t).wait()


@jax.jit
def pallas_parallel_sum__sliding_local_dilated__mixer_token_mlp__prompt_kernel(
    A_x: jax.Array,
    A_wqkv: jax.Array,
    A_wo: jax.Array,
    B_x: jax.Array,
    B_w1: jax.Array,
    B_b1: jax.Array,
    B_w2: jax.Array,
    B_b2: jax.Array,
):
    del B_x
    xt = jnp.transpose(A_x[0], (1, 0))
    any_spec = pl.BlockSpec(memory_space=pl.ANY)
    out_t = pl.pallas_call(
        _kernel,
        out_shape=jax.ShapeDtypeStruct((D, S), BF16),
        in_specs=[any_spec] * 7,
        out_specs=any_spec,
        scratch_shapes=[
            pltpu.VMEM((NT, D, LANES), BF16),
            pltpu.VMEM((S, F), BF16),
            pltpu.VMEM((F, S + LANES), BF16),
            pltpu.VMEM((D, 3 * D), BF16),
            pltpu.VMEM((D, D), BF16),
            pltpu.VMEM((F,), BF16),
            pltpu.VMEM((S,), BF16),
            pltpu.VMEM((NT, D, LANES), BF16),
            pltpu.VMEM((NT, D, LANES), BF16),
            pltpu.VMEM((NF, D, LANES), F32),
            pltpu.VMEM((NF, D, LANES), BF16),
            pltpu.VMEM((3 * D // 2, D), U32),
            pltpu.VMEM((D // 2, D), U32),
            pltpu.VMEM((4, 3 * D + 32, LANES), F32),
            pltpu.VMEM((4, D + 32, LANES), F32),
            pltpu.VMEM((NT, 2 * D, LANES), F32),
            pltpu.VMEM((NT, D, LANES), F32),
            pltpu.VMEM((NT, WIN * H, LANES), F32),
            pltpu.VMEM((NT, WIN * H, LANES), F32),
            pltpu.VMEM((D, LANES), F32),
            pltpu.VMEM((NT, D, LANES), BF16),
            pltpu.VMEM((NT, D, LANES), BF16),
            pltpu.VMEM((2, 8, LANES), F32),
            pltpu.SemaphoreType.DMA((N1 + 4,)),
        ],
        compiler_params=pltpu.CompilerParams(vmem_limit_bytes=100 * 1024 * 1024,
                                             disable_bounds_checks=True,
                                             disable_semaphore_checks=True),
    )(xt, A_wqkv, A_wo, B_w1, B_b1, B_w2, B_b2)
    return jnp.transpose(out_t, (1, 0))[None]
```

```python
import jax
import jax.numpy as jnp
import jax.experimental.pallas as pl
import jax.experimental.pallas.tpu as pltpu

S = 2048
D = 448
F = 1792
H = 16
DH = D // H
WIN = 8
DIL = 2
EPS = 1e-5
LOG2E = 1.4426950408889634
LANES = 128
NT = S // LANES
NF = F // LANES
F32 = jnp.float32
BF16 = jnp.bfloat16
U32 = jnp.uint32

P1_T = 2
P3_T = 2
N1 = NT // P1_T
OUT_SPLIT = [224, 384, D]
S1_LAG = 6
NA = 6


def _dot(a, b):
    return jnp.dot(a, b, preferred_element_type=F32)


def _gelu(x):
    c = 0.7978845608028654
    inner = x * (c + (c * 0.044715) * (x * x))
    hx = 0.5 * x
    return hx + hx * jnp.tanh(inner)


def _pack(v):
    return pltpu.bitcast(v.astype(BF16), U32)


def _unpack(v):
    return pltpu.bitcast(v, BF16)


def _kernel(x_hbm, wqkv_hbm, wo_hbm, w1_hbm, b1_hbm, w2_hbm, b2_hbm, out_hbm,
            x_v, w1_v, w2_v, wqkv_v, wo_v, b1_v, b2_v,
            xn_s, h_s, u_s, g_s, wt_s, wot_s, t32, o32, qk_s, v_s, l_s, p_s, o8_s, o_s, out_v, z_s,
            sems):
    c1 = P1_T * LANES
    SEM_LAST, SEM_W2, SEM_OUT = N1 + 1, N1 + 2, N1 + 3

    def x_copy(t, sem):
        col = t * LANES if isinstance(t, int) else pl.multiple_of(t * LANES, LANES)
        return pltpu.make_async_copy(x_hbm.at[:, pl.ds(col, LANES)], x_v.at[t], sems.at[sem])

    def w1_copy(row, sem, col=0, ncol=F):
        return pltpu.make_async_copy(w1_hbm.at[pl.ds(row, c1), pl.ds(col, ncol)],
                                     w1_v.at[pl.ds(row, c1), pl.ds(col, ncol)], sems.at[sem])

    def step_copies(i):
        row = i * c1 if isinstance(i, int) else pl.multiple_of(i * c1, c1)
        return [w1_copy(row, 2 + i)] + [x_copy((i + 1) * P1_T + j, 2 + i) for j in range(P1_T)]

    copies_0 = [x_copy(0, 0), x_copy(1, 0)]
    copies_a = [w1_copy(0, 1, 0, NA * LANES)]
    copies_b = [w1_copy(0, 2, NA * LANES, F - NA * LANES), x_copy(2, 2), x_copy(3, 2)]
    c_w1_last = w1_copy((N1 - 1) * c1, SEM_LAST)
    small = [pltpu.make_async_copy(src, dst, sems.at[SEM_LAST])
             for src, dst in ((wqkv_hbm, wqkv_v), (wo_hbm, wo_v), (b1_hbm, b1_v), (b2_hbm, b2_v))]
    c_w2 = pltpu.make_async_copy(w2_hbm, w2_v.at[:, pl.ds(0, S)], sems.at[SEM_W2])

    for c in copies_0 + copies_a + copies_b:
        c.start()
    for i in range(1, N1 - 1):
        for c in step_copies(i):
            c.start()
    c_w1_last.start()
    for c in small + [c_w2]:
        c.start(priority=1)

    z_s[...] = jnp.zeros_like(z_s)
    o8_s[...] = jnp.zeros_like(o8_s)

    def make_tie(zi):
        never8 = z_s[zi] != 0.0
        never16 = jnp.concatenate([z_s[zi], z_s[zi]], axis=0) != 0.0

        def tie(val, src):
            if val.dtype != src.dtype:
                src = pltpu.bitcast(src, val.dtype)
            if val.shape[0] == 16 and src.shape[0] == 8:
                src = jnp.concatenate([src, src], axis=0)
            return jax.lax.select(never8 if val.shape[0] == 8 else never16, src, val)
        return tie

    def make_hold(tie, results, ntile_par, n, lo=0.0, hi=1.0):
        pts = []
        for res in results:
            for c in range(0, res.shape[1] // LANES, ntile_par):
                pts += [(res, r, c * LANES) for r in range(0, res.shape[0], 8)]
        state = [0]

        def hold(v):
            k = state[0]
            state[0] += 1
            assert k < n
            res, row, col = pts[min(int((lo + (hi - lo) * k / n) * len(pts)), len(pts) - 1)]
            return tie(v, res[row:row + 8, col:col + LANES])
        return hold

    LG = 7
    NH = 6 * (DH // LG)

    def ln_pass(ld, dst, t, hold):
        def colmean(f, c):
            acc = None
            for g in range(DH // LG):
                cg = hold(c)
                cg = jnp.concatenate([cg, cg], axis=0)
                part = None
                for d in range(g * LG, (g + 1) * LG):
                    v = f(ld(d), cg, d == g * LG)
                    part = v if part is None else part + v
                acc = part if acc is None else acc + part
            m = jnp.sum(acc, axis=0, keepdims=True) * (1.0 / D)
            return jnp.broadcast_to(m, (8, LANES))

        def sq(v, m, first):
            c = v - m
            return c * c
        m = colmean(lambda v, c, first: v + c if first else v, jnp.zeros((8, LANES), F32))
        r = jax.lax.rsqrt(colmean(sq, m) + EPS)
        r = jnp.concatenate([r, r], axis=0)
        for g in range(DH // LG):
            mg = hold(m)
            mg = jnp.concatenate([mg, mg], axis=0)
            for d in range(g * LG, (g + 1) * LG):
                dst[t, pl.ds(d * H, H), :] = ((ld(d) - mg) * r).astype(BF16)

    def ln_tile(t, hold):
        ln_pass(lambda d: x_v[t, pl.ds(d * H, H), :].astype(F32), xn_s, t, hold)
        ln_pass(lambda d: xn_s[t, pl.ds(d * H, H), :].astype(F32), h_s, t, hold)

    def tiles(ref, t0, nt):
        return jnp.concatenate([ref[t0 + j] for j in range(nt)], axis=1)

    def mixer1(i, j0=0, j1=NF, first=False):
        row = i * c1 if isinstance(i, int) else pl.multiple_of(i * c1, c1)
        part = _dot(tiles(h_s, i * P1_T, P1_T), w1_v[pl.ds(row, c1), pl.ds(j0 * LANES, (j1 - j0) * LANES)])
        for j in range(j0, j1):
            pj = part[:, (j - j0) * LANES:(j - j0 + 1) * LANES]
            if first:
                u_s[j] = pj
            else:
                u_s[j] += pj
        return part

    with jax.named_scope("wait_x0"):
        for c in copies_0:
            c.wait()
    with jax.named_scope("ln0"):
        ln_tile(0, lambda v: v)
        ln_tile(1, lambda v: v)

    with jax.named_scope("wait_a"):
        for c in copies_a:
            c.wait()
    mixer1(0, 0, NA, first=True)

    with jax.named_scope("wait_b"):
        for c in copies_b:
            c.wait()
    tie = make_tie(0)
    part = mixer1(0, NA, NF, first=True)
    hold = make_hold(tie, [part], 2, 2 * NH, 0.0, 0.85)
    ln_tile(2, hold)
    ln_tile(3, hold)

    def p1_body(i, carry):
        with jax.named_scope("p1_wait"):
            for c in step_copies(i):
                c.wait()
        tie = make_tie(jnp.minimum(i, 1))
        part = mixer1(i)
        hold = make_hold(tie, [part], 2, P1_T * NH, 0.0, 0.9)
        for j in range(P1_T):
            ln_tile((i + 1) * P1_T + j, hold)
        return carry

    jax.lax.fori_loop(1, N1 - 1, p1_body, 0)

    with jax.named_scope("big_wait"):
        for c in [c_w1_last] + small:
            c.wait()
    tie = make_tie(0)
    part = mixer1(N1 - 1)

    def wt_transpose(j, hold):
        n = min(LANES, 3 * D - j * LANES)
        for c in range(4):
            r = min(LANES, D - c * LANES)
            blk = wqkv_v[pl.ds(c * LANES, r), pl.ds(j * LANES, n)]
            if n == LANES:
                blk = jnp.concatenate([_unpack(hold(_pack(blk[0:H]))), blk[H:]], axis=0)
            t32[c, pl.ds(j * LANES, n), pl.ds(0, r)] = blk.astype(F32).T

    def wt_gather(p):
        for d in range(DH):
            dst = (2 * d + p) * 8 if p < 2 else (2 * DH + d) * 8
            for c in range(4):
                r = min(LANES, D - c * LANES)
                v = t32[c, pl.ds(p * D + d, H, stride=DH), pl.ds(0, r)]
                wt_s[pl.ds(dst, 8), pl.ds(c * LANES, r)] = _pack(v)

    hold = make_hold(tie, [part], 2, 40, 0.0, 0.75)
    for j in range(7):
        wt_transpose(j, hold)
    wt_gather(0)
    wt_gather(1)
    for j in range(7, 11):
        wt_transpose(j, hold)
    wt_gather(2)

    def wo_prep(hold):
        for c in range(4):
            r = min(LANES, D - c * LANES)
            for g in range(4):
                blk = wo_v[pl.ds(g * 112, 112), pl.ds(c * LANES, r)].astype(F32)
                if r == LANES:
                    blk = jnp.concatenate([hold(blk[q * 8:q * 8 + 8]) for q in range(14)], axis=0)
                o32[c, pl.ds(g * 112, 112), pl.ds(0, r)] = blk
        for c in range(4):
            r = min(LANES, D - c * LANES)
            rows = jnp.concatenate(
                [o32[c, pl.ds(d, H, stride=DH), pl.ds(0, r)] for d in range(DH)], axis=0)
            wot_s[pl.ds(c * 64, r // 2), :] = _pack(rows.T)

    wo_prep(make_hold(tie, [part], 2, 3 * 56, 0.7, 1.0))

    lane = jax.lax.broadcasted_iota(jnp.int32, (H, LANES), 1)
    scale = DH ** -0.5

    top = {a: lane >= LANES - a for a in (2, 4, 6, 8)}
    low8 = lane < 8

    def shift_back(prev, cur, a):
        return pltpu.roll(jax.lax.select(top[a], prev, cur), a, 1)

    def shift_fwd8(cur, nxt):
        return pltpu.roll(jax.lax.select(low8, nxt, cur), LANES - 8, 1)

    def tree(op, vs):
        while len(vs) > 1:
            vs = [op(vs[i], vs[i + 1]) for i in range(0, len(vs), 2)]
        return vs[0]

    hist = []

    def s1_tile(t, res, hold=None):
        tn = min(t + 1, NT - 1)
        tp = max(t - 1, 0)
        acc = [None] * WIN
        for d in range(DH):
            rq = pl.ds(2 * d * H, H)
            rk = pl.ds((2 * d + 1) * H, H)
            q0 = qk_s[t, rq, :]
            k0 = qk_s[t, rk, :]
            if hold is None:
                qn = res[2 * d * H:(2 * d + 1) * H, :]
                k0 = tie(k0, qn)
            else:
                qn = q0
                k0 = hold(k0)
                qn = tie(qn, k0)
            kp = qk_s[tp, rk, :]
            pre = [jax.lax.select(low8, qn, q0)] + [jax.lax.select(top[a], kp, k0) for a in (2, 4, 6)]
            if len(hist) >= S1_LAG:
                pre = [tie(pre[i], hist[-S1_LAG][4 * (d % 2) + i]) for i in range(4)]
            q8 = pltpu.roll(pre[0], LANES - 8, 1)
            ks = [k0] + [pltpu.roll(pre[i], 2 * i, 1) for i in (1, 2, 3)]
            for a in range(4):
                t0 = q0 * ks[a]
                t8 = q8 * ks[a]
                acc[a] = t0 if d == 0 else acc[a] + t0
                acc[4 + a] = t8 if d == 0 else acc[4 + a] + t8
            hist.append(list(acc))
        for a in range(WIN):
            l_s[t, pl.ds(a * H, H), :] = acc[a]
        return tree(jnp.add, acc)

    def softmax_job(t, hh):
        tp = max(t - 1, 0)
        lane8 = lane[0:8]

        def rows(j):
            return pl.ds(j * H + hh * 8, 8)
        lg = [l_s[t, rows(j), :] for j in range(WIN)]
        for j in range(4, WIN):
            lg[j] = pltpu.roll(jnp.where(lane8 >= LANES - 8, l_s[tp, rows(j), :], lg[j]), 8, 1)
        if t == 0:
            lg = [lg[0]] + [jnp.where(lane8 >= DIL * j, lg[j], -1e9 / scale) for j in range(1, WIN)]
        m = tree(jnp.maximum, lg)
        e = [jnp.exp2((v - m) * (scale * LOG2E)) for v in lg]
        ssum = tree(jnp.add, e)
        inv = pl.reciprocal(ssum, approx=True)
        inv = inv * (2.0 - ssum * inv)
        for j in range(WIN):
            p_s[t, rows(j), :] = e[j] * inv

    def s2_tile(t, hold):
        tn = min(t + 1, NT - 1)
        tp = max(t - 1, 0)
        p0 = [p_s[t, pl.ds(a * H, H), :] for a in range(4)]
        p8 = [shift_fwd8(p_s[t, pl.ds((4 + a) * H, H), :], p_s[tn, pl.ds((4 + a) * H, H), :])
              for a in range(4)]
        for d in range(DH):
            r = pl.ds(d * H, H)
            v0 = hold(v_s[t, r, :])
            vp = v_s[tp, r, :]
            vs = [v0] + [shift_back(vp, v0, a) for a in (2, 4, 6)]
            o0 = (p0[0] * vs[0] + p0[1] * vs[1]) + (p0[2] * vs[2] + p0[3] * vs[3])
            o8 = (p8[0] * vs[0] + p8[1] * vs[1]) + (p8[2] * vs[2] + p8[3] * vs[3])
            o = o0 + shift_back(o8_s[r, :], o8, 8)
            o8_s[r, :] = o8
            o_s[t, r, :] = o.astype(BF16)

    def proj(dst, rows0, nrows, t, after=None):
        xn = xn_s[t]
        if after is not None:
            xn = jnp.concatenate([_unpack(tie(_pack(xn[0:2 * H]), after)), xn[2 * H:]], axis=0)
        res = _dot(_unpack(wt_s[pl.ds(rows0 // 2, nrows // 2), :]), xn)
        dst[t] = res
        return res

    b1 = b1_v[...].astype(F32).reshape(1, F)
    GR = 32
    gelu_jobs = [(j, rr) for j in range(NF) for rr in range(D // GR)]

    def gelu_job(j, rr, hold):
        bias = hold(jnp.broadcast_to(b1[:, j * LANES:(j + 1) * LANES], (8, LANES)))
        bias = jnp.concatenate([bias, bias], axis=0)
        for q in range(GR // H):
            row = rr * GR + q * H
            g_s[j, pl.ds(row, H), :] = _gelu(u_s[j, pl.ds(row, H), :] + bias).astype(BF16)

    def spread_gelu(res, njobs, lo=0.0, hi=1.0):
        njobs = min(njobs, len(gelu_jobs))
        hold = make_hold(tie, res, 1, njobs, lo, hi)
        for _ in range(njobs):
            gelu_job(*gelu_jobs.pop(0), hold)

    for half in range(2):
        ts = range(half * NT // 2, (half + 1) * NT // 2)
        fin = []
        for t in ts:
            res = proj(qk_s, 0, 2 * D, t, fin.pop(0) if len(fin) >= 2 else None)
            if t == 0:
                spread_gelu([res], 20)
            else:
                fin.append(s1_tile(t - 1, res))
                if half == 0:
                    fin.pop()
        vres = []
        for t in ts:
            k = t - ts[0]
            vres.append(proj(v_s, 2 * D, D, t, fin.pop(0) if fin and k in (0, 2, 5) else None))
            if half == 1 and k == 1:
                fin.append(s1_tile(NT - 1, None, make_hold(tie, vres, 1, DH)))
        if half == 0:
            spread_gelu(vres, 96, 0.07, 0.95)
        else:
            spread_gelu(vres[:2], 8)
            spread_gelu(vres[2:], 72)
        if half == 0:
            with jax.named_scope("w2_wait"):
                c_w2.wait()

            @pl.when(z_s[0, 0, 0] != 0.0)
            def _():
                o8_s[...] = jnp.zeros_like(o8_s)

            tie = make_tie(0)
            hist.clear()
    assert not gelu_jobs
    for t in range(NT):
        softmax_job(t, 0)
        softmax_job(t, 1)

    n3 = NT // P3_T
    c3 = P3_T * LANES

    out_copies = []

    def out_copy(t, r0, nr):
        c = pltpu.make_async_copy(out_v.at[t, pl.ds(r0, nr), :],
                                  out_hbm.at[pl.ds(r0, nr), pl.ds(t * LANES, LANES)], sems.at[SEM_OUT])
        c.start()
        out_copies.append(c)

    b2 = b2_v[...].astype(F32).reshape(1, S)
    ksplit = ((0, 4), (4, 8), (8, 12), (12, 14))
    gs = [tiles(g_s, k0, k1 - k0) for k0, k1 in ksplit]
    for i in range(n3):
        ys = []
        for g, (k0, k1) in zip(gs, ksplit):
            y = _dot(g,
                     w2_v[pl.ds(k0 * LANES, (k1 - k0) * LANES), pl.ds(i * c3, c3)])
            ys.append(y + ys[-1] if ys else y)
        hold = make_hold(tie, ys[:3], 1, P3_T * DH, 0.0, 0.9)
        for j in range(P3_T):
            s2_tile(i * P3_T + j, hold)
        y = _dot(_unpack(wot_s[...]), tiles(o_s, i * P3_T, P3_T)) + ys[-1]
        for j in range(P3_T):
            t = i * P3_T + j
            bias = jnp.broadcast_to(b2[:, t * LANES:(t + 1) * LANES], (H, LANES))
            for d in range(DH):
                r = pl.ds(d * H, H)
                val = x_v[t, r, :].astype(F32) + (y[d * H:(d + 1) * H, j * LANES:(j + 1) * LANES] + bias)
                out_v[t, r, :] = val.astype(BF16)
                if t == NT - 1 and (d + 1) * H in OUT_SPLIT:
                    r0 = ([0] + OUT_SPLIT)[OUT_SPLIT.index((d + 1) * H)]
                    out_copy(t, r0, (d + 1) * H - r0)
            if t < NT - 1:
                out_copy(t, 0, D)

    with jax.named_scope("out_wait"):
        for c in out_copies:
            c.wait()


@jax.jit
def pallas_parallel_sum__sliding_local_dilated__mixer_token_mlp__prompt_kernel(
    A_x: jax.Array,
    A_wqkv: jax.Array,
    A_wo: jax.Array,
    B_x: jax.Array,
    B_w1: jax.Array,
    B_b1: jax.Array,
    B_w2: jax.Array,
    B_b2: jax.Array,
):
    del B_x
    xt = jnp.transpose(A_x[0], (1, 0))
    any_spec = pl.BlockSpec(memory_space=pl.ANY)
    out_t = pl.pallas_call(
        _kernel,
        out_shape=jax.ShapeDtypeStruct((D, S), BF16),
        in_specs=[any_spec] * 7,
        out_specs=any_spec,
        scratch_shapes=[
            pltpu.VMEM((NT, D, LANES), BF16),
            pltpu.VMEM((S, F), BF16),
            pltpu.VMEM((F, S + LANES), BF16),
            pltpu.VMEM((D, 3 * D), BF16),
            pltpu.VMEM((D, D), BF16),
            pltpu.VMEM((F,), BF16),
            pltpu.VMEM((S,), BF16),
            pltpu.VMEM((NT, D, LANES), BF16),
            pltpu.VMEM((NT, D, LANES), BF16),
            pltpu.VMEM((NF, D, LANES), F32),
            pltpu.VMEM((NF, D, LANES), BF16),
            pltpu.VMEM((3 * D // 2, D), U32),
            pltpu.VMEM((D // 2, D), U32),
            pltpu.VMEM((4, 3 * D + 32, LANES), F32),
            pltpu.VMEM((4, D + 32, LANES), F32),
            pltpu.VMEM((NT, 2 * D, LANES), F32),
            pltpu.VMEM((NT, D, LANES), F32),
            pltpu.VMEM((NT, WIN * H, LANES), F32),
            pltpu.VMEM((NT, WIN * H, LANES), F32),
            pltpu.VMEM((D, LANES), F32),
            pltpu.VMEM((NT, D, LANES), BF16),
            pltpu.VMEM((NT, D, LANES), BF16),
            pltpu.VMEM((2, 8, LANES), F32),
            pltpu.SemaphoreType.DMA((N1 + 4,)),
        ],
        compiler_params=pltpu.CompilerParams(vmem_limit_bytes=100 * 1024 * 1024,
                                             disable_bounds_checks=True,
                                             disable_semaphore_checks=True),
    )(xt, A_wqkv, A_wo, B_w1, B_b1, B_w2, B_b2)
    return jnp.transpose(out_t, (1, 0))[None]
```

```python
import jax
import jax.numpy as jnp
import jax.experimental.pallas as pl
import jax.experimental.pallas.tpu as pltpu

S = 2048
D = 448
F = 1792
H = 16
DH = D // H
WIN = 8
DIL = 2
EPS = 1e-5
LOG2E = 1.4426950408889634
LANES = 128
NT = S // LANES
NF = F // LANES
F32 = jnp.float32
BF16 = jnp.bfloat16
U32 = jnp.uint32

P1_T = 2
P3_T = 2
N1 = NT // P1_T
V_EARLY = 5
OUT_SPLIT = [224, 384, D]
S1_LAG = 6
NA = 6


def _dot(a, b):
    return jnp.dot(a, b, preferred_element_type=F32)


def _gelu(x):
    c = 0.7978845608028654
    inner = x * (c + (c * 0.044715) * (x * x))
    hx = 0.5 * x
    return hx + hx * jnp.tanh(inner)


def _pack(v):
    return pltpu.bitcast(v.astype(BF16), U32)


def _unpack(v):
    return pltpu.bitcast(v, BF16)


def _kernel(x_hbm, wqkv_hbm, wo_hbm, w1_hbm, b1_hbm, w2_hbm, b2_hbm, out_hbm,
            x_v, w1_v, w2_v, wqkv_v, wo_v, b1_v, b2_v,
            xn_s, h_s, u_s, g_s, wt_s, wot_s, t32, o32, qk_s, v_s, l_s, p_s, o8_s, o_s, out_v, z_s,
            sems):
    c1 = P1_T * LANES
    SEM_LAST, SEM_W2, SEM_OUT = N1 + 1, N1 + 2, N1 + 3

    def x_copy(t, sem):
        col = t * LANES if isinstance(t, int) else pl.multiple_of(t * LANES, LANES)
        return pltpu.make_async_copy(x_hbm.at[:, pl.ds(col, LANES)], x_v.at[t], sems.at[sem])

    def w1_copy(row, sem, col=0, ncol=F):
        return pltpu.make_async_copy(w1_hbm.at[pl.ds(row, c1), pl.ds(col, ncol)],
                                     w1_v.at[pl.ds(row, c1), pl.ds(col, ncol)], sems.at[sem])

    def step_copies(i):
        row = i * c1 if isinstance(i, int) else pl.multiple_of(i * c1, c1)
        return [x_copy((i + 1) * P1_T + j, 2 + i) for j in range(P1_T)] + [w1_copy(row, 2 + i)]

    copies_0 = [x_copy(0, 0), x_copy(1, 0)]
    copies_a = [w1_copy(0, 1, 0, NA * LANES)]
    copies_b = [x_copy(2, 2), x_copy(3, 2), w1_copy(0, 2, NA * LANES, F - NA * LANES)]
    c_w1_last = w1_copy((N1 - 1) * c1, SEM_LAST)
    small = [pltpu.make_async_copy(src, dst, sems.at[SEM_LAST])
             for src, dst in ((wqkv_hbm, wqkv_v), (wo_hbm, wo_v), (b1_hbm, b1_v), (b2_hbm, b2_v))]
    c_w2 = pltpu.make_async_copy(w2_hbm, w2_v.at[:, pl.ds(0, S)], sems.at[SEM_W2])

    for c in copies_0 + copies_a + copies_b:
        c.start()
    for i in range(1, N1 - 1):
        for c in step_copies(i):
            c.start()
    c_w1_last.start()
    for c in small + [c_w2]:
        c.start(priority=1)

    z_s[...] = jnp.zeros_like(z_s)
    o8_s[...] = jnp.zeros_like(o8_s)

    def make_tie(zi):
        never8 = z_s[zi] != 0.0
        never16 = jnp.concatenate([z_s[zi], z_s[zi]], axis=0) != 0.0

        def tie(val, src):
            if val.dtype != src.dtype:
                src = pltpu.bitcast(src, val.dtype)
            if val.shape[0] == 16 and src.shape[0] == 8:
                src = jnp.concatenate([src, src], axis=0)
            return jax.lax.select(never8 if val.shape[0] == 8 else never16, src, val)
        return tie

    def make_hold(tie, results, ntile_par, n, lo=0.0, hi=1.0):
        pts = []
        for res in results:
            for c in range(0, res.shape[1] // LANES, ntile_par):
                pts += [(res, r, c * LANES) for r in range(0, res.shape[0], 8)]
        state = [0]

        def hold(v):
            k = state[0]
            state[0] += 1
            assert k < n
            res, row, col = pts[min(int((lo + (hi - lo) * k / n) * len(pts)), len(pts) - 1)]
            return tie(v, res[row:row + 8, col:col + LANES])
        return hold

    LG = 7
    NH = 6 * (DH // LG)

    def ln_pass(ld, dst, t, hold):
        def colmean(f, c):
            acc = None
            for g in range(DH // LG):
                cg = hold(c)
                cg = jnp.concatenate([cg, cg], axis=0)
                part = None
                for d in range(g * LG, (g + 1) * LG):
                    v = f(ld(d), cg, d == g * LG)
                    part = v if part is None else part + v
                acc = part if acc is None else acc + part
            m = jnp.sum(acc, axis=0, keepdims=True) * (1.0 / D)
            return jnp.broadcast_to(m, (8, LANES))

        def sq(v, m, first):
            c = v - m
            return c * c
        m = colmean(lambda v, c, first: v + c if first else v, jnp.zeros((8, LANES), F32))
        r = jax.lax.rsqrt(colmean(sq, m) + EPS)
        r = jnp.concatenate([r, r], axis=0)
        for g in range(DH // LG):
            mg = hold(m)
            mg = jnp.concatenate([mg, mg], axis=0)
            for d in range(g * LG, (g + 1) * LG):
                dst[t, pl.ds(d * H, H), :] = ((ld(d) - mg) * r).astype(BF16)

    def ln_tile(t, hold):
        ln_pass(lambda d: x_v[t, pl.ds(d * H, H), :].astype(F32), xn_s, t, hold)
        ln_pass(lambda d: xn_s[t, pl.ds(d * H, H), :].astype(F32), h_s, t, hold)

    def tiles(ref, t0, nt):
        return jnp.concatenate([ref[t0 + j] for j in range(nt)], axis=1)

    def mixer1(i, j0=0, j1=NF, first=False):
        row = i * c1 if isinstance(i, int) else pl.multiple_of(i * c1, c1)
        part = _dot(tiles(h_s, i * P1_T, P1_T), w1_v[pl.ds(row, c1), pl.ds(j0 * LANES, (j1 - j0) * LANES)])
        for j in range(j0, j1):
            pj = part[:, (j - j0) * LANES:(j - j0 + 1) * LANES]
            if first:
                u_s[j] = pj
            else:
                u_s[j] += pj
        return part

    with jax.named_scope("wait_x0"):
        for c in copies_0:
            c.wait()
    never_scalar = z_s[0, 0, 0] != 0.0
    with jax.named_scope("ln0"):
        ln_tile(0, lambda v: v)
        ln_tile(1, lambda v: v)

    with jax.named_scope("wait_a"):
        for c in copies_a:
            c.wait()
    mixer1(0, 0, NA, first=True)

    with jax.named_scope("wait_b"):
        for c in copies_b:
            c.wait()
    tie = make_tie(0)
    part = mixer1(0, NA, NF, first=True)
    hold = make_hold(tie, [part], 2, 2 * NH, 0.0, 0.85)
    ln_tile(2, hold)
    ln_tile(3, hold)

    def p1_body(i, carry):
        with jax.named_scope("p1_wait"):
            for c in step_copies(i):
                c.wait()
        tie = make_tie(jnp.minimum(i, 1))
        part = mixer1(i)
        hold = make_hold(tie, [part], 2, P1_T * NH, 0.0, 0.9)
        for j in range(P1_T):
            ln_tile((i + 1) * P1_T + j, hold)
        return carry

    jax.lax.fori_loop(1, N1 - 2, p1_body, 0)

    with jax.named_scope("big_wait"):
        for c in step_copies(N1 - 2) + [c_w1_last] + small:
            c.wait()
    tie = make_tie(0)
    part = mixer1(N1 - 2)
    hold = make_hold(tie, [part], 2, P1_T * NH, 0.0, 0.8)
    for j in range(P1_T):
        ln_tile((N1 - 1) * P1_T + j, hold)
    part = mixer1(N1 - 1)

    def wt_transpose(j, hold):
        n = min(LANES, 3 * D - j * LANES)
        for c in range(4):
            r = min(LANES, D - c * LANES)
            blk = wqkv_v[pl.ds(c * LANES, r), pl.ds(j * LANES, n)]
            if n == LANES:
                blk = jnp.concatenate([_unpack(hold(_pack(blk[0:H]))), blk[H:]], axis=0)
            t32[c, pl.ds(j * LANES, n), pl.ds(0, r)] = blk.astype(F32).T

    def wt_gather(p):
        for d in range(DH):
            dst = (2 * d + p) * 8 if p < 2 else (2 * DH + d) * 8
            for c in range(4):
                r = min(LANES, D - c * LANES)
                v = t32[c, pl.ds(p * D + d, H, stride=DH), pl.ds(0, r)]
                wt_s[pl.ds(dst, 8), pl.ds(c * LANES, r)] = _pack(v)

    hold = make_hold(tie, [part], 2, 40, 0.0, 0.75)
    for j in range(7):
        wt_transpose(j, hold)
    wt_gather(0)
    wt_gather(1)
    for j in range(7, 11):
        wt_transpose(j, hold)
    wt_gather(2)

    def wo_prep(hold):
        for c in range(4):
            r = min(LANES, D - c * LANES)
            for g in range(4):
                blk = wo_v[pl.ds(g * 112, 112), pl.ds(c * LANES, r)].astype(F32)
                if r == LANES:
                    blk = jnp.concatenate([hold(blk[q * 8:q * 8 + 8]) for q in range(14)], axis=0)
                o32[c, pl.ds(g * 112, 112), pl.ds(0, r)] = blk
        for c in range(4):
            r = min(LANES, D - c * LANES)
            rows = jnp.concatenate(
                [o32[c, pl.ds(d, H, stride=DH), pl.ds(0, r)] for d in range(DH)], axis=0)
            wot_s[pl.ds(c * 64, r // 2), :] = _pack(rows.T)

    wo_prep(make_hold(tie, [part], 2, 3 * 56, 0.7, 1.0))

    lane = jax.lax.broadcasted_iota(jnp.int32, (H, LANES), 1)
    scale = DH ** -0.5

    top = {a: lane >= LANES - a for a in (2, 4, 6, 8)}
    low8 = lane < 8

    def shift_back(prev, cur, a):
        return pltpu.roll(jax.lax.select(top[a], prev, cur), a, 1)

    def shift_fwd8(cur, nxt):
        return pltpu.roll(jax.lax.select(low8, nxt, cur), LANES - 8, 1)

    def tree(op, vs):
        while len(vs) > 1:
            vs = [op(vs[i], vs[i + 1]) for i in range(0, len(vs), 2)]
        return vs[0]

    hist = []

    def s1_tile(t, res, hold=None):
        tn = min(t + 1, NT - 1)
        tp = max(t - 1, 0)
        acc = [None] * WIN
        for d in range(DH):
            rq = pl.ds(2 * d * H, H)
            rk = pl.ds((2 * d + 1) * H, H)
            q0 = qk_s[t, rq, :]
            k0 = qk_s[t, rk, :]
            if hold is None:
                qn = res[2 * d * H:(2 * d + 1) * H, :]
                k0 = tie(k0, qn)
            else:
                qn = q0
                k0 = hold(k0)
                qn = tie(qn, k0)
            kp = qk_s[tp, rk, :]
            pre = [jax.lax.select(low8, qn, q0)] + [jax.lax.select(top[a], kp, k0) for a in (2, 4, 6)]
            if len(hist) >= S1_LAG:
                pre = [tie(pre[i], hist[-S1_LAG][4 * (d % 2) + i]) for i in range(4)]
            q8 = pltpu.roll(pre[0], LANES - 8, 1)
            ks = [k0] + [pltpu.roll(pre[i], 2 * i, 1) for i in (1, 2, 3)]
            for a in range(4):
                t0 = q0 * ks[a]
                t8 = q8 * ks[a]
                acc[a] = t0 if d == 0 else acc[a] + t0
                acc[4 + a] = t8 if d == 0 else acc[4 + a] + t8
            hist.append(list(acc))
        for a in range(WIN):
            l_s[t, pl.ds(a * H, H), :] = acc[a]
        return tree(jnp.add, acc)

    def softmax_job(t, hh):
        tp = max(t - 1, 0)
        lane8 = lane[0:8]

        def rows(j):
            return pl.ds(j * H + hh * 8, 8)
        lg = [l_s[t, rows(j), :] for j in range(WIN)]
        for j in range(4, WIN):
            lg[j] = pltpu.roll(jnp.where(lane8 >= LANES - 8, l_s[tp, rows(j), :], lg[j]), 8, 1)
        if t == 0:
            lg = [lg[0]] + [jnp.where(lane8 >= DIL * j, lg[j], -1e9 / scale) for j in range(1, WIN)]
        m = tree(jnp.maximum, lg)
        e = [jnp.exp2((v - m) * (scale * LOG2E)) for v in lg]
        ssum = tree(jnp.add, e)
        inv = pl.reciprocal(ssum, approx=True)
        inv = inv * (2.0 - ssum * inv)
        for j in range(WIN):
            p_s[t, rows(j), :] = e[j] * inv

    def s2_tile(t, hold):
        tn = min(t + 1, NT - 1)
        tp = max(t - 1, 0)
        p0 = [p_s[t, pl.ds(a * H, H), :] for a in range(4)]
        p8 = [shift_fwd8(p_s[t, pl.ds((4 + a) * H, H), :], p_s[tn, pl.ds((4 + a) * H, H), :])
              for a in range(4)]
        for d in range(DH):
            r = pl.ds(d * H, H)
            v0 = hold(v_s[t, r, :])
            vp = v_s[tp, r, :]
            vs = [v0] + [shift_back(vp, v0, a) for a in (2, 4, 6)]
            o0 = (p0[0] * vs[0] + p0[1] * vs[1]) + (p0[2] * vs[2] + p0[3] * vs[3])
            o8 = (p8[0] * vs[0] + p8[1] * vs[1]) + (p8[2] * vs[2] + p8[3] * vs[3])
            o = o0 + shift_back(o8_s[r, :], o8, 8)
            o8_s[r, :] = o8
            o_s[t, r, :] = o.astype(BF16)

    def proj(dst, rows0, nrows, t, after=None):
        xn = xn_s[t]
        if after is not None:
            xn = jnp.concatenate([_unpack(tie(_pack(xn[0:2 * H]), after)), xn[2 * H:]], axis=0)
        res = _dot(_unpack(wt_s[pl.ds(rows0 // 2, nrows // 2), :]), xn)
        dst[t] = res
        return res

    b1 = b1_v[...].astype(F32).reshape(1, F)
    GR = 32
    gelu_jobs = [(j, rr) for j in range(NF) for rr in range(D // GR)]

    def gelu_job(j, rr, hold):
        bias = hold(jnp.broadcast_to(b1[:, j * LANES:(j + 1) * LANES], (8, LANES)))
        bias = jnp.concatenate([bias, bias], axis=0)
        for q in range(GR // H):
            row = rr * GR + q * H
            g_s[j, pl.ds(row, H), :] = _gelu(u_s[j, pl.ds(row, H), :] + bias).astype(BF16)

    def spread_gelu(res, njobs, lo=0.0, hi=1.0):
        njobs = min(njobs, len(gelu_jobs))
        hold = make_hold(tie, res, 1, njobs, lo, hi)
        for _ in range(njobs):
            gelu_job(*gelu_jobs.pop(0), hold)

    for half in range(2):
        ts = range(half * NT // 2, (half + 1) * NT // 2)
        fin = []
        for t in ts:
            res = proj(qk_s, 0, 2 * D, t, fin.pop(0) if len(fin) >= 2 else None)
            if t == 0:
                spread_gelu([res], 20)
            else:
                fin.append(s1_tile(t - 1, res))
                if half == 0:
                    fin.pop()
        vres = []
        ts = range(V_EARLY) if half == 0 else range(V_EARLY, NT)
        for t in ts:
            k = t - ts[0]
            vres.append(proj(v_s, 2 * D, D, t, fin.pop(0) if fin and k in (0, 2, 5) else None))
            if half == 1 and k == 1:
                fin.append(s1_tile(NT - 1, None, make_hold(tie, vres, 1, DH)))
        if half == 0:
            spread_gelu(vres, 12 * V_EARLY - 4, 0.1, 0.93)
        else:
            spread_gelu(vres[:2], 8)
            spread_gelu(vres[2:], 200)
        if half == 0:
            with jax.named_scope("w2_wait"):
                c_w2.wait()

            @pl.when(never_scalar)
            def _():
                o8_s[...] = jnp.zeros_like(o8_s)

            tie = make_tie(0)
            hist.clear()
    assert not gelu_jobs
    for t in range(NT):
        softmax_job(t, 0)
        softmax_job(t, 1)

    n3 = NT // P3_T
    c3 = P3_T * LANES

    out_copies = []

    def out_copy(t, r0, nr):
        c = pltpu.make_async_copy(out_v.at[t, pl.ds(r0, nr), :],
                                  out_hbm.at[pl.ds(r0, nr), pl.ds(t * LANES, LANES)], sems.at[SEM_OUT])
        c.start()
        out_copies.append(c)

    b2 = b2_v[...].astype(F32).reshape(1, S)
    ksplit = ((0, 4), (4, 8), (8, 12), (12, 14))
    gs = [tiles(g_s, k0, k1 - k0) for k0, k1 in ksplit]
    for i in range(n3):
        ys = []
        for g, (k0, k1) in zip(gs, ksplit):
            y = _dot(g,
                     w2_v[pl.ds(k0 * LANES, (k1 - k0) * LANES), pl.ds(i * c3, c3)])
            ys.append(y + ys[-1] if ys else y)
        hold = make_hold(tie, ys[:3], 1, P3_T * DH, 0.0, 0.9)
        for j in range(P3_T):
            s2_tile(i * P3_T + j, hold)
        y = _dot(_unpack(wot_s[...]), tiles(o_s, i * P3_T, P3_T)) + ys[-1]
        for j in range(P3_T):
            t = i * P3_T + j
            bias = jnp.broadcast_to(b2[:, t * LANES:(t + 1) * LANES], (H, LANES))
            for d in range(DH):
                r = pl.ds(d * H, H)
                val = x_v[t, r, :].astype(F32) + (y[d * H:(d + 1) * H, j * LANES:(j + 1) * LANES] + bias)
                out_v[t, r, :] = val.astype(BF16)
                if t == NT - 1 and (d + 1) * H in OUT_SPLIT:
                    r0 = ([0] + OUT_SPLIT)[OUT_SPLIT.index((d + 1) * H)]
                    out_copy(t, r0, (d + 1) * H - r0)
            if t < NT - 1:
                out_copy(t, 0, D)

    with jax.named_scope("out_wait"):
        for c in out_copies:
            c.wait()


@jax.jit
def pallas_parallel_sum__sliding_local_dilated__mixer_token_mlp__prompt_kernel(
    A_x: jax.Array,
    A_wqkv: jax.Array,
    A_wo: jax.Array,
    B_x: jax.Array,
    B_w1: jax.Array,
    B_b1: jax.Array,
    B_w2: jax.Array,
    B_b2: jax.Array,
):
    del B_x
    xt = jnp.transpose(A_x[0], (1, 0))
    any_spec = pl.BlockSpec(memory_space=pl.ANY)
    out_t = pl.pallas_call(
        _kernel,
        out_shape=jax.ShapeDtypeStruct((D, S), BF16),
        in_specs=[any_spec] * 7,
        out_specs=any_spec,
        scratch_shapes=[
            pltpu.VMEM((NT, D, LANES), BF16),
            pltpu.VMEM((S, F), BF16),
            pltpu.VMEM((F, S + LANES), BF16),
            pltpu.VMEM((D, 3 * D), BF16),
            pltpu.VMEM((D, D), BF16),
            pltpu.VMEM((F,), BF16),
            pltpu.VMEM((S,), BF16),
            pltpu.VMEM((NT, D, LANES), BF16),
            pltpu.VMEM((NT, D, LANES), BF16),
            pltpu.VMEM((NF, D, LANES), F32),
            pltpu.VMEM((NF, D, LANES), BF16),
            pltpu.VMEM((3 * D // 2, D), U32),
            pltpu.VMEM((D // 2, D), U32),
            pltpu.VMEM((4, 3 * D + 32, LANES), F32),
            pltpu.VMEM((4, D + 32, LANES), F32),
            pltpu.VMEM((NT, 2 * D, LANES), F32),
            pltpu.VMEM((NT, D, LANES), F32),
            pltpu.VMEM((NT, WIN * H, LANES), F32),
            pltpu.VMEM((NT, WIN * H, LANES), F32),
            pltpu.VMEM((D, LANES), F32),
            pltpu.VMEM((NT, D, LANES), BF16),
            pltpu.VMEM((NT, D, LANES), BF16),
            pltpu.VMEM((2, 8, LANES), F32),
            pltpu.SemaphoreType.DMA((N1 + 4,)),
        ],
        compiler_params=pltpu.CompilerParams(vmem_limit_bytes=100 * 1024 * 1024,
                                             disable_bounds_checks=True,
                                             disable_semaphore_checks=True),
    )(xt, A_wqkv, A_wo, B_w1, B_b1, B_w2, B_b2)
    return jnp.transpose(out_t, (1, 0))[None]
```

```python
import jax
import jax.numpy as jnp
import jax.experimental.pallas as pl
import jax.experimental.pallas.tpu as pltpu

S = 2048
D = 448
F = 1792
H = 16
DH = D // H
WIN = 8
DIL = 2
EPS = 1e-5
LOG2E = 1.4426950408889634
LANES = 128
NT = S // LANES
NF = F // LANES
F32 = jnp.float32
BF16 = jnp.bfloat16
U32 = jnp.uint32

P1_T = 2
P3_T = 2
N1 = NT // P1_T
V_EARLY = 5
OUT_SPLIT = [224, 384, D]
S1_LAG = 6
NA = 6


def _dot(a, b):
    return jnp.dot(a, b, preferred_element_type=F32)


def _gelu(x):
    c = 0.7978845608028654
    inner = x * (c + (c * 0.044715) * (x * x))
    hx = 0.5 * x
    return hx + hx * jnp.tanh(inner)


def _pack(v):
    return pltpu.bitcast(v.astype(BF16), U32)


def _unpack(v):
    return pltpu.bitcast(v, BF16)


def _kernel(x_hbm, wqkv_hbm, wo_hbm, w1_hbm, b1_hbm, w2_hbm, b2_hbm, out_hbm,
            x_v, w1_v, w2_v, wqkv_v, wo_v, b1_v, b2_v,
            xn_s, h_s, u_s, g_s, wt_s, wot_s, t32, o32, qk_s, v_s, l_s, p_s, o8_s, o_s, out_v, z_s,
            sems):
    c1 = P1_T * LANES
    SEM_LAST, SEM_W2, SEM_OUT = N1 + 1, N1 + 2, N1 + 3

    def x_copy(t, sem):
        col = t * LANES if isinstance(t, int) else pl.multiple_of(t * LANES, LANES)
        return pltpu.make_async_copy(x_hbm.at[:, pl.ds(col, LANES)], x_v.at[t], sems.at[sem])

    def w1_copy(row, sem, col=0, ncol=F):
        return pltpu.make_async_copy(w1_hbm.at[pl.ds(row, c1), pl.ds(col, ncol)],
                                     w1_v.at[pl.ds(row, c1), pl.ds(col, ncol)], sems.at[sem])

    def step_copies(i):
        row = i * c1 if isinstance(i, int) else pl.multiple_of(i * c1, c1)
        return [x_copy((i + 1) * P1_T + j, 2 + i) for j in range(P1_T)] + [w1_copy(row, 2 + i)]

    copies_0 = [x_copy(0, 0), x_copy(1, 0)]
    copies_a = [w1_copy(0, 1, 0, NA * LANES)]
    copies_b = [x_copy(2, 2), x_copy(3, 2), w1_copy(0, 2, NA * LANES, F - NA * LANES)]
    c_w1_last = w1_copy((N1 - 1) * c1, SEM_LAST)
    small = [pltpu.make_async_copy(src, dst, sems.at[SEM_LAST])
             for src, dst in ((b1_hbm, b1_v), (wqkv_hbm, wqkv_v))]
    late = [pltpu.make_async_copy(src, dst, sems.at[SEM_W2])
            for src, dst in ((b2_hbm, b2_v), (wo_hbm, wo_v), (w2_hbm, w2_v.at[:, pl.ds(0, S)]))]

    for c in copies_0 + copies_a + copies_b:
        c.start()
    for i in range(1, N1 - 1):
        for c in step_copies(i):
            c.start()
    c_w1_last.start()
    for c in small + late:
        c.start(priority=1)

    z_s[...] = jnp.zeros_like(z_s)
    o8_s[...] = jnp.zeros_like(o8_s)

    def make_tie(zi):
        never8 = z_s[zi] != 0.0
        never16 = jnp.concatenate([z_s[zi], z_s[zi]], axis=0) != 0.0

        def tie(val, src):
            if val.dtype != src.dtype:
                src = pltpu.bitcast(src, val.dtype)
            if val.shape[0] == 16 and src.shape[0] == 8:
                src = jnp.concatenate([src, src], axis=0)
            return jax.lax.select(never8 if val.shape[0] == 8 else never16, src, val)
        return tie

    def make_hold(tie, results, ntile_par, n, lo=0.0, hi=1.0):
        pts = []
        for res in results:
            for c in range(0, res.shape[1] // LANES, ntile_par):
                pts += [(res, r, c * LANES) for r in range(0, res.shape[0], 8)]
        state = [0]

        def hold(v):
            k = state[0]
            state[0] += 1
            assert k < n
            res, row, col = pts[min(int((lo + (hi - lo) * k / n) * len(pts)), len(pts) - 1)]
            return tie(v, res[row:row + 8, col:col + LANES])
        return hold

    LG = 7
    NH = 6 * (DH // LG)

    def ln_pass(ld, dst, t, hold):
        def colmean(f, c):
            acc = None
            for g in range(DH // LG):
                cg = hold(c)
                cg = jnp.concatenate([cg, cg], axis=0)
                part = None
                for d in range(g * LG, (g + 1) * LG):
                    v = f(ld(d), cg, d == g * LG)
                    part = v if part is None else part + v
                acc = part if acc is None else acc + part
            m = jnp.sum(acc, axis=0, keepdims=True) * (1.0 / D)
            return jnp.broadcast_to(m, (8, LANES))

        def sq(v, m, first):
            c = v - m
            return c * c
        m = colmean(lambda v, c, first: v + c if first else v, jnp.zeros((8, LANES), F32))
        r = jax.lax.rsqrt(colmean(sq, m) + EPS)
        r = jnp.concatenate([r, r], axis=0)
        for g in range(DH // LG):
            mg = hold(m)
            mg = jnp.concatenate([mg, mg], axis=0)
            for d in range(g * LG, (g + 1) * LG):
                dst[t, pl.ds(d * H, H), :] = ((ld(d) - mg) * r).astype(BF16)

    def ln_tile(t, hold):
        ln_pass(lambda d: x_v[t, pl.ds(d * H, H), :].astype(F32), xn_s, t, hold)
        ln_pass(lambda d: xn_s[t, pl.ds(d * H, H), :].astype(F32), h_s, t, hold)

    def tiles(ref, t0, nt):
        return jnp.concatenate([ref[t0 + j] for j in range(nt)], axis=1)

    def mixer1(i, j0=0, j1=NF, first=False):
        row = i * c1 if isinstance(i, int) else pl.multiple_of(i * c1, c1)
        part = _dot(tiles(h_s, i * P1_T, P1_T), w1_v[pl.ds(row, c1), pl.ds(j0 * LANES, (j1 - j0) * LANES)])
        for j in range(j0, j1):
            pj = part[:, (j - j0) * LANES:(j - j0 + 1) * LANES]
            if first:
                u_s[j] = pj
            else:
                u_s[j] += pj
        return part

    with jax.named_scope("wait_x0"):
        for c in copies_0:
            c.wait()
    never_scalar = z_s[0, 0, 0] != 0.0
    with jax.named_scope("ln0"):
        ln_tile(0, lambda v: v)
        ln_tile(1, lambda v: v)

    with jax.named_scope("wait_a"):
        for c in copies_a:
            c.wait()
    mixer1(0, 0, NA, first=True)

    with jax.named_scope("wait_b"):
        for c in copies_b:
            c.wait()
    tie = make_tie(0)
    part = mixer1(0, NA, NF, first=True)
    hold = make_hold(tie, [part], 2, 2 * NH, 0.0, 0.85)
    ln_tile(2, hold)
    ln_tile(3, hold)

    def p1_body(i, carry):
        with jax.named_scope("p1_wait"):
            for c in step_copies(i):
                c.wait()
        tie = make_tie(jnp.minimum(i, 1))
        part = mixer1(i)
        hold = make_hold(tie, [part], 2, P1_T * NH, 0.0, 0.9)
        for j in range(P1_T):
            ln_tile((i + 1) * P1_T + j, hold)
        return carry

    jax.lax.fori_loop(1, N1 - 2, p1_body, 0)

    with jax.named_scope("big_wait"):
        for c in step_copies(N1 - 2) + [c_w1_last] + small:
            c.wait()
    tie = make_tie(0)
    part = mixer1(N1 - 2)
    hold = make_hold(tie, [part], 2, P1_T * NH, 0.0, 0.8)
    for j in range(P1_T):
        ln_tile((N1 - 1) * P1_T + j, hold)
    part = mixer1(N1 - 1)

    def wt_transpose(j, hold):
        n = min(LANES, 3 * D - j * LANES)
        for c in range(4):
            r = min(LANES, D - c * LANES)
            blk = wqkv_v[pl.ds(c * LANES, r), pl.ds(j * LANES, n)]
            if n == LANES:
                blk = jnp.concatenate([_unpack(hold(_pack(blk[0:H]))), blk[H:]], axis=0)
            t32[c, pl.ds(j * LANES, n), pl.ds(0, r)] = blk.astype(F32).T

    def wt_gather(p):
        for d in range(DH):
            dst = (2 * d + p) * 8 if p < 2 else (2 * DH + d) * 8
            for c in range(4):
                r = min(LANES, D - c * LANES)
                v = t32[c, pl.ds(p * D + d, H, stride=DH), pl.ds(0, r)]
                wt_s[pl.ds(dst, 8), pl.ds(c * LANES, r)] = _pack(v)

    hold = make_hold(tie, [part], 2, 40, 0.0, 0.75)
    for j in range(7):
        wt_transpose(j, hold)
    wt_gather(0)
    wt_gather(1)
    for j in range(7, 11):
        wt_transpose(j, hold)
    wt_gather(2)

    def wo_prep(hold):
        for c in range(4):
            r = min(LANES, D - c * LANES)
            for g in range(4):
                blk = wo_v[pl.ds(g * 112, 112), pl.ds(c * LANES, r)].astype(F32)
                if r == LANES:
                    blk = jnp.concatenate([hold(blk[q * 8:q * 8 + 8]) for q in range(14)], axis=0)
                o32[c, pl.ds(g * 112, 112), pl.ds(0, r)] = blk
        chk = None
        for c in range(4):
            r = min(LANES, D - c * LANES)
            rows = jnp.concatenate(
                [o32[c, pl.ds(d, H, stride=DH), pl.ds(0, r)] for d in range(DH)], axis=0)
            w = _pack(rows.T)
            wot_s[pl.ds(c * 64, r // 2), :] = w
            for q in range(0, r // 2, 8):
                chk = w[q:q + 8] if chk is None else chk | w[q:q + 8]
        return (chk[:, 0:LANES] | chk[:, LANES:2 * LANES]) | (chk[:, 2 * LANES:3 * LANES] | chk[:, D - LANES:D])

    lane = jax.lax.broadcasted_iota(jnp.int32, (H, LANES), 1)
    scale = DH ** -0.5

    top = {a: lane >= LANES - a for a in (2, 4, 6, 8)}
    low8 = lane < 8

    def shift_back(prev, cur, a):
        return pltpu.roll(jax.lax.select(top[a], prev, cur), a, 1)

    def shift_fwd8(cur, nxt):
        return pltpu.roll(jax.lax.select(low8, nxt, cur), LANES - 8, 1)

    def tree(op, vs):
        while len(vs) > 1:
            vs = [op(vs[i], vs[i + 1]) for i in range(0, len(vs), 2)]
        return vs[0]

    hist = []

    def s1_tile(t, res, hold=None):
        tp = max(t - 1, 0)
        acc = [None] * WIN
        for d in range(DH):
            rq = pl.ds(2 * d * H, H)
            rk = pl.ds((2 * d + 1) * H, H)
            q0 = qk_s[t, rq, :]
            k0 = qk_s[t, rk, :]
            if hold is None:
                qn = res[2 * d * H:(2 * d + 1) * H, :]
                k0 = tie(k0, qn)
            else:
                qn = q0
                k0 = hold(k0)
                qn = tie(qn, k0)
            kp = qk_s[tp, rk, :]
            pre = [jax.lax.select(low8, qn, q0)] + [jax.lax.select(top[a], kp, k0) for a in (2, 4, 6)]
            if len(hist) >= S1_LAG:
                pre = [tie(pre[i], hist[-S1_LAG][4 * (d % 2) + i]) for i in range(4)]
            q8 = pltpu.roll(pre[0], LANES - 8, 1)
            ks = [k0] + [pltpu.roll(pre[i], 2 * i, 1) for i in (1, 2, 3)]
            for a in range(4):
                t0 = q0 * ks[a]
                t8 = q8 * ks[a]
                acc[a] = t0 if d == 0 else acc[a] + t0
                acc[4 + a] = t8 if d == 0 else acc[4 + a] + t8
            hist.append(list(acc))
        for a in range(WIN):
            l_s[t, pl.ds(a * H, H), :] = acc[a]
        return tree(jnp.add, acc)

    def softmax_job(t, hh):
        tp = max(t - 1, 0)
        lane8 = lane[0:8]

        def rows(j):
            return pl.ds(j * H + hh * 8, 8)
        lg = [l_s[t, rows(j), :] for j in range(WIN)]
        for j in range(4, WIN):
            lg[j] = pltpu.roll(jnp.where(lane8 >= LANES - 8, l_s[tp, rows(j), :], lg[j]), 8, 1)
        if t == 0:
            lg = [lg[0]] + [jnp.where(lane8 >= DIL * j, lg[j], -1e9 / scale) for j in range(1, WIN)]
        m = tree(jnp.maximum, lg)
        e = [jnp.exp2((v - m) * (scale * LOG2E)) for v in lg]
        ssum = tree(jnp.add, e)
        inv = pl.reciprocal(ssum, approx=True)
        inv = inv * (2.0 - ssum * inv)
        for j in range(WIN):
            p_s[t, rows(j), :] = e[j] * inv

    def s2_tile(t, hold):
        tn = min(t + 1, NT - 1)
        tp = max(t - 1, 0)
        p0 = [p_s[t, pl.ds(a * H, H), :] for a in range(4)]
        p8 = [shift_fwd8(p_s[t, pl.ds((4 + a) * H, H), :], p_s[tn, pl.ds((4 + a) * H, H), :])
              for a in range(4)]
        for d in range(DH):
            r = pl.ds(d * H, H)
            v0 = hold(v_s[t, r, :])
            vp = v_s[tp, r, :]
            vs = [v0] + [shift_back(vp, v0, a) for a in (2, 4, 6)]
            o0 = (p0[0] * vs[0] + p0[1] * vs[1]) + (p0[2] * vs[2] + p0[3] * vs[3])
            o8 = (p8[0] * vs[0] + p8[1] * vs[1]) + (p8[2] * vs[2] + p8[3] * vs[3])
            o = o0 + shift_back(o8_s[r, :], o8, 8)
            o8_s[r, :] = o8
            o_s[t, r, :] = o.astype(BF16)

    def proj(dst, rows0, nrows, t, after=None):
        xn = xn_s[t]
        if after is not None:
            xn = jnp.concatenate([_unpack(tie(_pack(xn[0:2 * H]), after)), xn[2 * H:]], axis=0)
        res = _dot(_unpack(wt_s[pl.ds(rows0 // 2, nrows // 2), :]), xn)
        dst[t] = res
        return res

    b1 = b1_v[...].astype(F32).reshape(1, F)
    GR = 32
    gelu_jobs = [(j, rr) for j in range(NF) for rr in range(D // GR)]

    def gelu_job(j, rr, hold):
        bias = hold(jnp.broadcast_to(b1[:, j * LANES:(j + 1) * LANES], (8, LANES)))
        bias = jnp.concatenate([bias, bias], axis=0)
        for q in range(GR // H):
            row = rr * GR + q * H
            g_s[j, pl.ds(row, H), :] = _gelu(u_s[j, pl.ds(row, H), :] + bias).astype(BF16)

    def spread_gelu(res, njobs, lo=0.0, hi=1.0):
        njobs = min(njobs, len(gelu_jobs))
        hold = make_hold(tie, res, 1, njobs, lo, hi)
        for _ in range(njobs):
            gelu_job(*gelu_jobs.pop(0), hold)

    for half in range(2):
        ts = range(half * NT // 2, (half + 1) * NT // 2)
        fin = []
        for t in ts:
            res = proj(qk_s, 0, 2 * D, t, fin.pop(0) if len(fin) >= 2 else None)
            if t == 0:
                spread_gelu([res], 20)
            else:
                fin.append(s1_tile(t - 1, res))
                if half == 0:
                    fin.pop()
        vres = []
        ts = range(V_EARLY) if half == 0 else range(V_EARLY, NT)
        for t in ts:
            k = t - ts[0]
            vres.append(proj(v_s, 2 * D, D, t, fin.pop(0) if fin and k in (0, 2, 5, 9) else None))
            if half == 1 and k == 1:
                fin.append(s1_tile(NT - 1, None, make_hold(tie, vres, 1, DH)))
            if half == 1 and k == 5:
                fin.append(wo_prep(make_hold(tie, vres[3:], 1, 3 * 56)))
        if half == 0:
            spread_gelu(vres, 12 * V_EARLY - 4, 0.1, 0.93)
        else:
            spread_gelu(vres[:2], 8)
            spread_gelu(vres[2:], 200)
        if half == 0:
            with jax.named_scope("w2_wait"):
                for c in late:
                    c.wait()

            @pl.when(never_scalar)
            def _():
                o8_s[...] = jnp.zeros_like(o8_s)

            tie = make_tie(0)
            hist.clear()
    assert not gelu_jobs
    for t in range(NT):
        softmax_job(t, 0)
        softmax_job(t, 1)

    n3 = NT // P3_T
    c3 = P3_T * LANES

    out_copies = []

    def out_copy(t, r0, nr):
        c = pltpu.make_async_copy(out_v.at[t, pl.ds(r0, nr), :],
                                  out_hbm.at[pl.ds(r0, nr), pl.ds(t * LANES, LANES)], sems.at[SEM_OUT])
        c.start()
        out_copies.append(c)

    b2 = b2_v[...].astype(F32).reshape(1, S)
    ksplit = ((0, 4), (4, 8), (8, 12), (12, 14))
    gs = [tiles(g_s, k0, k1 - k0) for k0, k1 in ksplit]
    for i in range(n3):
        ys = []
        for g, (k0, k1) in zip(gs, ksplit):
            y = _dot(g, w2_v[pl.ds(k0 * LANES, (k1 - k0) * LANES), pl.ds(i * c3, c3)])
            ys.append(y + ys[-1] if ys else y)
        hold = make_hold(tie, ys[:3], 1, P3_T * DH, 0.0, 0.9)
        for j in range(P3_T):
            s2_tile(i * P3_T + j, hold)
        y = _dot(_unpack(wot_s[...]), tiles(o_s, i * P3_T, P3_T)) + ys[-1]
        for j in range(P3_T):
            t = i * P3_T + j
            bias = jnp.broadcast_to(b2[:, t * LANES:(t + 1) * LANES], (H, LANES))
            for d in range(DH):
                r = pl.ds(d * H, H)
                val = x_v[t, r, :].astype(F32) + (y[d * H:(d + 1) * H, j * LANES:(j + 1) * LANES] + bias)
                out_v[t, r, :] = val.astype(BF16)
                if t == NT - 1 and (d + 1) * H in OUT_SPLIT:
                    r0 = ([0] + OUT_SPLIT)[OUT_SPLIT.index((d + 1) * H)]
                    out_copy(t, r0, (d + 1) * H - r0)
            if t < NT - 1:
                out_copy(t, 0, D)

    with jax.named_scope("out_wait"):
        for c in out_copies:
            c.wait()


@jax.jit
def pallas_parallel_sum__sliding_local_dilated__mixer_token_mlp__prompt_kernel(
    A_x: jax.Array,
    A_wqkv: jax.Array,
    A_wo: jax.Array,
    B_x: jax.Array,
    B_w1: jax.Array,
    B_b1: jax.Array,
    B_w2: jax.Array,
    B_b2: jax.Array,
):
    del B_x
    xt = jnp.transpose(A_x[0], (1, 0))
    any_spec = pl.BlockSpec(memory_space=pl.ANY)
    out_t = pl.pallas_call(
        _kernel,
        out_shape=jax.ShapeDtypeStruct((D, S), BF16),
        in_specs=[any_spec] * 7,
        out_specs=any_spec,
        scratch_shapes=[
            pltpu.VMEM((NT, D, LANES), BF16),
            pltpu.VMEM((S, F), BF16),
            pltpu.VMEM((F, S + LANES), BF16),
            pltpu.VMEM((D, 3 * D), BF16),
            pltpu.VMEM((D, D), BF16),
            pltpu.VMEM((F,), BF16),
            pltpu.VMEM((S,), BF16),
            pltpu.VMEM((NT, D, LANES), BF16),
            pltpu.VMEM((NT, D, LANES), BF16),
            pltpu.VMEM((NF, D, LANES), F32),
            pltpu.VMEM((NF, D, LANES), BF16),
            pltpu.VMEM((3 * D // 2, D), U32),
            pltpu.VMEM((D // 2, D), U32),
            pltpu.VMEM((4, 3 * D + 32, LANES), F32),
            pltpu.VMEM((4, D + 32, LANES), F32),
            pltpu.VMEM((NT, 2 * D, LANES), F32),
            pltpu.VMEM((NT, D, LANES), F32),
            pltpu.VMEM((NT, WIN * H, LANES), F32),
            pltpu.VMEM((NT, WIN * H, LANES), F32),
            pltpu.VMEM((D, LANES), F32),
            pltpu.VMEM((NT, D, LANES), BF16),
            pltpu.VMEM((NT, D, LANES), BF16),
            pltpu.VMEM((2, 8, LANES), F32),
            pltpu.SemaphoreType.DMA((N1 + 4,)),
        ],
        compiler_params=pltpu.CompilerParams(vmem_limit_bytes=100 * 1024 * 1024,
                                             disable_bounds_checks=True,
                                             disable_semaphore_checks=True),
    )(xt, A_wqkv, A_wo, B_w1, B_b1, B_w2, B_b2)
    return jnp.transpose(out_t, (1, 0))[None]
```

```python
import jax
import jax.numpy as jnp
import jax.experimental.pallas as pl
import jax.experimental.pallas.tpu as pltpu

S = 2048
D = 448
F = 1792
H = 16
DH = D // H
WIN = 8
DIL = 2
EPS = 1e-5
LOG2E = 1.4426950408889634
LANES = 128
NT = S // LANES
NF = F // LANES
F32 = jnp.float32
BF16 = jnp.bfloat16
U32 = jnp.uint32

P1_T = 2
P3_T = 2
N1 = NT // P1_T
V_EARLY = 5
OUT_SPLIT = [224, 352, 416, D]
S1_LAG = 6
NA = 6


def _dot(a, b):
    return jnp.dot(a, b, preferred_element_type=F32)


def _gelu(x):
    c = 0.7978845608028654
    inner = x * (c + (c * 0.044715) * (x * x))
    hx = 0.5 * x
    return hx + hx * jnp.tanh(inner)


def _pack(v):
    return pltpu.bitcast(v.astype(BF16), U32)


def _unpack(v):
    return pltpu.bitcast(v, BF16)


def _kernel(x_hbm, wqkv_hbm, wo_hbm, w1_hbm, b1_hbm, w2_hbm, b2_hbm, out_hbm,
            x_v, w1_v, w2_v, wqkv_v, wo_v, b1_v, b2_v,
            xn_s, h_s, u_s, g_s, wt_s, wot_s, t32, o32, qk_s, v_s, l_s, p_s, o8_s, o_s, out_v, z_s,
            sems):
    c1 = P1_T * LANES
    SEM_LAST, SEM_W2, SEM_OUT = N1 + 1, N1 + 2, N1 + 3

    def x_copy(t, sem):
        col = t * LANES if isinstance(t, int) else pl.multiple_of(t * LANES, LANES)
        return pltpu.make_async_copy(x_hbm.at[:, pl.ds(col, LANES)], x_v.at[t], sems.at[sem])

    def w1_copy(row, sem, col=0, ncol=F):
        return pltpu.make_async_copy(w1_hbm.at[pl.ds(row, c1), pl.ds(col, ncol)],
                                     w1_v.at[pl.ds(row, c1), pl.ds(col, ncol)], sems.at[sem])

    def step_copies(i):
        row = i * c1 if isinstance(i, int) else pl.multiple_of(i * c1, c1)
        return [x_copy((i + 1) * P1_T + j, 2 + i) for j in range(P1_T)] + [w1_copy(row, 2 + i)]

    copies_0 = [x_copy(0, 0), x_copy(1, 0)]
    copies_a = [w1_copy(0, 1, 0, NA * LANES)]
    copies_b = [x_copy(2, 2), x_copy(3, 2), w1_copy(0, 2, NA * LANES, F - NA * LANES)]
    c_w1_last = w1_copy((N1 - 1) * c1, SEM_LAST)
    small = [pltpu.make_async_copy(src, dst, sems.at[SEM_LAST])
             for src, dst in ((b1_hbm, b1_v), (wqkv_hbm, wqkv_v))]
    late = [pltpu.make_async_copy(src, dst, sems.at[SEM_W2])
            for src, dst in ((b2_hbm, b2_v), (wo_hbm, wo_v), (w2_hbm, w2_v.at[:, pl.ds(0, S)]))]

    for c in copies_0 + copies_a + copies_b:
        c.start()
    for i in range(1, N1 - 1):
        for c in step_copies(i):
            c.start()
    c_w1_last.start()
    for c in small + late:
        c.start(priority=1)

    z_s[...] = jnp.zeros_like(z_s)
    o8_s[...] = jnp.zeros_like(o8_s)

    def make_tie(zi):
        never8 = z_s[zi] != 0.0
        never16 = jnp.concatenate([z_s[zi], z_s[zi]], axis=0) != 0.0

        def tie(val, src):
            if val.dtype != src.dtype:
                src = pltpu.bitcast(src, val.dtype)
            if val.shape[0] == 16 and src.shape[0] == 8:
                src = jnp.concatenate([src, src], axis=0)
            return jax.lax.select(never8 if val.shape[0] == 8 else never16, src, val)
        return tie

    def make_hold(tie, results, ntile_par, n, lo=0.0, hi=1.0):
        pts = []
        for res in results:
            for c in range(0, res.shape[1] // LANES, ntile_par):
                pts += [(res, r, c * LANES) for r in range(0, res.shape[0], 8)]
        state = [0]

        def hold(v):
            k = state[0]
            state[0] += 1
            assert k < n
            res, row, col = pts[min(int((lo + (hi - lo) * k / n) * len(pts)), len(pts) - 1)]
            return tie(v, res[row:row + 8, col:col + LANES])
        return hold

    LG = 7
    NH = 6 * (DH // LG)

    def slab(v, d):
        return v[d * H:(d + 1) * H]

    def ln_pass(src, dst, t, hold):
        def sweep(f, c):
            x = src[t]
            out = []
            for g in range(DH // LG):
                cg = hold(c)
                cg = jnp.concatenate([cg, cg], axis=0)
                out.append([f(slab(x, d).astype(F32), cg, d == g * LG)
                            for d in range(g * LG, (g + 1) * LG)])
            return out

        def colmean(groups):
            acc = None
            for vs in groups:
                part = vs[0]
                for v in vs[1:]:
                    part = part + v
                acc = part if acc is None else acc + part
            m = jnp.sum(acc, axis=0, keepdims=True) * (1.0 / D)
            return jnp.broadcast_to(m, (8, LANES))

        def sq(v, m, first):
            c = v - m
            return c * c
        m = colmean(sweep(lambda v, c, first: v + c if first else v, jnp.zeros((8, LANES), F32)))
        r = jax.lax.rsqrt(colmean(sweep(sq, m)) + EPS)
        r = jnp.concatenate([r, r], axis=0)
        for g in range(DH // LG):
            mg = hold(m)
            mg = jnp.concatenate([mg, mg], axis=0)
            for d in range(g * LG, (g + 1) * LG):
                rows = pl.ds(d * H, H)
                dst[t, rows, :] = ((src[t, rows, :].astype(F32) - mg) * r).astype(BF16)

    def ln_tile(t, hold):
        ln_pass(x_v, xn_s, t, hold)
        ln_pass(xn_s, h_s, t, hold)

    def tiles(ref, t0, nt):
        return jnp.concatenate([ref[t0 + j] for j in range(nt)], axis=1)

    def mixer1(i, j0=0, j1=NF, first=False):
        row = i * c1 if isinstance(i, int) else pl.multiple_of(i * c1, c1)
        part = _dot(tiles(h_s, i * P1_T, P1_T), w1_v[pl.ds(row, c1), pl.ds(j0 * LANES, (j1 - j0) * LANES)])
        for j in range(j0, j1):
            pj = part[:, (j - j0) * LANES:(j - j0 + 1) * LANES]
            if first:
                u_s[j] = pj
            else:
                u_s[j] += pj
        return part

    with jax.named_scope("wait_x0"):
        for c in copies_0:
            c.wait()
    never_scalar = z_s[0, 0, 0] != 0.0
    with jax.named_scope("ln0"):
        ln_tile(0, lambda v: v)
        ln_tile(1, lambda v: v)

    with jax.named_scope("wait_a"):
        for c in copies_a:
            c.wait()
    mixer1(0, 0, NA, first=True)

    with jax.named_scope("wait_b"):
        for c in copies_b:
            c.wait()
    tie = make_tie(0)
    part = mixer1(0, NA, NF, first=True)
    hold = make_hold(tie, [part], 2, 2 * NH, 0.0, 0.85)
    ln_tile(2, hold)
    ln_tile(3, hold)

    def p1_body(i, carry):
        with jax.named_scope("p1_wait"):
            for c in step_copies(i):
                c.wait()
        tie = make_tie(jnp.minimum(i, 1))
        part = mixer1(i)
        hold = make_hold(tie, [part], 2, P1_T * NH, 0.0, 0.9)
        for j in range(P1_T):
            ln_tile((i + 1) * P1_T + j, hold)
        return carry

    jax.lax.fori_loop(1, N1 - 2, p1_body, 0)

    with jax.named_scope("big_wait"):
        for c in step_copies(N1 - 2) + [c_w1_last] + small:
            c.wait()
    tie = make_tie(0)
    part = mixer1(N1 - 2)
    hold = make_hold(tie, [part], 2, P1_T * NH, 0.0, 0.8)
    for j in range(P1_T):
        ln_tile((N1 - 1) * P1_T + j, hold)
    part = mixer1(N1 - 1)

    def wt_transpose(j, hold):
        n = min(LANES, 3 * D - j * LANES)
        for c in range(4):
            r = min(LANES, D - c * LANES)
            blk = wqkv_v[pl.ds(c * LANES, r), pl.ds(j * LANES, n)]
            if n == LANES:
                blk = jnp.concatenate([_unpack(hold(_pack(blk[0:H]))), blk[H:]], axis=0)
            t32[c, pl.ds(j * LANES, n), pl.ds(0, r)] = blk.astype(F32).T

    def wt_gather(p):
        for d in range(DH):
            dst = (2 * d + p) * 8 if p < 2 else (2 * DH + d) * 8
            v = [t32[c, pl.ds(p * D + d, H, stride=DH), pl.ds(0, min(LANES, D - c * LANES))]
                 for c in range(4)]
            wt_s[pl.ds(dst, 8), :] = _pack(jnp.concatenate(v, axis=1))

    hold = make_hold(tie, [part], 2, 40, 0.0, 0.75)
    for j in range(7):
        wt_transpose(j, hold)
    wt_gather(0)
    wt_gather(1)
    for j in range(7, 11):
        wt_transpose(j, hold)
    wt_gather(2)

    def wo_prep(hold):
        for c in range(4):
            r = min(LANES, D - c * LANES)
            for g in range(4):
                blk = wo_v[pl.ds(g * 112, 112), pl.ds(c * LANES, r)].astype(F32)
                if r == LANES:
                    blk = jnp.concatenate([hold(blk[q * 8:q * 8 + 8]) for q in range(14)], axis=0)
                o32[c, pl.ds(g * 112, 112), pl.ds(0, r)] = blk
        chk = None
        for c in range(4):
            r = min(LANES, D - c * LANES)
            rows = jnp.concatenate(
                [o32[c, pl.ds(d, H, stride=DH), pl.ds(0, r)] for d in range(DH)], axis=0)
            w = _pack(rows.T)
            wot_s[pl.ds(c * 64, r // 2), :] = w
            for q in range(0, r // 2, 8):
                chk = w[q:q + 8] if chk is None else chk | w[q:q + 8]
        return (chk[:, 0:LANES] | chk[:, LANES:2 * LANES]) | (chk[:, 2 * LANES:3 * LANES] | chk[:, D - LANES:D])

    lane = jax.lax.broadcasted_iota(jnp.int32, (H, LANES), 1)
    scale = DH ** -0.5

    top = {a: lane >= LANES - a for a in (2, 4, 6, 8)}
    low8 = lane < 8

    def shift_back(prev, cur, a):
        return pltpu.roll(jax.lax.select(top[a], prev, cur), a, 1)

    def shift_fwd8(cur, nxt):
        return pltpu.roll(jax.lax.select(low8, nxt, cur), LANES - 8, 1)

    def tree(op, vs):
        while len(vs) > 1:
            vs = [op(vs[i], vs[i + 1]) for i in range(0, len(vs), 2)]
        return vs[0]

    hist = []

    def s1_tile(t, res, hold=None):
        tp = max(t - 1, 0)
        acc = [None] * WIN
        cur = qk_s[t]
        prev = qk_s[tp]
        for d in range(DH):
            q0 = slab(cur, 2 * d)
            k0 = slab(cur, 2 * d + 1)
            if hold is None:
                qn = slab(res, 2 * d)
                k0 = tie(k0, qn)
            else:
                qn = q0
                k0 = hold(k0)
                qn = tie(qn, k0)
            kp = slab(prev, 2 * d + 1)
            pre = [jax.lax.select(low8, qn, q0)] + [jax.lax.select(top[a], kp, k0) for a in (2, 4, 6)]
            if len(hist) >= S1_LAG:
                pre = [tie(pre[i], hist[-S1_LAG][4 * (d % 2) + i]) for i in range(4)]
            q8 = pltpu.roll(pre[0], LANES - 8, 1)
            ks = [k0] + [pltpu.roll(pre[i], 2 * i, 1) for i in (1, 2, 3)]
            for a in range(4):
                t0 = q0 * ks[a]
                t8 = q8 * ks[a]
                acc[a] = t0 if d == 0 else acc[a] + t0
                acc[4 + a] = t8 if d == 0 else acc[4 + a] + t8
            hist.append(list(acc))
        l_s[t] = jnp.concatenate(acc, axis=0)
        return tree(jnp.add, acc)

    def softmax_tile(t):
        cur = l_s[t]
        prev = l_s[max(t - 1, 0)]
        lg = [slab(cur, j) if j < 4 else shift_back(slab(prev, j), slab(cur, j), 8) for j in range(WIN)]
        if t == 0:
            lg = [lg[0]] + [jnp.where(lane >= DIL * j, lg[j], -1e9 / scale) for j in range(1, WIN)]
        m = tree(jnp.maximum, lg)
        e = [jnp.exp2((v - m) * (scale * LOG2E)) for v in lg]
        ssum = tree(jnp.add, e)
        inv = pl.reciprocal(ssum, approx=True)
        inv = inv * (2.0 - ssum * inv)
        p_s[t] = jnp.concatenate([v * inv for v in e], axis=0)

    def s2_tile(t, hold):
        p = p_s[t]
        pn = p_s[min(t + 1, NT - 1)]
        p0 = [slab(p, a) for a in range(4)]
        p8 = [shift_fwd8(slab(p, 4 + a), slab(pn, 4 + a)) for a in range(4)]
        cur = v_s[t]
        prev = v_s[max(t - 1, 0)]
        o8_prev = o8_s[...]
        os, o8s = [], []
        for d in range(DH):
            v0 = hold(slab(cur, d))
            vs = [v0] + [shift_back(slab(prev, d), v0, a) for a in (2, 4, 6)]
            o0 = (p0[0] * vs[0] + p0[1] * vs[1]) + (p0[2] * vs[2] + p0[3] * vs[3])
            o8 = (p8[0] * vs[0] + p8[1] * vs[1]) + (p8[2] * vs[2] + p8[3] * vs[3])
            os.append(o0 + shift_back(slab(o8_prev, d), o8, 8))
            o8s.append(o8)
        o8_s[...] = jnp.concatenate(o8s, axis=0)
        o_s[t] = jnp.concatenate(os, axis=0).astype(BF16)

    def proj(dst, rows0, nrows, t, after=None):
        xn = xn_s[t]
        if after is not None:
            xn = jnp.concatenate([_unpack(tie(_pack(xn[0:2 * H]), after)), xn[2 * H:]], axis=0)
        res = _dot(_unpack(wt_s[pl.ds(rows0 // 2, nrows // 2), :]), xn)
        dst[t] = res
        return res

    b1 = b1_v[...].astype(F32).reshape(1, F)
    GR = 32
    gelu_jobs = [(j, rr) for j in range(NF) for rr in range(D // GR)]

    def gelu_job(j, rr, hold):
        bias = hold(jnp.broadcast_to(b1[:, j * LANES:(j + 1) * LANES], (8, LANES)))
        bias = jnp.concatenate([bias] * (GR // 8), axis=0)
        rows = pl.ds(rr * GR, GR)
        g_s[j, rows, :] = _gelu(u_s[j, rows, :] + bias).astype(BF16)

    def spread_gelu(res, njobs, lo=0.0, hi=1.0):
        njobs = min(njobs, len(gelu_jobs))
        hold = make_hold(tie, res, 1, njobs, lo, hi)
        for _ in range(njobs):
            gelu_job(*gelu_jobs.pop(0), hold)

    for half in range(2):
        ts = range(half * NT // 2, (half + 1) * NT // 2)
        fin = []
        for t in ts:
            res = proj(qk_s, 0, 2 * D, t, fin.pop(0) if len(fin) >= 2 else None)
            if t == 0:
                spread_gelu([res], 20)
            else:
                fin.append(s1_tile(t - 1, res))
                if half == 0:
                    fin.pop()
        vres = []
        ts = range(V_EARLY) if half == 0 else range(V_EARLY, NT)
        for t in ts:
            k = t - ts[0]
            vres.append(proj(v_s, 2 * D, D, t, fin.pop(0) if fin and k in (0, 2, 5, 9) else None))
            if half == 1 and k == 1:
                fin.append(s1_tile(NT - 1, None, make_hold(tie, vres, 1, DH)))
            if half == 1 and k == 5:
                fin.append(wo_prep(make_hold(tie, vres[3:], 1, 3 * 56)))
        if half == 0:
            spread_gelu(vres, 12 * V_EARLY - 8, 0.1, 0.88)
        else:
            spread_gelu(vres[:2], 8)
            spread_gelu(vres[2:], 200, 0.0, 0.9)
        if half == 0:
            with jax.named_scope("w2_wait"):
                for c in late:
                    c.wait()

            @pl.when(never_scalar)
            def _():
                o8_s[...] = jnp.zeros_like(o8_s)

            tie = make_tie(0)
            hist.clear()
    assert not gelu_jobs
    for t in range(NT):
        softmax_tile(t)

    n3 = NT // P3_T
    c3 = P3_T * LANES

    out_copies = []

    def out_copy(t, r0, nr):
        c = pltpu.make_async_copy(out_v.at[t, pl.ds(r0, nr), :],
                                  out_hbm.at[pl.ds(r0, nr), pl.ds(t * LANES, LANES)], sems.at[SEM_OUT])
        c.start()
        out_copies.append(c)

    b2 = b2_v[...].astype(F32).reshape(1, S)
    ksplit = ((0, 4), (4, 8), (8, 12), (12, 14))
    gs = [tiles(g_s, k0, k1 - k0) for k0, k1 in ksplit]
    for i in range(n3):
        ys = []
        for g, (k0, k1) in zip(gs, ksplit):
            y = _dot(g, w2_v[pl.ds(k0 * LANES, (k1 - k0) * LANES), pl.ds(i * c3, c3)])
            ys.append(y + ys[-1] if ys else y)
        hold = make_hold(tie, ys[:3], 1, P3_T * DH, 0.0, 0.9)
        for j in range(P3_T):
            s2_tile(i * P3_T + j, hold)
        y = _dot(_unpack(wot_s[...]), tiles(o_s, i * P3_T, P3_T)) + ys[-1]
        for j in range(P3_T):
            t = i * P3_T + j
            val = x_v[t].astype(F32) + (y[:, j * LANES:(j + 1) * LANES] + b2[:, t * LANES:(t + 1) * LANES])
            ends = OUT_SPLIT if t == NT - 1 else [D]
            for r0, r1 in zip([0] + ends, ends):
                out_v[t, pl.ds(r0, r1 - r0), :] = val[r0:r1].astype(BF16)
                out_copy(t, r0, r1 - r0)

    with jax.named_scope("out_wait"):
        for c in out_copies:
            c.wait()


@jax.jit
def pallas_parallel_sum__sliding_local_dilated__mixer_token_mlp__prompt_kernel(
    A_x: jax.Array,
    A_wqkv: jax.Array,
    A_wo: jax.Array,
    B_x: jax.Array,
    B_w1: jax.Array,
    B_b1: jax.Array,
    B_w2: jax.Array,
    B_b2: jax.Array,
):
    del B_x
    xt = jnp.transpose(A_x.reshape(S, D), (1, 0))
    any_spec = pl.BlockSpec(memory_space=pl.ANY)
    out_t = pl.pallas_call(
        _kernel,
        out_shape=jax.ShapeDtypeStruct((D, S), BF16),
        in_specs=[any_spec] * 7,
        out_specs=any_spec,
        scratch_shapes=[
            pltpu.VMEM((NT, D, LANES), BF16),
            pltpu.VMEM((S, F), BF16),
            pltpu.VMEM((F, S + LANES), BF16),
            pltpu.VMEM((D, 3 * D), BF16),
            pltpu.VMEM((D, D), BF16),
            pltpu.VMEM((F,), BF16),
            pltpu.VMEM((S,), BF16),
            pltpu.VMEM((NT, D, LANES), BF16),
            pltpu.VMEM((NT, D, LANES), BF16),
            pltpu.VMEM((NF, D, LANES), F32),
            pltpu.VMEM((NF, D, LANES), BF16),
            pltpu.VMEM((3 * D // 2, D), U32),
            pltpu.VMEM((D // 2, D), U32),
            pltpu.VMEM((4, 3 * D + 32, LANES), F32),
            pltpu.VMEM((4, D + 32, LANES), F32),
            pltpu.VMEM((NT, 2 * D, LANES), F32),
            pltpu.VMEM((NT, D, LANES), F32),
            pltpu.VMEM((NT, WIN * H, LANES), F32),
            pltpu.VMEM((NT, WIN * H, LANES), F32),
            pltpu.VMEM((D, LANES), F32),
            pltpu.VMEM((NT, D, LANES), BF16),
            pltpu.VMEM((NT, D, LANES), BF16),
            pltpu.VMEM((2, 8, LANES), F32),
            pltpu.SemaphoreType.DMA((N1 + 4,)),
        ],
        compiler_params=pltpu.CompilerParams(vmem_limit_bytes=100 * 1024 * 1024,
                                             disable_bounds_checks=True,
                                             disable_semaphore_checks=True),
    )(xt, A_wqkv, A_wo, B_w1, B_b1, B_w2, B_b2)
    return jnp.transpose(out_t, (1, 0)).reshape(1, S, D)
```
